```python
import jax
import jax.numpy as jnp

def _softmax(x, axis=-1):
    return jax.nn.softmax(x, axis=axis)

def _gelu(x):
    return jax.nn.gelu(x, approximate=True)

def _silu(x):
    return jax.nn.silu(x)

def _sigmoid(x):
    return jax.nn.sigmoid(x)

def _layernorm(x, axis=-1, eps=1e-05):
    m = jnp.mean(x, axis=axis, keepdims=True)
    v = jnp.var(x, axis=axis, keepdims=True)
    return (x - m) / jnp.sqrt(v + eps)

def _scatter_add(tgt, idx, src, axis=0):
    return tgt.at[idx].add(src)

def _segment_sum(src, seg, n):
    return jax.ops.segment_sum(src, seg, n)

class _Rng:

    def __init__(self, key):
        self._k = key

    def _next(self):
        self._k, sub = jax.random.split(self._k)
        return sub

    def normal(self, shape):
        return jax.random.normal(self._next(), shape, dtype=jnp.bfloat16)

    def randint(self, lo, hi, shape):
        return jax.random.randint(self._next(), shape, lo, hi, dtype=jnp.int32)

    def uniform(self, shape, lo=0.0, hi=1.0):
        return jax.random.uniform(self._next(), shape, jnp.bfloat16, lo, hi)

    def permutation(self, n):
        return jax.random.permutation(self._next(), n)
kernel_name = 'interleave_layers__memory_aug_infini_attn__moe_arch_mod__prompt'

def setup_inputs():
    _rng = _Rng(jax.random.key(int.from_bytes(__import__("os").urandom(4), "little")))
    _w = lambda a: (lambda t: t.astype(jnp.bfloat16) if jnp.issubdtype(t.dtype, jnp.floating) else t)(jnp.asarray(a))

    def _A_setup():
        B, S, D, H = (1, 2048, 1024, 32)
        N = 4
        L = max(1, S // N)
        sc = D ** (-0.5)
        return {'x': _w((lambda *s: _rng.normal(s) * 0.05)(B, N * L, D)), 'wq': _w((lambda *s: _rng.normal(s) * 0.05)(D, D) * sc), 'wk': _w((lambda *s: _rng.normal(s) * 0.05)(D, D) * sc), 'wv': _w((lambda *s: _rng.normal(s) * 0.05)(D, D) * sc), 'wo': _w((lambda *s: _rng.normal(s) * 0.05)(D, D) * sc), 'beta': _w((lambda *s: _rng.normal(s) * 0.05)(H))}
    _A_in = _A_setup()

    def _B_setup():
        B, S, D, F, C = (1, 2048, 1024, 3584, 2)
        return {'x': _w((lambda *s: _rng.normal(s) * 0.05)(B, S, D)), 'w_r': _w((lambda *s: _rng.normal(s) * 0.05)(D)), 'w_gate': _w((lambda *s: _rng.normal(s) * 0.05)(D, F)), 'w_up': _w((lambda *s: _rng.normal(s) * 0.05)(D, F)), 'w_down': _w((lambda *s: _rng.normal(s) * 0.05)(F, D))}
    _B_in = _B_setup()
    return {'A_x': _A_in['x'], 'A_wq': _A_in['wq'], 'A_wk': _A_in['wk'], 'A_wv': _A_in['wv'], 'A_wo': _A_in['wo'], 'A_beta': _A_in['beta'], 'B_x': _B_in['x'], 'B_w_r': _B_in['w_r'], 'B_w_gate': _B_in['w_gate'], 'B_w_up': _B_in['w_up'], 'B_w_down': _B_in['w_down']}

def reference(A_x, A_wq, A_wk, A_wv, A_wo, A_beta, B_x, B_w_r, B_w_gate, B_w_up, B_w_down):

    def _A_ref(x, wq, wk, wv, wo, beta):
        B, S, D = x.shape
        H = 32
        Dh = D // H
        N = 4
        L = S // N
        q = (lambda x, *d: x.transpose(*d))((x @ wq).reshape(B, S, H, Dh), 0, 2, 1, 3).reshape(B, H, N, L, Dh)
        k = (lambda x, *d: x.transpose(*d))((x @ wk).reshape(B, S, H, Dh), 0, 2, 1, 3).reshape(B, H, N, L, Dh)
        v = (lambda x, *d: x.transpose(*d))((x @ wv).reshape(B, S, H, Dh), 0, 2, 1, 3).reshape(B, H, N, L, Dh)
        phi = lambda t: jnp.where(t > 0, t + 1.0, jnp.exp(t))
        scale = Dh ** (-0.5)
        ar = jnp.arange(L)
        mask = (lambda x, dt: x.astype(dt))(ar[:, None] < ar[None, :], x.dtype) * -1000000000.0
        g = _sigmoid(beta).reshape(1, H, 1, 1)
        M = jnp.einsum('bhd,bhe->bhde', q[:, :, 0, 0, :] * 0.0, q[:, :, 0, 0, :] * 0.0)
        z = q[:, :, 0, 0, :] * 0.0
        outs = []
        for s in range(N):
            qs, ks, vs = (q[:, :, s].copy(), k[:, :, s].copy(), v[:, :, s].copy())
            logits = jnp.einsum('bhqd,bhkd->bhqk', qs, ks) * scale + mask
            p = _softmax(logits, axis=-1)
            a_dot = jnp.einsum('bhqk,bhkd->bhqd', p, vs)
            pq = phi(qs)
            num = jnp.einsum('bhld,bhde->bhle', pq, M)
            den = jnp.einsum('bhld,bhd->bhl', pq, z)[..., None] + 1e-06
            a_mem = num / den
            o = g * a_mem + (1.0 - g) * a_dot
            outs.append(o)
            pk = phi(ks)
            M = M + jnp.einsum('bhld,bhle->bhde', pk, vs)
            z = z + jnp.einsum('bhld->bhd', pk)
        o = (lambda x, *d: x.transpose(*d))(jnp.stack(outs, 2).reshape(B, H, S, Dh), 0, 2, 1, 3).reshape(B, S, D)
        return o @ wo

    def _B_ref(x, w_r, w_gate, w_up, w_down):
        B, S, D = x.shape
        C = 2
        r = x @ w_r
        idx = jnp.argsort(-r, axis=-1)[:, :C]
        idx_e = jnp.repeat(idx.reshape(B, C, 1), D, axis=2)
        x_sel = jnp.take_along_axis(x, idx_e, axis=1)
        g = _silu(x_sel @ w_gate)
        u = x_sel @ w_up
        y = g * u @ w_down
        r_sel = _sigmoid(jnp.take_along_axis(r, idx, axis=1))
        y = y * r_sel.reshape(B, C, 1)
        b_off = (jnp.arange(B) * S).reshape(B, 1)
        flat_idx = (idx + b_off).reshape(B * C)
        zero = (x * 0.0).reshape(B * S, D)
        upd = _scatter_add(zero, flat_idx, y.reshape(B * C, D), axis=0)
        return x + upd.reshape(B, S, D)
    x = A_x
    x = x + _A_ref(_layernorm(x, axis=-1), A_wq, A_wk, A_wv, A_wo, A_beta)
    x = x + _B_ref(_layernorm(x, axis=-1), B_w_r, B_w_gate, B_w_up, B_w_down)
    x = x + _A_ref(_layernorm(x, axis=-1), A_wq, A_wk, A_wv, A_wo, A_beta)
    x = x + _B_ref(_layernorm(x, axis=-1), B_w_r, B_w_gate, B_w_up, B_w_down)
    return x
```

```python
import jax
import jax.numpy as jnp
from jax import lax
import jax.experimental.pallas as pl
import jax.experimental.pallas.tpu as pltpu

bf16 = jnp.bfloat16
f32 = jnp.float32
u32 = jnp.uint32
i32 = jnp.int32

S = 2048
D = 1024
L = 512
NSEG = 4
NG = 8
F = 3584
CH = 64
SUB = 16
NEG = -1e30
QSCALE = (32 ** -0.5) * 1.4426950408889634
NT = (((1,), (1,)), ((), ()))

SEM_X0 = 0
SEM_XR = 1
SEM_W = 9
SEM_WO = 33
SEM_SM = 34
SEM_FF = 36
SEM_OUT = 39
SEM_FIX = 50
NSEM = 52


def _rb(x):
    return x.astype(bf16).astype(f32)


def _pack(x):
    return pltpu.bitcast(x.astype(bf16), u32)


def _unpack(u):
    return pltpu.bitcast(u, bf16)


def _phi(t):
    return jnp.where(t > 0, t + 1.0, jnp.exp(t))


def _ln(x):
    m = jnp.sum(x, axis=-1, keepdims=True) * (1.0 / D)
    mb = _rb(m)
    e = x - mb
    dm = m - mb
    v = jnp.sum(e * e, axis=-1, keepdims=True) * (1.0 / D) - dm * dm
    v = jnp.maximum(v, 0.0)
    den = _rb(jnp.sqrt(_rb(_rb(v) + 1e-5)))
    return (_rb(e) * (1.0 / den)).astype(bf16)


def _merge(*streams):
    live = [[g, w, 0.0] for g, w in streams]
    while live:
        item = min(live, key=lambda t: t[2])
        try:
            next(item[0])
            item[2] += 1.0 / item[1]
        except StopIteration:
            live.remove(item)


def _kernel(x_hbm, wq_hbm, wk_hbm, wv_hbm, wo_hbm, beta_hbm, wr_hbm, wg_hbm, wu_hbm, wd_hbm,
            out_hbm,
            x_ref, xn_ref, x1_ref, w_ref, wo_ref, wg_ref, wu_ref, wd_ref,
            beta_ref, wr_ref, wrf_ref, gate_ref, m_ref, r_ref,
            q0, pq0, k0, pk0, vt0, q1, pq1, k1, pk1, vt1, oa_ref, ob_ref, sems):
    qkv = ((q0, pq0, k0, pk0, vt0), (q1, pq1, k1, pk1, vt1))
    o_refs = (oa_ref, ob_ref)

    def cp_x0():
        return pltpu.make_async_copy(x_hbm.at[0], x_ref.at[0], sems.at[SEM_X0])

    def cp_xr(g):
        r0 = pl.multiple_of(g * CH, CH)
        return pltpu.make_async_copy(x_hbm.at[1:NSEG, pl.ds(r0, CH), :],
                                     x_ref.at[1:NSEG, pl.ds(r0, CH), :], sems.at[SEM_XR + g])

    def cp_w(g, j):
        c0 = pl.multiple_of(g * 128, 128)
        src = (wq_hbm, wk_hbm, wv_hbm)[j]
        return pltpu.make_async_copy(src.at[:, pl.ds(c0, 128)],
                                     w_ref.at[g, :, 128 * j:128 * j + 128], sems.at[SEM_W + 3 * g + j])

    def cp_wo():
        return pltpu.make_async_copy(wo_hbm, wo_ref, sems.at[SEM_WO])

    def cp_small():
        return (pltpu.make_async_copy(beta_hbm, beta_ref, sems.at[SEM_SM]),
                pltpu.make_async_copy(wr_hbm, wr_ref, sems.at[SEM_SM + 1]))

    def cp_ff():
        return (pltpu.make_async_copy(wg_hbm, wg_ref, sems.at[SEM_FF]),
                pltpu.make_async_copy(wu_hbm, wu_ref, sems.at[SEM_FF + 1]),
                pltpu.make_async_copy(wd_hbm, wd_ref, sems.at[SEM_FF + 2]))

    def cp_out_seg(s):
        return pltpu.make_async_copy(x_ref.at[s], out_hbm.at[s], sems.at[SEM_OUT + s])

    def cp_out_chunk(c):
        r0 = pl.multiple_of(c * CH, CH)
        return pltpu.make_async_copy(x_ref.at[NSEG - 1, pl.ds(r0, CH), :],
                                     out_hbm.at[NSEG - 1, pl.ds(r0, CH), :], sems.at[SEM_OUT + 3 + c])

    def proj(seg, g, par):
        q_r, pq_r, k_r, pk_r, vt_r = qkv[par]
        for m in range(4):
            xn = _unpack(xn_ref[seg, 64 * m:64 * m + 64, :])
            y = jnp.dot(xn, w_ref[g], preferred_element_type=f32)
            q = y[:, 0:128]
            k = y[:, 128:256]
            v = y[:, 256:384]
            q_r[64 * m:64 * m + 64, :] = _pack(q * QSCALE)
            pq_r[64 * m:64 * m + 64, :] = _pack(_phi(q))
            k_r[64 * m:64 * m + 64, :] = _pack(k)
            pk_r[64 * m:64 * m + 64, :] = _pack(_phi(k))
            vt_r[0:64, 128 * m:128 * m + 128] = _pack(v.T)
            yield

    def attn(g, par, o_r, use_mem, do_update, lag=5, order=(3, 2, 1, 0)):
        q_r, pq_r, k_r, pk_r, vt_r = qkv[par]
        row = lax.broadcasted_iota(i32, (128, 512), 0)
        col = lax.broadcasted_iota(i32, (128, 512), 1)
        tri4 = row <= (col & 127)
        lane = lax.broadcasted_iota(i32, (64, 128), 1)
        hmask = [jnp.where((lane >> 5) == j, jnp.uint32(0xFFFFFFFF), jnp.uint32(0)) for j in range(4)]
        blocks = [(i, kb) for i in order for kb in range(i + 1)]
        nb = len(blocks)
        sv, pm, mx, wq, acc, ls = {}, {}, {}, {}, {}, {}
        nd = None
        if use_mem:
            ml = m_ref[g].astype(bf16)
            nd = lax.dot_general(ml, _unpack(pq_r[...]), NT, preferred_element_type=f32)
        if do_update:
            upd = jnp.dot(_unpack(vt_r[...]), _unpack(pk_r[...]), preferred_element_type=f32)
            r2 = lax.broadcasted_iota(i32, (144, 128), 0)
            c2 = lax.broadcasted_iota(i32, (144, 128), 1) >> 5
            keep = jnp.where(r2 < 128, r2 >> 5, r2 - 128) == c2
            upd = jnp.where(keep, upd, 0.0)
            m_ref[g] = (m_ref[g] + upd) if use_mem else upd
        yield
        for pos in range(nb + lag):
            if pos < nb:
                i, kb = blocks[pos]
                if kb == 0:
                    qu = q_r[64 * i:64 * i + 64, :]
                    wq[i] = _unpack(jnp.concatenate([qu & hmask[j] for j in range(4)], axis=0))
                s = lax.dot_general(_unpack(k_r[64 * kb:64 * kb + 64, :]), wq[i], NT,
                                    preferred_element_type=f32)
                if kb == i:
                    s = jnp.where(tri4, s, NEG)
                bm = jnp.max(s.reshape(16, 8, 512), axis=0)
                pm[i] = bm if kb == 0 else jnp.maximum(pm[i], bm)
                sv[pos] = s
                if kb == i:
                    mx[i] = jnp.max(pm[i], axis=0, keepdims=True)
            qp = pos - lag
            if qp >= 0:
                i, kb = blocks[qp]
                p = jnp.exp2(sv.pop(qp) - mx[i])
                ps = jnp.sum(p.reshape(16, 8, 512), axis=0)
                ls[i] = ps if kb == 0 else ls[i] + ps
                for j in range(4):
                    o = jnp.dot(_unpack(vt_r[16 * j:16 * j + 16, 128 * kb:128 * kb + 128]),
                                p[:, 128 * j:128 * j + 128].astype(bf16), preferred_element_type=f32)
                    acc[i, j] = o if kb == 0 else acc[i, j] + o
                if kb == i:
                    lsum = jnp.sum(ls[i], axis=0, keepdims=True)
                    parts = []
                    for j in range(4):
                        gt = gate_ref[pl.ds(4 * g + j, 1), :]
                        omg = gate_ref[pl.ds(32 + 4 * g + j, 1), :]
                        ot = acc[i, j] * (omg / lsum[:, 128 * j:128 * j + 128])
                        if use_mem:
                            den = nd[128 + j:129 + j, 128 * i:128 * i + 128] + 1e-6
                            ot = ot + nd[32 * j:32 * j + 32, 128 * i:128 * i + 128] * (gt / den)
                        parts.append(ot)
                    ot = jnp.concatenate(parts, axis=0)
                    o_r[g, 64 * i:64 * i + 64, :] = _pack(ot.T)
            yield

    def ln_first(c):
        for seg in range(1, NSEG):
            for t in range(CH // SUB):
                r0 = pl.multiple_of(c * CH + t * SUB, SUB)
                h0 = pl.multiple_of(c * (CH // 2) + t * (SUB // 2), SUB // 2)
                xv = x_ref[seg, pl.ds(r0, SUB), :].astype(f32)
                xn_ref[seg, pl.ds(h0, SUB // 2), :] = pltpu.bitcast(_ln(xv), u32)
                yield

    def resid(seg, c, o_r, next_ln):
        h0 = pl.multiple_of(c * (CH // 2), CH // 2)
        out = None
        for g in range(NG):
            part = jnp.dot(_unpack(o_r[g, pl.ds(h0, CH // 2), :]), wo_ref[128 * g:128 * g + 128, :],
                           preferred_element_type=f32)
            out = part if out is None else out + part
            if g % 2 == 1:
                yield
        lane = lax.broadcasted_iota(i32, (SUB, 128), 1)
        for t in range(CH // SUB):
            r0 = pl.multiple_of(c * CH + t * SUB, SUB)
            x1 = _rb(x_ref[seg, pl.ds(r0, SUB), :].astype(f32) + _rb(out[SUB * t:SUB * t + SUB]))
            x1_ref[seg, pl.ds(r0, SUB), :] = x1
            xn2 = _ln(x1).astype(f32)
            r = _rb(jnp.sum(xn2 * wrf_ref[...], axis=-1, keepdims=True))
            r_ref[SUB * t:SUB * t + SUB, :] = jnp.where(lane == seg * NG + c, r, r_ref[SUB * t:SUB * t + SUB, :])
            x2 = (x1 + xn2).astype(bf16)
            x_ref[seg, pl.ds(r0, SUB), :] = x2
            if next_ln:
                hh = pl.multiple_of(c * (CH // 2) + t * (SUB // 2), SUB // 2)
                xn_ref[seg, pl.ds(hh, SUB // 2), :] = pltpu.bitcast(_ln(x2.astype(f32)), u32)
            yield

    cp_x0().start()
    for j in range(3):
        cp_w(0, j).start()
    for cp in cp_small():
        cp.start()
    for j in range(3):
        cp_w(1, j).start()
    cp_xr(0).start()

    ones = jnp.full((8, 512), 0x3F803F80, u32)
    vt0[64:72, :] = ones
    vt1[64:72, :] = ones

    cp_x0().wait()
    for g in range(2, NG):
        for j in range(3):
            cp_w(g, j).start()
        cp_xr(g - 1).start()
    cp_xr(NG - 1).start()
    cp_wo().start()

    def ln0_body(t, carry):
        r0 = pl.multiple_of(t * SUB, SUB)
        h0 = pl.multiple_of(t * (SUB // 2), SUB // 2)
        xn_ref[0, pl.ds(h0, SUB // 2), :] = pltpu.bitcast(_ln(x_ref[0, pl.ds(r0, SUB), :].astype(f32)), u32)
        return carry
    lax.fori_loop(0, L // SUB, ln0_body, 0, unroll=4)

    for cp in cp_small():
        cp.wait()
    wrf_ref[...] = wr_ref[...].astype(f32)
    gl = _rb(jax.nn.sigmoid(beta_ref[...].astype(f32)))
    hr = lax.broadcasted_iota(i32, (32, 32), 0)
    hc = lax.broadcasted_iota(i32, (32, 32), 1)
    gcol = jnp.sum(jnp.where(hr == hc, gl, 0.0), axis=1, keepdims=True)
    gate_ref[0:32, :] = jnp.broadcast_to(gcol, (32, 128))
    gate_ref[32:64, :] = jnp.broadcast_to(_rb(1.0 - gcol), (32, 128))
    for j in range(3):
        cp_w(0, j).wait()

    def layer(li, carry):
        first = li == 0
        r_ref[...] = jnp.full((CH, 128), -jnp.inf, f32)
        _merge((proj(0, 0, 0), 1))

        for s in range(NSEG):
            def pair(p, c2, s=s, last=False):
                for par in range(2):
                    g = 2 * p + par
                    if s == 0:
                        @pl.when(first)
                        def _():
                            cp_xr(g).wait()

                            @pl.when(g + 1 < NG)
                            def _():
                                gn = jnp.minimum(g + 1, NG - 1)
                                for j in range(3):
                                    cp_w(gn, j).wait()
                    streams = []
                    if not (last and par == 1):
                        gn = g + 1
                        streams.append((proj(s + gn // NG, gn % NG, 1 - par), 4))
                    streams.append((attn(g, par, o_refs[s % 2], s > 0, s < NSEG - 1), 16))
                    if s == 0:
                        streams.append((ln_first(g), 12))
                    else:
                        streams.append((resid(s - 1, g, o_refs[(s - 1) % 2], s == 1), 8))
                    _merge(*streams)
                return c2

            if s == 1:
                @pl.when(first)
                def _():
                    cp_wo().wait()
                    for cp in cp_ff():
                        cp.start()
            if s >= 2:
                @pl.when(li == 1)
                def _():
                    cp_out_seg(s - 2).start()
            if s < NSEG - 1:
                lax.fori_loop(0, NG // 2, pair, 0)
            else:
                lax.fori_loop(0, NG // 2 - 1, pair, 0)
                pair(NG // 2 - 1, 0, last=True)

        @pl.when(li == 1)
        def _():
            cp_out_seg(NSEG - 2).start()

        def tail(c, c2):
            _merge((resid(NSEG - 1, c, o_refs[(NSEG - 1) % 2], False), 1))

            @pl.when(li == 1)
            def _():
                cp_out_chunk(c).start()
            return c2
        lax.fori_loop(0, NG, tail, 0)

        rm = r_ref[...]
        idx = (lax.broadcasted_iota(i32, (CH, 128), 1) * CH + lax.broadcasted_iota(i32, (CH, 128), 0)).astype(f32)
        big = float(S)
        m1 = jnp.max(rm, axis=(0, 1), keepdims=True)
        i1 = jnp.min(jnp.where(rm == m1, idx, big), axis=(0, 1), keepdims=True)
        rm2 = jnp.where(idx == i1, -jnp.inf, rm)
        m2 = jnp.max(rm2, axis=(0, 1), keepdims=True)
        i2 = jnp.min(jnp.where(jnp.logical_and(rm2 == m2, idx != i1), idx, big), axis=(0, 1), keepdims=True)
        toks = [jnp.clip(jnp.max(iv).astype(i32), 0, S - 1) for iv in (i1, i2)]

        @pl.when(first)
        def _():
            for cp in cp_ff():
                cp.wait()

        row = lax.broadcasted_iota(i32, (SUB, D), 0)
        x1s = jnp.where(row == 0, x1_ref[toks[0] // L, pl.ds(toks[0] % L, 1), :],
                        jnp.where(row == 1, x1_ref[toks[1] // L, pl.ds(toks[1] % L, 1), :], 0.0))
        xs = _ln(x1s)
        ga = _rb(jnp.dot(xs, wg_ref[...], preferred_element_type=f32))
        up = _rb(jnp.dot(xs, wu_ref[...], preferred_element_type=f32))
        hdn = (_rb(ga * _rb(jax.nn.sigmoid(ga))) * up).astype(bf16)
        y = _rb(jnp.dot(hdn, wd_ref[...], preferred_element_type=f32))
        rsel = jnp.where(lax.broadcasted_iota(i32, (SUB, 1), 0) == 0, m1, m2)
        y = _rb(y * _rb(jax.nn.sigmoid(rsel)))
        x2s = _rb(x1s + _rb(xs.astype(f32) + y))
        xns = _ln(x2s).astype(f32)

        @pl.when(li == 1)
        def _():
            for s in range(NSEG - 1):
                cp_out_seg(s).wait()
            for c in range(NG):
                cp_out_chunk(c).wait()

        blks = []
        for n, t in enumerate(toks):
            sg = t // L
            b0 = pl.multiple_of((t % L) // SUB * SUB, SUB)
            hb = pl.multiple_of((t % L) // SUB * (SUB // 2), SUB // 2)
            hit = row == (t % SUB)
            old = x_ref[sg, pl.ds(b0, SUB), :].astype(f32)
            x_ref[sg, pl.ds(b0, SUB), :] = jnp.where(hit, x2s[n:n + 1], old).astype(bf16)
            oldn = _unpack(xn_ref[sg, pl.ds(hb, SUB // 2), :]).astype(f32)
            xn_ref[sg, pl.ds(hb, SUB // 2), :] = _pack(jnp.where(hit, xns[n:n + 1], oldn))
            blks.append((sg, b0))

        @pl.when(li == 1)
        def _():
            def cp_fix(n):
                sg, b0 = blks[n]
                return pltpu.make_async_copy(x_ref.at[sg, pl.ds(b0, SUB), :],
                                             out_hbm.at[sg, pl.ds(b0, SUB), :], sems.at[SEM_FIX + n])
            differ = (toks[0] // SUB) != (toks[1] // SUB)
            cp_fix(0).start()

            @pl.when(differ)
            def _():
                cp_fix(1).start()
                cp_fix(1).wait()
            cp_fix(0).wait()
        return carry

    lax.fori_loop(0, 2, layer, 0)


@jax.jit
def pallas_interleave_layers__memory_aug_infini_attn__moe_arch_mod__prompt_kernel(
    A_x: jax.Array,
    A_wq: jax.Array,
    A_wk: jax.Array,
    A_wv: jax.Array,
    A_wo: jax.Array,
    A_beta: jax.Array,
    B_x: jax.Array,
    B_w_r: jax.Array,
    B_w_gate: jax.Array,
    B_w_up: jax.Array,
    B_w_down: jax.Array,
):
    del B_x
    qkv_bufs = [pltpu.VMEM((L // 2, 128), u32)] * 4 + [pltpu.VMEM((72, L), u32)]
    scratch = [
        pltpu.VMEM((NSEG, L, D), bf16),
        pltpu.VMEM((NSEG, L // 2, D), u32),
        pltpu.VMEM((NSEG, L, D), f32),
        pltpu.VMEM((NG, D, 384), bf16),
        pltpu.VMEM((D, D), bf16),
        pltpu.VMEM((D, F), bf16),
        pltpu.VMEM((D, F), bf16),
        pltpu.VMEM((F, D), bf16),
        pltpu.VMEM((1, 32), bf16),
        pltpu.VMEM((1, D), bf16),
        pltpu.VMEM((1, D), f32),
        pltpu.VMEM((64, 128), f32),
        pltpu.VMEM((NG, 144, 128), f32),
        pltpu.VMEM((CH, 128), f32),
        *qkv_bufs, *qkv_bufs,
        pltpu.VMEM((NG, L // 2, 128), u32),
        pltpu.VMEM((NG, L // 2, 128), u32),
        pltpu.SemaphoreType.DMA((NSEM,)),
    ]
    out = pl.pallas_call(
        _kernel,
        out_shape=jax.ShapeDtypeStruct((NSEG, L, D), bf16),
        in_specs=[pl.BlockSpec(memory_space=pl.ANY)] * 10,
        out_specs=pl.BlockSpec(memory_space=pl.ANY),
        scratch_shapes=scratch,
        compiler_params=pltpu.CompilerParams(vmem_limit_bytes=100 * 2 ** 20),
    )(A_x.reshape(NSEG, L, D), A_wq, A_wk, A_wv, A_wo, A_beta.reshape(1, 32), B_w_r.reshape(1, D),
      B_w_gate, B_w_up, B_w_down)
    return out.reshape(1, S, D)
```

```python
import jax
import jax.numpy as jnp
from jax import lax
import jax.experimental.pallas as pl
import jax.experimental.pallas.tpu as pltpu

bf16 = jnp.bfloat16
f32 = jnp.float32
u32 = jnp.uint32
i32 = jnp.int32

S = 2048
D = 1024
L = 512
NSEG = 4
NG = 8
F = 3584
CH = 64
SUB = 16
NEG = -1e30
QSCALE = (32 ** -0.5) * 1.4426950408889634
NT = (((1,), (1,)), ((), ()))

SEM_X0 = 0
SEM_XR = 1
SEM_W = 9
SEM_WO = 33
SEM_SM = 34
SEM_FF = 36
SEM_OUT = 39
SEM_FIX = 43
NSEM = 45
NF = F // 128

CFG = dict(rep={}, maxreg=False, lnmode=0)


def _loop(name, n, body):
    rep = CFG['rep'].get(name, 1)
    if rep == 1:
        return lax.fori_loop(0, n, body, 0)
    return lax.fori_loop(0, n * rep, lambda i, c: body(i // rep, c), 0)


def _rb(x):
    return x.astype(bf16).astype(f32)


def _pack(x):
    return pltpu.bitcast(x.astype(bf16), u32)


def _unpack(u):
    return pltpu.bitcast(u, bf16)


def _phi(t):
    return jnp.where(t > 0, t + 1.0, jnp.exp(t))


def _dot(a, b):
    return jnp.dot(a, b, preferred_element_type=f32)


def _ln(x, mode=0):
    m = jnp.sum(x, axis=-1, keepdims=True) * (1.0 / D)
    if mode == 0:
        e = x - m
        v = jnp.sum(e * e, axis=-1, keepdims=True) * (1.0 / D)
        return e * lax.rsqrt(v + 1e-5)
    c = _rb(m)
    e = x - c
    v = jnp.sum(e * e, axis=-1, keepdims=True) * (1.0 / D) - (m - c) * (m - c)
    w = _rb(_rb(jnp.maximum(v, 0.0)) + 1e-5)
    den = _rb(w * lax.rsqrt(w))
    if mode == 2:
        return _rb(_rb(e) / den)
    return e * (1.0 / den)


def _kernel(x_hbm, wq_hbm, wk_hbm, wv_hbm, wo_hbm, beta_hbm, wr_hbm, wg_hbm, wu_hbm, wd_hbm,
            out_hbm,
            x_ref, xn_ref, x1_ref, w_ref, wo_ref, wg_ref, wu_ref, wd_ref,
            beta_ref, wr_ref, wrf_ref, gate_ref, bias_ref, m_ref, r_ref, nd_ref,
            s0_ref, s1_ref, s2_ref, s3_ref,
            q0, pq0, k0, pk0, vt0, q1, pq1, k1, pk1, vt1, oa_ref, ob_ref, sems):
    qkv = ((q0, pq0, k0, pk0, vt0), (q1, pq1, k1, pk1, vt1))
    o_refs = (oa_ref, ob_ref)
    s_refs = (s0_ref, s1_ref, s2_ref, s3_ref)

    def cp_x0():
        return pltpu.make_async_copy(x_hbm.at[0], x_ref.at[0], sems.at[SEM_X0])

    def cp_xr(g):
        r0 = pl.multiple_of(g * CH, CH)
        return pltpu.make_async_copy(x_hbm.at[1:NSEG, pl.ds(r0, CH), :],
                                     x_ref.at[1:NSEG, pl.ds(r0, CH), :], sems.at[SEM_XR + g])

    def cp_w(g, j):
        c0 = pl.multiple_of(g * 128, 128)
        src = (wq_hbm, wk_hbm, wv_hbm)[j]
        return pltpu.make_async_copy(src.at[:, pl.ds(c0, 128)], w_ref.at[3 * g + j], sems.at[SEM_W + 3 * g + j])

    def slabs(src, dst, n, sem):
        return [pltpu.make_async_copy(src.at[:, 128 * c:128 * c + 128], dst.at[c], sems.at[sem]) for c in range(n)]

    def cp_wo():
        return slabs(wo_hbm, wo_ref, NG, SEM_WO)

    def cp_small():
        return (pltpu.make_async_copy(beta_hbm, beta_ref, sems.at[SEM_SM]),
                pltpu.make_async_copy(wr_hbm, wr_ref, sems.at[SEM_SM + 1]))

    def cp_ff():
        return (slabs(wg_hbm, wg_ref, NF, SEM_FF) + slabs(wu_hbm, wu_ref, NF, SEM_FF + 1)
                + slabs(wd_hbm, wd_ref, NG, SEM_FF + 2))

    def cp_out_seg(s):
        return pltpu.make_async_copy(x_ref.at[s], out_hbm.at[s], sems.at[SEM_OUT + s])

    def proj_items(seg, g, par):
        q_r, pq_r, k_r, pk_r, vt_r = qkv[par]
        part = {}

        def item(m, n, h):
            xn = _unpack(xn_ref[seg, 64 * m:64 * m + 64, 512 * h:512 * h + 512])
            y = _dot(xn, w_ref[3 * g + n, 512 * h:512 * h + 512, :])
            if h == 0:
                part[m, n] = y
                return
            y = y + part.pop((m, n))
            if n == 0:
                q_r[64 * m:64 * m + 64, :] = _pack(y * QSCALE)
                pq_r[64 * m:64 * m + 64, :] = _pack(_phi(y))
            elif n == 1:
                k_r[64 * m:64 * m + 64, :] = _pack(y)
                pk_r[64 * m:64 * m + 64, :] = _pack(_phi(y))
            else:
                vt_r[0:64, 128 * m:128 * m + 128] = _pack(y.T)
        return item

    def attn_items(g, par, o_r, use_mem):
        q_r, pq_r, k_r, pk_r, vt_r = qkv[par]
        mx, parts = {}, {}

        def nd():
            ml = m_ref[g].astype(bf16)
            nd_ref[...] = lax.dot_general(ml, _unpack(pq_r[...]), NT, preferred_element_type=f32)

        def upd():
            u = _dot(_unpack(vt_r[...]), _unpack(pk_r[...]))
            r2 = lax.broadcasted_iota(i32, (144, 128), 0)
            c2 = lax.broadcasted_iota(i32, (144, 128), 1) >> 5
            keep = jnp.where(r2 < 128, r2 >> 5, r2 - 128) == c2
            u = jnp.where(keep, u, 0.0)
            m_ref[g] = (m_ref[g] + u) if use_mem else u

        def qk(i):
            lane = lax.broadcasted_iota(i32, (64, 128), 1)
            qu = q_r[64 * i:64 * i + 64, :]
            wq = _unpack(jnp.concatenate(
                [jnp.where((lane >> 5) == j, qu, jnp.uint32(0)) for j in range(4)], axis=0))
            n = 128 * (i + 1)
            s = lax.dot_general(_unpack(k_r[0:n // 2, :]), wq, NT,
                                preferred_element_type=f32)
            sd = s[n - 128:n] + jnp.concatenate([bias_ref[...]] * 4, axis=1)
            if i > 0:
                s_refs[i][0:n - 128, :] = s[0:n - 128]
            s_refs[i][n - 128:n, :] = sd
            if CFG['maxreg']:
                pm = jnp.max(sd.reshape(16, 8, 512), axis=0)
                if i > 0:
                    pm = jnp.maximum(pm, jnp.max(s[0:n - 128].reshape(16 * i, 8, 512), axis=0))
                mx[i] = jnp.max(pm, axis=0, keepdims=True)

        def ex(i, j):
            n = 128 * (i + 1)
            if CFG['maxreg']:
                m = mx[i][:, 128 * j:128 * j + 128]
            else:
                m = jnp.max(jnp.max(s_refs[i][:, 128 * j:128 * j + 128].reshape(n // 8, 8, 128), axis=0),
                            axis=0, keepdims=True)
            p = jnp.exp2(s_refs[i][:, 128 * j:128 * j + 128] - m)
            lsum = jnp.sum(jnp.sum(p.reshape(n // 8, 8, 128), axis=0), axis=0, keepdims=True)
            o = _dot(_unpack(vt_r[16 * j:16 * j + 16, 0:n]), p.astype(bf16))
            gt = gate_ref[pl.ds(4 * g + j, 1), :]
            omg = gate_ref[pl.ds(32 + 4 * g + j, 1), :]
            o = o * (omg / lsum)
            if use_mem:
                den = nd_ref[128 + j:129 + j, 128 * i:128 * i + 128] + 1e-6
                o = o + nd_ref[32 * j:32 * j + 32, 128 * i:128 * i + 128] * (gt / den)
            parts[i, j] = o
            if j == 3:
                ot = jnp.concatenate([parts.pop((i, jj)) for jj in range(4)], axis=0)
                o_r[g, 64 * i:64 * i + 64, :] = _pack(ot.T)
        return nd, upd, qk, ex

    def ln1(seg, r):
        r0 = pl.multiple_of(r * SUB, SUB)
        h0 = pl.multiple_of(r * (SUB // 2), SUB // 2)
        xn_ref[seg, pl.ds(h0, SUB // 2), :] = _pack(_ln(x_ref[seg, pl.ds(r0, SUB), :].astype(f32)))

    def oproj(seg, r0, rows, n, o_r, k0=0, k1=NG):
        h0 = pl.multiple_of(r0 // 2, rows // 2)
        r0 = pl.multiple_of(r0, rows)
        lhs = _unpack(jnp.concatenate([o_r[g, pl.ds(h0, rows // 2), :] for g in range(k0, k1)], axis=1))
        y = _dot(lhs, wo_ref[n, 128 * k0:128 * k1, :])
        cols = slice(128 * n, 128 * n + 128)
        if k0 > 0:
            y = y + x1_ref[seg, pl.ds(r0, rows), cols]
        if k1 == NG:
            y = _rb(x_ref[seg, pl.ds(r0, rows), cols].astype(f32) + y)
        x1_ref[seg, pl.ds(r0, rows), cols] = y

    def ln2(seg, c, t):
        r0 = pl.multiple_of(c * CH + t * SUB, SUB)
        lane = lax.broadcasted_iota(i32, (SUB, 128), 1)
        x1 = x1_ref[seg, pl.ds(r0, SUB), :]
        xn2 = _ln(x1, CFG['lnmode'])
        r = _rb(jnp.sum(xn2 * wrf_ref[...], axis=-1, keepdims=True))
        r_ref[SUB * t:SUB * t + SUB, :] = jnp.where(lane == seg * NG + c, r, r_ref[SUB * t:SUB * t + SUB, :])
        x_ref[seg, pl.ds(r0, SUB), :] = (x1 + xn2).astype(bf16)

    def group(s, g, par, last=False):
        nd, upd, qk, ex = attn_items(g, par, o_refs[s % 2], s > 0)
        fill = []
        extra = []
        if s > 0:
            for n in range(NG):
                fill.append((128, lambda n=n: oproj(s - 1, g * CH, CH, n, o_refs[(s - 1) % 2])))
            extra = [lambda t=t: ln2(s - 1, g, t) for t in range(CH // SUB)]
        else:
            extra = [lambda seg=seg, t=t: ln1(seg, g * (CH // SUB) + t)
                     for seg in range(1, NSEG) for t in range(CH // SUB)]
        n_o = len(fill)
        if not last:
            gn = g + 1
            pj = proj_items(s + gn // NG, gn % NG, 1 - par)
            for m, n in [(m, n) for m in range(4) for n in range(2)] + [(m, 2) for m in range(4)]:
                for h in range(2):
                    fill.append((128, lambda m=m, n=n, h=h: pj(m, n, h)))
        else:
            for m in range(4):
                for n in range(NG):
                    fill.append((128, lambda m=m, n=n: oproj(s, 128 * m, 128, n, o_refs[s % 2], 0, 4)))
        fill = iter(fill)
        nfill = [0]

        def f(k=1):
            for _ in range(k):
                next(fill)[1]()
                nfill[0] += 1
                if extra and nfill[0] > n_o + 1 and (nfill[0] % 2 == 0 or s == 0):
                    extra.pop(0)()

        if s > 0:
            f(2)
            nd()
        qk(3)
        f(2)
        qk(2)
        f(1)
        for j in range(4):
            ex(3, j)
            f(1)
        qk(1)
        for j in range(4):
            f(1)
            ex(2, j)
        qk(0)
        if s < NSEG - 1:
            upd()
        f(1)
        ex(1, 0)
        ex(1, 1)
        f(1)
        ex(1, 2)
        ex(1, 3)
        f(1)
        for j in range(4):
            ex(0, j)
        for it in fill:
            it[1]()
            nfill[0] += 1
            if extra and (nfill[0] % 2 == 0 or s == 0):
                extra.pop(0)()
        for e in extra:
            e()

    cp_x0().start()
    for j in range(3):
        cp_w(0, j).start()
    for cp in cp_small():
        cp.start()
    for j in range(3):
        cp_w(1, j).start()
    cp_xr(0).start()

    ones = jnp.full((8, 512), 0x3F803F80, u32)
    vt0[64:72, :] = ones
    vt1[64:72, :] = ones
    bias_ref[...] = jnp.where(lax.broadcasted_iota(i32, (128, 128), 0) <= lax.broadcasted_iota(i32, (128, 128), 1),
                              0.0, NEG)

    cp_x0().wait()
    for g in range(2, NG):
        for j in range(3):
            cp_w(g, j).start()
        cp_xr(g - 1).start()
    cp_xr(NG - 1).start()
    for cp in cp_wo():
        cp.start()

    def ln0_body(t, carry):
        ln1(0, t)
        return carry
    lax.fori_loop(0, L // SUB, ln0_body, 0, unroll=4)

    for cp in cp_small():
        cp.wait()
    wrf_ref[...] = wr_ref[...].astype(f32)
    gl = _rb(jax.nn.sigmoid(beta_ref[...].astype(f32)))
    hr = lax.broadcasted_iota(i32, (32, 32), 0)
    hc = lax.broadcasted_iota(i32, (32, 32), 1)
    gcol = jnp.sum(jnp.where(hr == hc, gl, 0.0), axis=1, keepdims=True)
    gate_ref[0:32, :] = jnp.broadcast_to(gcol, (32, 128))
    gate_ref[32:64, :] = jnp.broadcast_to(_rb(1.0 - gcol), (32, 128))
    for j in range(3):
        cp_w(0, j).wait()

    def layer(li, carry):
        first = li == 0
        r_ref[...] = jnp.full((CH, 128), -jnp.inf, f32)
        pj = proj_items(0, 0, 0)
        for m in range(4):
            for n in range(3):
                pj(m, n, 0)
                pj(m, n, 1)

        for s in range(NSEG):
            def pair(p, c2, s=s, last=False):
                if s == 0:
                    @pl.when(first)
                    def _():
                        for par in range(2):
                            g = 2 * p + par
                            cp_xr(g).wait()

                            @pl.when(g + 1 < NG)
                            def _():
                                gn = jnp.minimum(g + 1, NG - 1)
                                for j in range(3):
                                    cp_w(gn, j).wait()
                for par in range(2):
                    group(s, 2 * p + par, par, last and par == 1)
                return c2

            if s == 1:
                @pl.when(first)
                def _():
                    for cp in cp_wo():
                        cp.wait()
                    for cp in cp_ff():
                        cp.start()
            if s >= 2:
                @pl.when(li == 1)
                def _():
                    cp_out_seg(s - 2).start()
            if s < NSEG - 1:
                _loop('s%d' % s, NG // 2, pair)
            else:
                _loop('s%d' % s, NG // 2 - 1, pair)
                pair(NG // 2 - 1, 0, last=True)

        s = NSEG - 1
        pend = []
        for m in (3, 2, 1, 0):
            for n in range(NG):
                oproj(s, 128 * m, 128, n, o_refs[s % 2], 4, NG)
                if pend:
                    pend.pop(0)()
            pend = [lambda c=c, t=t: ln2(s, c, t) for c in (2 * m, 2 * m + 1) for t in range(CH // SUB)]
        for e in pend:
            e()

        @pl.when(li == 1)
        def _():
            cp_out_seg(NSEG - 2).start()
            cp_out_seg(NSEG - 1).start()

        rm = r_ref[...]
        idx = (lax.broadcasted_iota(i32, (CH, 128), 1) * CH + lax.broadcasted_iota(i32, (CH, 128), 0)).astype(f32)
        big = float(S)
        m1 = jnp.max(rm, axis=(0, 1), keepdims=True)
        i1 = jnp.min(jnp.where(rm == m1, idx, big), axis=(0, 1), keepdims=True)
        rm2 = jnp.where(idx == i1, -jnp.inf, rm)
        m2 = jnp.max(rm2, axis=(0, 1), keepdims=True)
        i2 = jnp.min(jnp.where(jnp.logical_and(rm2 == m2, idx != i1), idx, big), axis=(0, 1), keepdims=True)
        toks = [jnp.clip(jnp.max(iv).astype(i32), 0, S - 1) for iv in (i1, i2)]

        @pl.when(first)
        def _():
            for cp in cp_ff():
                cp.wait()

        row = lax.broadcasted_iota(i32, (SUB, D), 0)
        x1s = jnp.where(row == 0, x1_ref[toks[0] // L, pl.ds(toks[0] % L, 1), :],
                        jnp.where(row == 1, x1_ref[toks[1] // L, pl.ds(toks[1] % L, 1), :], 0.0))
        xs = _ln(x1s, 2 * CFG['lnmode']).astype(bf16)
        hs = []
        for c in range(NF):
            ga = _rb(_dot(xs, wg_ref[c]))
            up = _rb(_dot(xs, wu_ref[c]))
            hs.append((_rb(ga * _rb(jax.nn.sigmoid(ga))) * up).astype(bf16))
            ln1(0, c)
        hdn = jnp.concatenate(hs, axis=1)
        ys = []
        for c in range(NG):
            ys.append(_dot(hdn, wd_ref[c]))
            if NF + c < L // SUB:
                ln1(0, NF + c)
        y = _rb(jnp.concatenate(ys, axis=1))
        rsel = jnp.where(lax.broadcasted_iota(i32, (SUB, 1), 0) == 0, m1, m2)
        y = _rb(y * _rb(jax.nn.sigmoid(rsel)))
        x2s = _rb(x1s + _rb(xs.astype(f32) + y))
        xns = _ln(x2s)

        @pl.when(li == 1)
        def _():
            for s in range(NSEG):
                cp_out_seg(s).wait()

        blks = []
        for n, t in enumerate(toks):
            sg = t // L
            b0 = pl.multiple_of((t % L) // SUB * SUB, SUB)
            hb = pl.multiple_of((t % L) // SUB * (SUB // 2), SUB // 2)
            hit = row == (t % SUB)
            old = x_ref[sg, pl.ds(b0, SUB), :].astype(f32)
            x_ref[sg, pl.ds(b0, SUB), :] = jnp.where(hit, x2s[n:n + 1], old).astype(bf16)
            oldn = _unpack(xn_ref[sg, pl.ds(hb, SUB // 2), :]).astype(f32)
            xn_ref[sg, pl.ds(hb, SUB // 2), :] = _pack(jnp.where(hit, xns[n:n + 1], oldn))
            blks.append((sg, b0))

        @pl.when(li == 1)
        def _():
            def cp_fix(n):
                sg, b0 = blks[n]
                return pltpu.make_async_copy(x_ref.at[sg, pl.ds(b0, SUB), :],
                                             out_hbm.at[sg, pl.ds(b0, SUB), :], sems.at[SEM_FIX + n])
            differ = (toks[0] // SUB) != (toks[1] // SUB)
            cp_fix(0).start()

            @pl.when(differ)
            def _():
                cp_fix(1).start()
                cp_fix(1).wait()
            cp_fix(0).wait()
        return carry

    lax.fori_loop(0, 2, layer, 0)


@jax.jit
def pallas_interleave_layers__memory_aug_infini_attn__moe_arch_mod__prompt_kernel(
    A_x: jax.Array,
    A_wq: jax.Array,
    A_wk: jax.Array,
    A_wv: jax.Array,
    A_wo: jax.Array,
    A_beta: jax.Array,
    B_x: jax.Array,
    B_w_r: jax.Array,
    B_w_gate: jax.Array,
    B_w_up: jax.Array,
    B_w_down: jax.Array,
):
    del B_x
    qkv_bufs = [pltpu.VMEM((L // 2, 128), u32)] * 4 + [pltpu.VMEM((72, L), u32)]
    scratch = [
        pltpu.VMEM((NSEG, L, D), bf16),
        pltpu.VMEM((NSEG, L // 2, D), u32),
        pltpu.VMEM((NSEG, L, D), f32),
        pltpu.VMEM((3 * NG, D, 128), bf16),
        pltpu.VMEM((NG, D, 128), bf16),
        pltpu.VMEM((NF, D, 128), bf16),
        pltpu.VMEM((NF, D, 128), bf16),
        pltpu.VMEM((NG, F, 128), bf16),
        pltpu.VMEM((1, 32), bf16),
        pltpu.VMEM((1, D), bf16),
        pltpu.VMEM((1, D), f32),
        pltpu.VMEM((64, 128), f32),
        pltpu.VMEM((128, 128), f32),
        pltpu.VMEM((NG, 144, 128), f32),
        pltpu.VMEM((CH, 128), f32),
        pltpu.VMEM((144, L), f32),
        pltpu.VMEM((128, L), f32), pltpu.VMEM((256, L), f32),
        pltpu.VMEM((384, L), f32), pltpu.VMEM((512, L), f32),
        *qkv_bufs, *qkv_bufs,
        pltpu.VMEM((NG, L // 2, 128), u32),
        pltpu.VMEM((NG, L // 2, 128), u32),
        pltpu.SemaphoreType.DMA((NSEM,)),
    ]
    out = pl.pallas_call(
        _kernel,
        out_shape=jax.ShapeDtypeStruct((NSEG, L, D), bf16),
        in_specs=[pl.BlockSpec(memory_space=pl.ANY)] * 10,
        out_specs=pl.BlockSpec(memory_space=pl.ANY),
        scratch_shapes=scratch,
        compiler_params=pltpu.CompilerParams(vmem_limit_bytes=100 * 2 ** 20),
    )(A_x.reshape(NSEG, L, D), A_wq, A_wk, A_wv, A_wo, A_beta.reshape(1, 32), B_w_r.reshape(1, D),
      B_w_gate, B_w_up, B_w_down)
    return out.reshape(1, S, D)
```

```python
import jax
import jax.numpy as jnp
from jax import lax
import jax.experimental.pallas as pl
import jax.experimental.pallas.tpu as pltpu

bf16 = jnp.bfloat16
f32 = jnp.float32
u32 = jnp.uint32
i32 = jnp.int32

S = 2048
D = 1024
L = 512
NSEG = 4
NG = 8
F = 3584
CH = 64
SUB = 16
NEG = -1e30
QSCALE = (32 ** -0.5) * 1.4426950408889634
NT = (((1,), (1,)), ((), ()))

SEM_X0 = 0
SEM_XR = 1
SEM_W = 9
SEM_WO = 33
SEM_SM = 34
SEM_FF = 36
SEM_OUT = 39
SEM_FIX = 43
NSEM = 45
NF = F // 128

CFG = dict(rep={}, maxreg=False, lnmode=0, nl=2, prewait=False, gp=2)


def _loop(name, n, body):
    rep = CFG['rep'].get(name, 1)
    if rep == 1:
        return lax.fori_loop(0, n, body, 0)
    return lax.fori_loop(0, n * rep, lambda i, c: body(i // rep, c), 0)


def _rb(x):
    return x.astype(bf16).astype(f32)


def _pack(x):
    return pltpu.bitcast(x.astype(bf16), u32)


def _unpack(u):
    return pltpu.bitcast(u, bf16)


def _phi(t):
    return jnp.where(t > 0, t + 1.0, jnp.exp(t))


def _dot(a, b):
    return jnp.dot(a, b, preferred_element_type=f32)


def _ln(x, mode=0):
    m = jnp.sum(x, axis=-1, keepdims=True) * (1.0 / D)
    if mode == 0:
        e = x - m
        v = jnp.sum(e * e, axis=-1, keepdims=True) * (1.0 / D)
        return e * lax.rsqrt(v + 1e-5)
    c = _rb(m)
    e = x - c
    v = jnp.sum(e * e, axis=-1, keepdims=True) * (1.0 / D) - (m - c) * (m - c)
    w = _rb(_rb(jnp.maximum(v, 0.0)) + 1e-5)
    den = _rb(w * lax.rsqrt(w))
    if mode == 2:
        return _rb(_rb(e) / den)
    return e * (1.0 / den)


def _kernel(x_hbm, wq_hbm, wk_hbm, wv_hbm, wo_hbm, beta_hbm, wr_hbm, wg_hbm, wu_hbm, wd_hbm,
            out_hbm,
            x_ref, xn_ref, x1_ref, w_ref, wo_ref, wg_ref, wu_ref, wd_ref,
            beta_ref, wr_ref, wrf_ref, gate_ref, bias_ref, m_ref, r_ref, nd_ref,
            s0_ref, s1_ref, s2_ref, s3_ref,
            q0, pq0, k0, pk0, vt0, q1, pq1, k1, pk1, vt1, oa_ref, ob_ref, sems):
    qkv = ((q0, pq0, k0, pk0, vt0), (q1, pq1, k1, pk1, vt1))
    o_refs = (oa_ref, ob_ref)
    s_refs = (s0_ref, s1_ref, s2_ref, s3_ref)
    w_u, wo_u, wg_u, wu_u, wd_u = (r.bitcast(u32) for r in (w_ref, wo_ref, wg_ref, wu_ref, wd_ref))

    def cp_x0():
        return pltpu.make_async_copy(x_hbm.at[0], x_ref.at[0], sems.at[SEM_X0])

    def cp_xr(g):
        r0 = pl.multiple_of(g * CH, CH)
        return pltpu.make_async_copy(x_hbm.at[1:NSEG, pl.ds(r0, CH), :],
                                     x_ref.at[1:NSEG, pl.ds(r0, CH), :], sems.at[SEM_XR + g])

    def cp_w(g, j):
        c0 = pl.multiple_of(g * 128, 128)
        src = (wq_hbm, wk_hbm, wv_hbm)[j]
        return pltpu.make_async_copy(src.at[:, pl.ds(c0, 128)], w_ref.at[3 * g + j], sems.at[SEM_W + 3 * g + j])

    def slabs(src, dst, n, sem):
        return [pltpu.make_async_copy(src.at[:, 128 * c:128 * c + 128], dst.at[c], sems.at[sem]) for c in range(n)]

    def cp_wo():
        return slabs(wo_hbm, wo_ref, NG, SEM_WO)

    def cp_small():
        return (pltpu.make_async_copy(beta_hbm, beta_ref, sems.at[SEM_SM]),
                pltpu.make_async_copy(wr_hbm, wr_ref, sems.at[SEM_SM + 1]))

    def cp_ff():
        return (slabs(wg_hbm, wg_ref, NF, SEM_FF) + slabs(wu_hbm, wu_ref, NF, SEM_FF + 1)
                + slabs(wd_hbm, wd_ref, NG, SEM_FF + 2))

    def cp_out_seg(s):
        return pltpu.make_async_copy(x_ref.at[s], out_hbm.at[s], sems.at[SEM_OUT + s])

    def proj_items(seg, g, par):
        q_r, pq_r, k_r, pk_r, vt_r = qkv[par]
        part = {}

        def item(m, n, h):
            xn = _unpack(xn_ref[seg, 64 * m:64 * m + 64, 512 * h:512 * h + 512])
            y = _dot(xn, _unpack(w_u[3 * g + n, 256 * h:256 * h + 256, :]))
            if h == 0:
                part[m, n] = y
                return
            y = y + part.pop((m, n))
            if n == 0:
                q_r[64 * m:64 * m + 64, :] = _pack(y * QSCALE)
                pq_r[64 * m:64 * m + 64, :] = _pack(_phi(y))
            elif n == 1:
                k_r[64 * m:64 * m + 64, :] = _pack(y)
                pk_r[64 * m:64 * m + 64, :] = _pack(_phi(y))
            else:
                vt_r[0:64, 128 * m:128 * m + 128] = _pack(y.T)
        return item

    def attn_items(g, par, o_r, use_mem):
        q_r, pq_r, k_r, pk_r, vt_r = qkv[par]
        mx, parts = {}, {}

        def nd():
            ml = m_ref[g].astype(bf16)
            nd_ref[...] = lax.dot_general(ml, _unpack(pq_r[...]), NT, preferred_element_type=f32)

        def upd():
            u = _dot(_unpack(vt_r[...]), _unpack(pk_r[...]))
            r2 = lax.broadcasted_iota(i32, (144, 128), 0)
            c2 = lax.broadcasted_iota(i32, (144, 128), 1) >> 5
            keep = jnp.where(r2 < 128, r2 >> 5, r2 - 128) == c2
            u = jnp.where(keep, u, 0.0)
            m_ref[g] = (m_ref[g] + u) if use_mem else u

        def qk(i):
            lane = lax.broadcasted_iota(i32, (64, 128), 1)
            qu = q_r[64 * i:64 * i + 64, :]
            wq = _unpack(jnp.concatenate(
                [jnp.where((lane >> 5) == j, qu, jnp.uint32(0)) for j in range(4)], axis=0))
            n = 128 * (i + 1)
            s = lax.dot_general(_unpack(k_r[0:n // 2, :]), wq, NT,
                                preferred_element_type=f32)
            sd = s[n - 128:n] + jnp.concatenate([bias_ref[...]] * 4, axis=1)
            if i > 0:
                s_refs[i][0:n - 128, :] = s[0:n - 128]
            s_refs[i][n - 128:n, :] = sd
            if CFG['maxreg']:
                pm = jnp.max(sd.reshape(16, 8, 512), axis=0)
                if i > 0:
                    pm = jnp.maximum(pm, jnp.max(s[0:n - 128].reshape(16 * i, 8, 512), axis=0))
                mx[i] = jnp.max(pm, axis=0, keepdims=True)

        def ex(i, j):
            n = 128 * (i + 1)
            if CFG['maxreg']:
                m = mx[i][:, 128 * j:128 * j + 128]
            else:
                m = jnp.max(jnp.max(s_refs[i][:, 128 * j:128 * j + 128].reshape(n // 8, 8, 128), axis=0),
                            axis=0, keepdims=True)
            p = jnp.exp2(s_refs[i][:, 128 * j:128 * j + 128] - m)
            lsum = jnp.sum(jnp.sum(p.reshape(n // 8, 8, 128), axis=0), axis=0, keepdims=True)
            o = _dot(_unpack(vt_r[16 * j:16 * j + 16, 0:n]), p.astype(bf16))
            gt = gate_ref[pl.ds(4 * g + j, 1), :]
            omg = gate_ref[pl.ds(32 + 4 * g + j, 1), :]
            o = o * (omg / lsum)
            if use_mem:
                den = nd_ref[128 + j:129 + j, 128 * i:128 * i + 128] + 1e-6
                o = o + nd_ref[32 * j:32 * j + 32, 128 * i:128 * i + 128] * (gt / den)
            parts[i, j] = o
            if j == 3:
                ot = jnp.concatenate([parts.pop((i, jj)) for jj in range(4)], axis=0)
                o_r[g, 64 * i:64 * i + 64, :] = _pack(ot.T)
        return nd, upd, qk, ex

    def ln1(seg, r):
        r0 = pl.multiple_of(r * SUB, SUB)
        h0 = pl.multiple_of(r * (SUB // 2), SUB // 2)
        xn_ref[seg, pl.ds(h0, SUB // 2), :] = _pack(_ln(x_ref[seg, pl.ds(r0, SUB), :].astype(f32)))

    def oproj(seg, r0, rows, n, o_r, k0=0, k1=NG):
        h0 = pl.multiple_of(r0 // 2, rows // 2)
        r0 = pl.multiple_of(r0, rows)
        lhs = _unpack(jnp.concatenate([o_r[g, pl.ds(h0, rows // 2), :] for g in range(k0, k1)], axis=1))
        y = _dot(lhs, _unpack(wo_u[n, 64 * k0:64 * k1, :]))
        cols = slice(128 * n, 128 * n + 128)
        if k0 > 0:
            y = y + x1_ref[seg, pl.ds(r0, rows), cols]
        if k1 == NG:
            y = _rb(x_ref[seg, pl.ds(r0, rows), cols].astype(f32) + y)
        x1_ref[seg, pl.ds(r0, rows), cols] = y

    def ln2(seg, c, t):
        r0 = pl.multiple_of(c * CH + t * SUB, SUB)
        lane = lax.broadcasted_iota(i32, (SUB, 128), 1)
        x1 = x1_ref[seg, pl.ds(r0, SUB), :]
        xn2 = _ln(x1, CFG['lnmode'])
        r = _rb(jnp.sum(xn2 * wrf_ref[...], axis=-1, keepdims=True))
        r_ref[SUB * t:SUB * t + SUB, :] = jnp.where(lane == seg * NG + c, r, r_ref[SUB * t:SUB * t + SUB, :])
        x_ref[seg, pl.ds(r0, SUB), :] = (x1 + xn2).astype(bf16)

    def group(s, g, par, last=False):
        nd, upd, qk, ex = attn_items(g, par, o_refs[s % 2], s > 0)
        fill = []
        extra = []
        if s > 0:
            for n in range(NG):
                fill.append((128, lambda n=n: oproj(s - 1, g * CH, CH, n, o_refs[(s - 1) % 2])))
            extra = [lambda t=t: ln2(s - 1, g, t) for t in range(CH // SUB)]
        else:
            extra = [lambda seg=seg, t=t: ln1(seg, g * (CH // SUB) + t)
                     for seg in range(1, NSEG) for t in range(CH // SUB)]
        n_o = len(fill)
        if not last:
            gn = g + 1
            pj = proj_items(s + gn // NG, gn % NG, 1 - par)
            for m, n in [(m, n) for m in range(4) for n in range(2)] + [(m, 2) for m in range(4)]:
                for h in range(2):
                    fill.append((128, lambda m=m, n=n, h=h: pj(m, n, h)))
        else:
            for m in range(4):
                for n in range(NG):
                    fill.append((128, lambda m=m, n=n: oproj(s, 128 * m, 128, n, o_refs[s % 2], 0, 4)))
        fill = iter(fill)
        nfill = [0]

        def f(k=1):
            for _ in range(k):
                next(fill)[1]()
                nfill[0] += 1
                if extra and nfill[0] > n_o + 1 and (nfill[0] % 2 == 0 or s == 0):
                    extra.pop(0)()

        if s > 0:
            f(2)
            nd()
        qk(3)
        f(2)
        qk(2)
        f(1)
        for j in range(4):
            ex(3, j)
            f(1)
        qk(1)
        for j in range(4):
            f(1)
            ex(2, j)
        qk(0)
        if s < NSEG - 1:
            upd()
        f(1)
        ex(1, 0)
        ex(1, 1)
        f(1)
        ex(1, 2)
        ex(1, 3)
        f(1)
        for j in range(4):
            ex(0, j)
        for it in fill:
            it[1]()
            nfill[0] += 1
            if extra and (nfill[0] % 2 == 0 or s == 0):
                extra.pop(0)()
        for e in extra:
            e()

    cp_x0().start()
    for j in range(3):
        cp_w(0, j).start()
    for cp in cp_small():
        cp.start()
    for j in range(3):
        cp_w(1, j).start()
    cp_xr(0).start()

    ones = jnp.full((8, 512), 0x3F803F80, u32)
    vt0[64:72, :] = ones
    vt1[64:72, :] = ones
    bias_ref[...] = jnp.where(lax.broadcasted_iota(i32, (128, 128), 0) <= lax.broadcasted_iota(i32, (128, 128), 1),
                              0.0, NEG)

    cp_x0().wait()
    for g in range(2, NG):
        for j in range(3):
            cp_w(g, j).start()
        cp_xr(g - 1).start()
    cp_xr(NG - 1).start()
    for cp in cp_wo():
        cp.start()

    def ln0_body(t, carry):
        ln1(0, t)
        return carry
    lax.fori_loop(0, L // SUB, ln0_body, 0, unroll=4)

    for cp in cp_small():
        cp.wait()
    wrf_ref[...] = wr_ref[...].astype(f32)
    gl = _rb(jax.nn.sigmoid(beta_ref[...].astype(f32)))
    hr = lax.broadcasted_iota(i32, (32, 32), 0)
    hc = lax.broadcasted_iota(i32, (32, 32), 1)
    gcol = jnp.sum(jnp.where(hr == hc, gl, 0.0), axis=1, keepdims=True)
    gate_ref[0:32, :] = jnp.broadcast_to(gcol, (32, 128))
    gate_ref[32:64, :] = jnp.broadcast_to(_rb(1.0 - gcol), (32, 128))
    for j in range(3):
        cp_w(0, j).wait()
    if CFG['prewait']:
        for g in range(NG):
            cp_xr(g).wait()
            for j in range(3 * (g > 0)):
                cp_w(g, j).wait()

    def layer(li, carry):
        first = li == 0
        r_ref[...] = jnp.full((CH, 128), -jnp.inf, f32)
        pj = proj_items(0, 0, 0)
        for m in range(4):
            for n in range(3):
                pj(m, n, 0)
                pj(m, n, 1)

        for s in range(NSEG):
            def pair(p, c2, s=s, last=False):
                if s == 0 and not CFG['prewait']:
                    @pl.when(first)
                    def _():
                        for par in range(2):
                            g = 2 * p + par
                            cp_xr(g).wait()

                            @pl.when(g + 1 < NG)
                            def _():
                                gn = jnp.minimum(g + 1, NG - 1)
                                for j in range(3):
                                    cp_w(gn, j).wait()
                for par in range(2):
                    group(s, 2 * p + par, par, last and par == 1)
                return c2

            if s == 1:
                @pl.when(first)
                def _():
                    for cp in cp_wo():
                        cp.wait()
                    for cp in cp_ff():
                        cp.start()
            if s >= 2:
                @pl.when(li == CFG['nl'] - 1)
                def _():
                    cp_out_seg(s - 2).start()
            if s in (1, 2) and CFG['gp'] > 2:
                np_ = CFG['gp'] // 2

                def multi(p, c2, pair=pair):
                    for u in range(np_):
                        pair(np_ * p + u, c2)
                    return c2
                if np_ == NG // 2 and not CFG['rep']:
                    multi(0, 0)
                else:
                    _loop('s%d' % s, NG // 2 // np_, multi)
            elif s < NSEG - 1:
                _loop('s%d' % s, NG // 2, pair)
            else:
                _loop('s%d' % s, NG // 2 - 1, pair)
                pair(NG // 2 - 1, 0, last=True)

        s = NSEG - 1
        pend = []
        for m in (3, 2, 1, 0):
            for n in range(NG):
                oproj(s, 128 * m, 128, n, o_refs[s % 2], 4, NG)
                if pend:
                    pend.pop(0)()
            pend = [lambda c=c, t=t: ln2(s, c, t) for c in (2 * m, 2 * m + 1) for t in range(CH // SUB)]
        for e in pend:
            e()

        @pl.when(li == CFG['nl'] - 1)
        def _():
            cp_out_seg(NSEG - 2).start()
            cp_out_seg(NSEG - 1).start()

        rm = r_ref[...]
        idx = (lax.broadcasted_iota(i32, (CH, 128), 1) * CH + lax.broadcasted_iota(i32, (CH, 128), 0)).astype(f32)
        big = float(S)
        m1 = jnp.max(rm, axis=(0, 1), keepdims=True)
        i1 = jnp.min(jnp.where(rm == m1, idx, big), axis=(0, 1), keepdims=True)
        rm2 = jnp.where(idx == i1, -jnp.inf, rm)
        m2 = jnp.max(rm2, axis=(0, 1), keepdims=True)
        i2 = jnp.min(jnp.where(jnp.logical_and(rm2 == m2, idx != i1), idx, big), axis=(0, 1), keepdims=True)
        toks = [jnp.clip(jnp.max(iv).astype(i32), 0, S - 1) for iv in (i1, i2)]

        @pl.when(first)
        def _():
            for cp in cp_ff():
                cp.wait()

        row = lax.broadcasted_iota(i32, (SUB, D), 0)
        x1s = jnp.where(row == 0, x1_ref[toks[0] // L, pl.ds(toks[0] % L, 1), :],
                        jnp.where(row == 1, x1_ref[toks[1] // L, pl.ds(toks[1] % L, 1), :], 0.0))
        xs = _ln(x1s, 2 * CFG['lnmode']).astype(bf16)
        hs = []
        for c in range(NF):
            ga = _rb(_dot(xs, _unpack(wg_u[c])))
            up = _rb(_dot(xs, _unpack(wu_u[c])))
            hs.append((_rb(ga * _rb(jax.nn.sigmoid(ga))) * up).astype(bf16))
            ln1(0, c)
        hdn = jnp.concatenate(hs, axis=1)
        ys = []
        for c in range(NG):
            ys.append(_dot(hdn, _unpack(wd_u[c])))
            if NF + c < L // SUB:
                ln1(0, NF + c)
        y = _rb(jnp.concatenate(ys, axis=1))
        rsel = jnp.where(lax.broadcasted_iota(i32, (SUB, 1), 0) == 0, m1, m2)
        y = _rb(y * _rb(jax.nn.sigmoid(rsel)))
        x2s = _rb(x1s + _rb(xs.astype(f32) + y))
        xns = _ln(x2s)

        @pl.when(li == CFG['nl'] - 1)
        def _():
            for s in range(NSEG):
                cp_out_seg(s).wait()

        blks = []
        for n, t in enumerate(toks):
            sg = t // L
            b0 = pl.multiple_of((t % L) // SUB * SUB, SUB)
            hb = pl.multiple_of((t % L) // SUB * (SUB // 2), SUB // 2)
            hit = row == (t % SUB)
            old = x_ref[sg, pl.ds(b0, SUB), :].astype(f32)
            x_ref[sg, pl.ds(b0, SUB), :] = jnp.where(hit, x2s[n:n + 1], old).astype(bf16)
            oldn = _unpack(xn_ref[sg, pl.ds(hb, SUB // 2), :]).astype(f32)
            xn_ref[sg, pl.ds(hb, SUB // 2), :] = _pack(jnp.where(hit, xns[n:n + 1], oldn))
            blks.append((sg, b0))

        @pl.when(li == CFG['nl'] - 1)
        def _():
            def cp_fix(n):
                sg, b0 = blks[n]
                return pltpu.make_async_copy(x_ref.at[sg, pl.ds(b0, SUB), :],
                                             out_hbm.at[sg, pl.ds(b0, SUB), :], sems.at[SEM_FIX + n])
            differ = (toks[0] // SUB) != (toks[1] // SUB)
            cp_fix(0).start()

            @pl.when(differ)
            def _():
                cp_fix(1).start()
                cp_fix(1).wait()
            cp_fix(0).wait()
        return carry

    lax.fori_loop(0, CFG['nl'], layer, 0)


@jax.jit
def pallas_interleave_layers__memory_aug_infini_attn__moe_arch_mod__prompt_kernel(
    A_x: jax.Array,
    A_wq: jax.Array,
    A_wk: jax.Array,
    A_wv: jax.Array,
    A_wo: jax.Array,
    A_beta: jax.Array,
    B_x: jax.Array,
    B_w_r: jax.Array,
    B_w_gate: jax.Array,
    B_w_up: jax.Array,
    B_w_down: jax.Array,
):
    del B_x
    qkv_bufs = [pltpu.VMEM((L // 2, 128), u32)] * 4 + [pltpu.VMEM((72, L), u32)]
    scratch = [
        pltpu.VMEM((NSEG, L, D), bf16),
        pltpu.VMEM((NSEG, L // 2, D), u32),
        pltpu.VMEM((NSEG, L, D), f32),
        pltpu.VMEM((3 * NG, D, 128), bf16),
        pltpu.VMEM((NG, D, 128), bf16),
        pltpu.VMEM((NF, D, 128), bf16),
        pltpu.VMEM((NF, D, 128), bf16),
        pltpu.VMEM((NG, F, 128), bf16),
        pltpu.VMEM((1, 32), bf16),
        pltpu.VMEM((1, D), bf16),
        pltpu.VMEM((1, D), f32),
        pltpu.VMEM((64, 128), f32),
        pltpu.VMEM((128, 128), f32),
        pltpu.VMEM((NG, 144, 128), f32),
        pltpu.VMEM((CH, 128), f32),
        pltpu.VMEM((144, L), f32),
        pltpu.VMEM((128, L), f32), pltpu.VMEM((256, L), f32),
        pltpu.VMEM((384, L), f32), pltpu.VMEM((512, L), f32),
        *qkv_bufs, *qkv_bufs,
        pltpu.VMEM((NG, L // 2, 128), u32),
        pltpu.VMEM((NG, L // 2, 128), u32),
        pltpu.SemaphoreType.DMA((NSEM,)),
    ]
    out = pl.pallas_call(
        _kernel,
        out_shape=jax.ShapeDtypeStruct((NSEG, L, D), bf16),
        in_specs=[pl.BlockSpec(memory_space=pl.ANY)] * 10,
        out_specs=pl.BlockSpec(memory_space=pl.ANY),
        scratch_shapes=scratch,
        compiler_params=pltpu.CompilerParams(vmem_limit_bytes=100 * 2 ** 20),
    )(A_x.reshape(NSEG, L, D), A_wq, A_wk, A_wv, A_wo, A_beta.reshape(1, 32), B_w_r.reshape(1, D),
      B_w_gate, B_w_up, B_w_down)
    return out.reshape(1, S, D)
```

```python
import jax
import jax.numpy as jnp
from jax import lax
import jax.experimental.pallas as pl
import jax.experimental.pallas.tpu as pltpu

bf16 = jnp.bfloat16
f32 = jnp.float32
u32 = jnp.uint32
i32 = jnp.int32

S = 2048
D = 1024
L = 512
NSEG = 4
NG = 8
F = 3584
CH = 64
SUB = 16
NEG = -1e30
QSCALE = (32 ** -0.5) * 1.4426950408889634
NT = (((1,), (1,)), ((), ()))

SEM_X0 = 0
SEM_XR = 1
SEM_W = 9
SEM_WO = 33
SEM_SM = 34
SEM_FF = 36
SEM_OUT = 39
SEM_FIX = 43
NSEM = 45
NF = F // 128

CFG = dict(rep={}, maxreg=False, lnmode=0, nl=2, prewait=False, gp=2)


def _loop(name, n, body):
    rep = CFG['rep'].get(name, 1)
    if rep == 1:
        return lax.fori_loop(0, n, body, 0)
    return lax.fori_loop(0, n * rep, lambda i, c: body(i // rep, c), 0)


def _rb(x):
    return x.astype(bf16).astype(f32)


def _pack(x):
    return pltpu.bitcast(x.astype(bf16), u32)


def _unpack(u):
    return pltpu.bitcast(u, bf16)


def _phi(t):
    return jnp.where(t > 0, t + 1.0, jnp.exp(t))


def _dot(a, b):
    return jnp.dot(a, b, preferred_element_type=f32)


def _unskew(ps):
    shape, dt = next((p.shape, p.dtype) for p in ps if p is not None)
    c = lax.broadcasted_iota(i32, shape, 1) >> 5
    even = (c & 1) == 0
    lo = c < 2
    mid = jnp.logical_or(c == 1, c == 2)

    def sel(mask, a, b):
        if a is None and b is None:
            return None
        z = jnp.zeros(shape, dt)
        return jnp.where(mask, z if a is None else a, z if b is None else b)
    x0, x1 = sel(even, ps[0], ps[1]), sel(even, ps[1], ps[0])
    x2, x3 = sel(even, ps[2], ps[3]), sel(even, ps[3], ps[2])
    return [sel(lo, x0, x2), sel(mid, x1, x3), sel(lo, x2, x0), sel(mid, x3, x1)]


def _ln(x, mode=0):
    m = jnp.sum(x, axis=-1, keepdims=True) * (1.0 / D)
    if mode == 0:
        e = x - m
        v = jnp.sum(e * e, axis=-1, keepdims=True) * (1.0 / D)
        return e * lax.rsqrt(v + 1e-5)
    c = _rb(m)
    e = x - c
    v = jnp.sum(e * e, axis=-1, keepdims=True) * (1.0 / D) - (m - c) * (m - c)
    w = _rb(_rb(jnp.maximum(v, 0.0)) + 1e-5)
    den = _rb(w * lax.rsqrt(w))
    if mode == 2:
        return _rb(_rb(e) / den)
    return e * (1.0 / den)


def _kernel(x_hbm, wq_hbm, wk_hbm, wv_hbm, wo_hbm, beta_hbm, wr_hbm, wg_hbm, wu_hbm, wd_hbm,
            out_hbm,
            x_ref, xn_ref, x1_ref, w_ref, wo_ref, wg_ref, wu_ref, wd_ref,
            beta_ref, wr_ref, wrf_ref, gate_ref, bias_ref, m_ref, r_ref, nd_ref,
            s0_ref, s1_ref, s2_ref, s3_ref,
            q0, pq0, k0, pk0, vt0, q1, pq1, k1, pk1, vt1, oa_ref, ob_ref, sems):
    qkv = ((q0, pq0, k0, pk0, vt0), (q1, pq1, k1, pk1, vt1))
    o_refs = (oa_ref, ob_ref)
    s_refs = (s0_ref, s1_ref, s2_ref, s3_ref)
    w_u, wo_u, wg_u, wu_u, wd_u = (r.bitcast(u32) for r in (w_ref, wo_ref, wg_ref, wu_ref, wd_ref))

    def cp_x0():
        return pltpu.make_async_copy(x_hbm.at[0], x_ref.at[0], sems.at[SEM_X0])

    def cp_xr(g):
        r0 = pl.multiple_of(g * CH, CH)
        return pltpu.make_async_copy(x_hbm.at[1:NSEG, pl.ds(r0, CH), :],
                                     x_ref.at[1:NSEG, pl.ds(r0, CH), :], sems.at[SEM_XR + g])

    def cp_w(g, j):
        c0 = pl.multiple_of(g * 128, 128)
        src = (wq_hbm, wk_hbm, wv_hbm)[j]
        return pltpu.make_async_copy(src.at[:, pl.ds(c0, 128)], w_ref.at[3 * g + j], sems.at[SEM_W + 3 * g + j])

    def slabs(src, dst, n, sem):
        return [pltpu.make_async_copy(src.at[:, 128 * c:128 * c + 128], dst.at[c], sems.at[sem]) for c in range(n)]

    def cp_wo():
        return slabs(wo_hbm, wo_ref, NG, SEM_WO)

    def cp_small():
        return (pltpu.make_async_copy(beta_hbm, beta_ref, sems.at[SEM_SM]),
                pltpu.make_async_copy(wr_hbm, wr_ref, sems.at[SEM_SM + 1]))

    def cp_ff():
        return (slabs(wg_hbm, wg_ref, NF, SEM_FF) + slabs(wu_hbm, wu_ref, NF, SEM_FF + 1)
                + slabs(wd_hbm, wd_ref, NG, SEM_FF + 2))

    def cp_out_seg(s):
        return pltpu.make_async_copy(x_ref.at[s], out_hbm.at[s], sems.at[SEM_OUT + s])

    def proj_items(seg, g, par):
        q_r, pq_r, k_r, pk_r, vt_r = qkv[par]
        part = {}

        def item(m, n, h):
            xn = _unpack(xn_ref[seg, 64 * m:64 * m + 64, 512 * h:512 * h + 512])
            y = _dot(xn, _unpack(w_u[3 * g + n, 256 * h:256 * h + 256, :]))
            if h == 0:
                part[m, n] = y
                return
            y = y + part.pop((m, n))
            if n == 0:
                q_r[64 * m:64 * m + 64, :] = _pack(y * QSCALE)
                pq_r[64 * m:64 * m + 64, :] = _pack(_phi(y))
            elif n == 1:
                k_r[64 * m:64 * m + 64, :] = _pack(y)
                pk_r[64 * m:64 * m + 64, :] = _pack(_phi(y))
            else:
                vt_r[0:64, 128 * m:128 * m + 128] = _pack(y.T)
        return item

    def attn_items(g, par, o_r, use_mem):
        q_r, pq_r, k_r, pk_r, vt_r = qkv[par]
        st = {}

        def nd():
            ml = m_ref[g].astype(bf16)
            nd_ref[...] = lax.dot_general(ml, _unpack(pq_r[...]), NT, preferred_element_type=f32)

        def upd():
            u = _dot(_unpack(vt_r[...]), _unpack(pk_r[...]))
            r2 = lax.broadcasted_iota(i32, (144, 128), 0)
            c2 = lax.broadcasted_iota(i32, (144, 128), 1) >> 5
            keep = jnp.where(r2 < 128, r2 >> 5, r2 - 128) == c2
            u = jnp.where(keep, u, 0.0)
            m_ref[g] = (m_ref[g] + u) if use_mem else u

        def qk(i):
            lane = lax.broadcasted_iota(i32, (16, 128), 1) >> 5
            for be in (range(4) if i % 2 else range(3, -1, -1)):
                b = 4 * i + be
                n = 32 * (b + 1)
                qu = q_r[16 * b:16 * b + 16, :]
                wq = _unpack(jnp.concatenate(
                    [jnp.where(lane == (c - be) % 4, qu, jnp.uint32(0)) for c in range(4)], axis=0))
                s = lax.dot_general(_unpack(k_r[0:n // 2, :]), wq, NT, preferred_element_type=f32)
                cols = slice(128 * be, 128 * be + 128)
                if b > 0:
                    s_refs[i][0:n - 32, cols] = s[0:n - 32]
                s_refs[i][n - 32:n, cols] = s[n - 32:n] + bias_ref[...]

        def mx(i):
            for be in range(4):
                n = 32 * (4 * i + be + 1)
                sv = s_refs[i][0:n, 128 * be:128 * be + 128]
                st[i, 'm', be] = jnp.max(jnp.max(sv.reshape(n // 8, 8, 128), axis=0), axis=0, keepdims=True)

        def ex(i, t):
            ps = []
            for be in range(4):
                n = 128 if t < i else 32 * (be + 1)
                p = jnp.exp2(s_refs[i][128 * t:128 * t + n, 128 * be:128 * be + 128] - st[i, 'm', be])
                ls = jnp.sum(p.reshape(n // 8, 8, 128), axis=0)
                st[i, 'l', be] = ls if t == 0 else st[i, 'l', be] + ls
                ps.append(_pack(p))
            if t < i:
                ts = _unskew(ps)
            else:
                blk = [_unskew([ps[be][16 * u:16 * u + 16] if be >= u else None for be in range(4)])
                       for u in range(4)]
                ts = [jnp.concatenate([blk[u][j] for u in range(4)], axis=0) for j in range(4)]
            for j in range(4):
                o = _dot(_unpack(vt_r[16 * j:16 * j + 16, 128 * t:128 * t + 128]), _unpack(ts[j]))
                st[i, 'o', j] = o if t == 0 else st[i, 'o', j] + o
            if t < i:
                return
            ls = _unskew([jnp.sum(st.pop((i, 'l', be)), axis=0, keepdims=True) for be in range(4)])
            parts = []
            for j in range(4):
                gt = gate_ref[pl.ds(4 * g + j, 1), :]
                omg = gate_ref[pl.ds(32 + 4 * g + j, 1), :]
                o = st.pop((i, 'o', j)) * (omg / ls[j])
                if j > 0:
                    o = pltpu.roll(o, 128 - 32 * j, 1)
                if use_mem:
                    den = nd_ref[128 + j:129 + j, 128 * i:128 * i + 128] + 1e-6
                    o = o + nd_ref[32 * j:32 * j + 32, 128 * i:128 * i + 128] * (gt / den)
                parts.append(o)
            ot = jnp.concatenate(parts, axis=0)
            o_r[g, 64 * i:64 * i + 64, :] = _pack(ot.T)
        return nd, upd, qk, mx, ex

    def ln1(seg, r):
        r0 = pl.multiple_of(r * SUB, SUB)
        h0 = pl.multiple_of(r * (SUB // 2), SUB // 2)
        xn_ref[seg, pl.ds(h0, SUB // 2), :] = _pack(_ln(x_ref[seg, pl.ds(r0, SUB), :].astype(f32)))

    def oproj(seg, r0, rows, n, o_r, k0=0, k1=NG):
        h0 = pl.multiple_of(r0 // 2, rows // 2)
        r0 = pl.multiple_of(r0, rows)
        lhs = _unpack(jnp.concatenate([o_r[g, pl.ds(h0, rows // 2), :] for g in range(k0, k1)], axis=1))
        y = _dot(lhs, _unpack(wo_u[n, 64 * k0:64 * k1, :]))
        cols = slice(128 * n, 128 * n + 128)
        if k0 > 0:
            y = y + x1_ref[seg, pl.ds(r0, rows), cols]
        if k1 == NG:
            y = _rb(x_ref[seg, pl.ds(r0, rows), cols].astype(f32) + y)
        x1_ref[seg, pl.ds(r0, rows), cols] = y

    def ln2(seg, c, t):
        r0 = pl.multiple_of(c * CH + t * SUB, SUB)
        lane = lax.broadcasted_iota(i32, (SUB, 128), 1)
        x1 = x1_ref[seg, pl.ds(r0, SUB), :]
        xn2 = _ln(x1, CFG['lnmode'])
        r = _rb(jnp.sum(xn2 * wrf_ref[...], axis=-1, keepdims=True))
        r_ref[SUB * t:SUB * t + SUB, :] = jnp.where(lane == seg * NG + c, r, r_ref[SUB * t:SUB * t + SUB, :])
        x_ref[seg, pl.ds(r0, SUB), :] = (x1 + xn2).astype(bf16)

    def group(s, g, par, last=False):
        nd, upd, qk, mx, ex = attn_items(g, par, o_refs[s % 2], s > 0)
        fill = []
        extra = []
        if s > 0:
            for n in range(NG):
                fill.append((128, lambda n=n: oproj(s - 1, g * CH, CH, n, o_refs[(s - 1) % 2])))
            extra = [lambda t=t: ln2(s - 1, g, t) for t in range(CH // SUB)]
        else:
            extra = [lambda seg=seg, t=t: ln1(seg, g * (CH // SUB) + t)
                     for seg in range(1, NSEG) for t in range(CH // SUB)]
        n_o = len(fill)
        if not last:
            gn = g + 1
            pj = proj_items(s + gn // NG, gn % NG, 1 - par)
            for m, n in [(m, n) for m in range(4) for n in range(2)] + [(m, 2) for m in range(4)]:
                for h in range(2):
                    fill.append((128, lambda m=m, n=n, h=h: pj(m, n, h)))
        else:
            for m in range(4):
                for n in range(NG):
                    fill.append((128, lambda m=m, n=n: oproj(s, 128 * m, 128, n, o_refs[s % 2], 0, 4)))
        fill = iter(fill)
        nfill = [0]

        def f(k=1):
            for _ in range(k):
                next(fill)[1]()
                nfill[0] += 1
                if extra and nfill[0] > n_o + 1 and (nfill[0] % 2 == 0 or s == 0):
                    extra.pop(0)()

        if s > 0:
            f(2)
            nd()
        qk(3)
        f(2)
        mx(3)
        qk(2)
        f(1)
        for t in range(4):
            ex(3, t)
            f(1)
        mx(2)
        qk(1)
        for t in range(3):
            f(1)
            ex(2, t)
        mx(1)
        qk(0)
        if s < NSEG - 1:
            upd()
        f(1)
        ex(1, 0)
        f(1)
        ex(1, 1)
        mx(0)
        f(1)
        ex(0, 0)
        for it in fill:
            it[1]()
            nfill[0] += 1
            if extra and (nfill[0] % 2 == 0 or s == 0):
                extra.pop(0)()
        for e in extra:
            e()

    cp_x0().start()
    for j in range(3):
        cp_w(0, j).start()
    for cp in cp_small():
        cp.start()
    for j in range(3):
        cp_w(1, j).start()
    cp_xr(0).start()

    ones = jnp.full((8, 512), 0x3F803F80, u32)
    vt0[64:72, :] = ones
    vt1[64:72, :] = ones
    bias_ref[...] = jnp.where(lax.broadcasted_iota(i32, (32, 128), 0)
                              <= (lax.broadcasted_iota(i32, (32, 128), 1) & 31), 0.0, NEG)

    cp_x0().wait()
    for g in range(2, NG):
        for j in range(3):
            cp_w(g, j).start()
        cp_xr(g - 1).start()
    cp_xr(NG - 1).start()
    for cp in cp_wo():
        cp.start()

    def ln0_body(t, carry):
        ln1(0, t)
        return carry
    lax.fori_loop(0, L // SUB, ln0_body, 0, unroll=4)

    for cp in cp_small():
        cp.wait()
    wrf_ref[...] = wr_ref[...].astype(f32)
    gl = _rb(jax.nn.sigmoid(beta_ref[...].astype(f32)))
    hr = lax.broadcasted_iota(i32, (32, 32), 0)
    hc = lax.broadcasted_iota(i32, (32, 32), 1)
    gcol = jnp.sum(jnp.where(hr == hc, gl, 0.0), axis=1, keepdims=True)
    gate_ref[0:32, :] = jnp.broadcast_to(gcol, (32, 128))
    gate_ref[32:64, :] = jnp.broadcast_to(_rb(1.0 - gcol), (32, 128))
    for j in range(3):
        cp_w(0, j).wait()
    if CFG['prewait']:
        for g in range(NG):
            cp_xr(g).wait()
            for j in range(3 * (g > 0)):
                cp_w(g, j).wait()

    def layer(li, carry):
        first = li == 0
        r_ref[...] = jnp.full((CH, 128), -jnp.inf, f32)
        pj = proj_items(0, 0, 0)
        for m in range(4):
            for n in range(3):
                pj(m, n, 0)
                pj(m, n, 1)

        for s in range(NSEG):
            def pair(p, c2, s=s, last=False):
                if s == 0 and not CFG['prewait']:
                    @pl.when(first)
                    def _():
                        for par in range(2):
                            g = 2 * p + par
                            cp_xr(g).wait()

                            @pl.when(g + 1 < NG)
                            def _():
                                gn = jnp.minimum(g + 1, NG - 1)
                                for j in range(3):
                                    cp_w(gn, j).wait()
                for par in range(2):
                    group(s, 2 * p + par, par, last and par == 1)
                return c2

            if s == 1:
                @pl.when(first)
                def _():
                    for cp in cp_wo():
                        cp.wait()
                    for cp in cp_ff():
                        cp.start()
            if s >= 2:
                @pl.when(li == CFG['nl'] - 1)
                def _():
                    cp_out_seg(s - 2).start()
            if s in (1, 2) and CFG['gp'] > 2:
                np_ = CFG['gp'] // 2

                def multi(p, c2, pair=pair):
                    for u in range(np_):
                        pair(np_ * p + u, c2)
                    return c2
                if np_ == NG // 2 and not CFG['rep']:
                    multi(0, 0)
                else:
                    _loop('s%d' % s, NG // 2 // np_, multi)
            elif s < NSEG - 1:
                _loop('s%d' % s, NG // 2, pair)
            else:
                _loop('s%d' % s, NG // 2 - 1, pair)
                pair(NG // 2 - 1, 0, last=True)

        s = NSEG - 1
        pend = []
        for m in (3, 2, 1, 0):
            for n in range(NG):
                oproj(s, 128 * m, 128, n, o_refs[s % 2], 4, NG)
                if pend:
                    pend.pop(0)()
            pend = [lambda c=c, t=t: ln2(s, c, t) for c in (2 * m, 2 * m + 1) for t in range(CH // SUB)]
        for e in pend:
            e()

        @pl.when(li == CFG['nl'] - 1)
        def _():
            cp_out_seg(NSEG - 2).start()
            cp_out_seg(NSEG - 1).start()

        rm = r_ref[...]
        idx = (lax.broadcasted_iota(i32, (CH, 128), 1) * CH + lax.broadcasted_iota(i32, (CH, 128), 0)).astype(f32)
        big = float(S)
        m1 = jnp.max(rm, axis=(0, 1), keepdims=True)
        i1 = jnp.min(jnp.where(rm == m1, idx, big), axis=(0, 1), keepdims=True)
        rm2 = jnp.where(idx == i1, -jnp.inf, rm)
        m2 = jnp.max(rm2, axis=(0, 1), keepdims=True)
        i2 = jnp.min(jnp.where(jnp.logical_and(rm2 == m2, idx != i1), idx, big), axis=(0, 1), keepdims=True)
        toks = [jnp.clip(jnp.max(iv).astype(i32), 0, S - 1) for iv in (i1, i2)]

        @pl.when(first)
        def _():
            for cp in cp_ff():
                cp.wait()

        row = lax.broadcasted_iota(i32, (SUB, D), 0)
        x1s = jnp.where(row == 0, x1_ref[toks[0] // L, pl.ds(toks[0] % L, 1), :],
                        jnp.where(row == 1, x1_ref[toks[1] // L, pl.ds(toks[1] % L, 1), :], 0.0))
        xs = _ln(x1s, 2 * CFG['lnmode']).astype(bf16)
        hs = []
        for c in range(NF):
            ga = _rb(_dot(xs, _unpack(wg_u[c])))
            up = _rb(_dot(xs, _unpack(wu_u[c])))
            hs.append((_rb(ga * _rb(jax.nn.sigmoid(ga))) * up).astype(bf16))
            ln1(0, c)
        hdn = jnp.concatenate(hs, axis=1)
        ys = []
        for c in range(NG):
            ys.append(_dot(hdn, _unpack(wd_u[c])))
            if NF + c < L // SUB:
                ln1(0, NF + c)
        y = _rb(jnp.concatenate(ys, axis=1))
        rsel = jnp.where(lax.broadcasted_iota(i32, (SUB, 1), 0) == 0, m1, m2)
        y = _rb(y * _rb(jax.nn.sigmoid(rsel)))
        x2s = _rb(x1s + _rb(xs.astype(f32) + y))
        xns = _ln(x2s)

        @pl.when(li == CFG['nl'] - 1)
        def _():
            for s in range(NSEG):
                cp_out_seg(s).wait()

        blks = []
        for n, t in enumerate(toks):
            sg = t // L
            b0 = pl.multiple_of((t % L) // SUB * SUB, SUB)
            hb = pl.multiple_of((t % L) // SUB * (SUB // 2), SUB // 2)
            hit = row == (t % SUB)
            old = x_ref[sg, pl.ds(b0, SUB), :].astype(f32)
            x_ref[sg, pl.ds(b0, SUB), :] = jnp.where(hit, x2s[n:n + 1], old).astype(bf16)
            oldn = _unpack(xn_ref[sg, pl.ds(hb, SUB // 2), :]).astype(f32)
            xn_ref[sg, pl.ds(hb, SUB // 2), :] = _pack(jnp.where(hit, xns[n:n + 1], oldn))
            blks.append((sg, b0))

        @pl.when(li == CFG['nl'] - 1)
        def _():
            def cp_fix(n):
                sg, b0 = blks[n]
                return pltpu.make_async_copy(x_ref.at[sg, pl.ds(b0, SUB), :],
                                             out_hbm.at[sg, pl.ds(b0, SUB), :], sems.at[SEM_FIX + n])
            differ = (toks[0] // SUB) != (toks[1] // SUB)
            cp_fix(0).start()

            @pl.when(differ)
            def _():
                cp_fix(1).start()
                cp_fix(1).wait()
            cp_fix(0).wait()
        return carry

    lax.fori_loop(0, CFG['nl'], layer, 0)


@jax.jit
def pallas_interleave_layers__memory_aug_infini_attn__moe_arch_mod__prompt_kernel(
    A_x: jax.Array,
    A_wq: jax.Array,
    A_wk: jax.Array,
    A_wv: jax.Array,
    A_wo: jax.Array,
    A_beta: jax.Array,
    B_x: jax.Array,
    B_w_r: jax.Array,
    B_w_gate: jax.Array,
    B_w_up: jax.Array,
    B_w_down: jax.Array,
):
    del B_x
    qkv_bufs = [pltpu.VMEM((L // 2, 128), u32)] * 4 + [pltpu.VMEM((72, L), u32)]
    scratch = [
        pltpu.VMEM((NSEG, L, D), bf16),
        pltpu.VMEM((NSEG, L // 2, D), u32),
        pltpu.VMEM((NSEG, L, D), f32),
        pltpu.VMEM((3 * NG, D, 128), bf16),
        pltpu.VMEM((NG, D, 128), bf16),
        pltpu.VMEM((NF, D, 128), bf16),
        pltpu.VMEM((NF, D, 128), bf16),
        pltpu.VMEM((NG, F, 128), bf16),
        pltpu.VMEM((1, 32), bf16),
        pltpu.VMEM((1, D), bf16),
        pltpu.VMEM((1, D), f32),
        pltpu.VMEM((64, 128), f32),
        pltpu.VMEM((32, 128), f32),
        pltpu.VMEM((NG, 144, 128), f32),
        pltpu.VMEM((CH, 128), f32),
        pltpu.VMEM((144, L), f32),
        pltpu.VMEM((128, L), f32), pltpu.VMEM((256, L), f32),
        pltpu.VMEM((384, L), f32), pltpu.VMEM((512, L), f32),
        *qkv_bufs, *qkv_bufs,
        pltpu.VMEM((NG, L // 2, 128), u32),
        pltpu.VMEM((NG, L // 2, 128), u32),
        pltpu.SemaphoreType.DMA((NSEM,)),
    ]
    out = pl.pallas_call(
        _kernel,
        out_shape=jax.ShapeDtypeStruct((NSEG, L, D), bf16),
        in_specs=[pl.BlockSpec(memory_space=pl.ANY)] * 10,
        out_specs=pl.BlockSpec(memory_space=pl.ANY),
        scratch_shapes=scratch,
        compiler_params=pltpu.CompilerParams(vmem_limit_bytes=100 * 2 ** 20),
    )(A_x.reshape(NSEG, L, D), A_wq, A_wk, A_wv, A_wo, A_beta.reshape(1, 32), B_w_r.reshape(1, D),
      B_w_gate, B_w_up, B_w_down)
    return out.reshape(1, S, D)
```

```python
import jax
import jax.numpy as jnp
from jax import lax
import jax.experimental.pallas as pl
import jax.experimental.pallas.tpu as pltpu

bf16 = jnp.bfloat16
f32 = jnp.float32
u32 = jnp.uint32
i32 = jnp.int32

S = 2048
D = 1024
L = 512
NSEG = 4
NG = 8
F = 3584
CH = 64
SUB = 16
NEG = -1e30
QSCALE = (32 ** -0.5) * 1.4426950408889634
NT = (((1,), (1,)), ((), ()))

SEM_X0 = 0
SEM_XR = 1
SEM_W = 9
SEM_WO = 33
SEM_SM = 34
SEM_FF = 36
SEM_OUT = 39
SEM_FIX = 43
NSEM = 45
NF = F // 128
PORDER = [(m, n) for m in range(4) for n in range(2)] + [(m, 2) for m in range(4)]

CFG = dict(
    rep={}, lnmode=0, nl=2, prewait=False, gp=2, pace=True,
    pre='Q3',
    sched='M3 f p30 f n q2 v30 p31 f f v31 p32 f f m2 v32 p33 f f v33 p20 f f q1 v20 p21 f x f v21 p22 f x f '
          'm1 v22 p10 f x f q0 v10 p11 f x f u v11 m0 f p00 f f v00 F Q3',
    sched0='M3 f p30 x f x q2 v30 p31 f x f x v31 p32 f x f x m2 v32 p33 f x f x v33 p20 f x f x q1 v20 p21 f f '
           'v21 p22 f f m1 v22 p10 f f q0 v10 p11 f f u v11 m0 f p00 f f v00 F Q3',
    schedL='M3 f p30 f n q2 v30 p31 f f v31 p32 f f m2 v32 p33 f f v33 p20 f f q1 v20 p21 f x f v21 p22 f x f '
          'm1 v22 p10 f x f q0 v10 p11 f x f v11 m0 f p00 f f v00 F',
)


def _loop(name, n, body):
    rep = CFG['rep'].get(name, 1)
    if rep == 1:
        return lax.fori_loop(0, n, body, 0)
    return lax.fori_loop(0, n * rep, lambda i, c: body(i // rep, c), 0)


def _rb(x):
    return x.astype(bf16).astype(f32)


def _pack(x):
    return pltpu.bitcast(x.astype(bf16), u32)


def _unpack(u):
    return pltpu.bitcast(u, bf16)


def _phi(t):
    return jnp.where(t > 0, t + 1.0, jnp.exp(t))


def _dot(a, b):
    return jnp.dot(a, b, preferred_element_type=f32)


def _unskew(ps):
    shape, dt = next((p.shape, p.dtype) for p in ps if p is not None)
    c = lax.broadcasted_iota(i32, shape, 1) >> 5
    even = (c & 1) == 0
    lo = c < 2
    mid = jnp.logical_or(c == 1, c == 2)

    def sel(mask, a, b):
        if a is None and b is None:
            return None
        z = jnp.zeros(shape, dt)
        return jnp.where(mask, z if a is None else a, z if b is None else b)
    x0, x1 = sel(even, ps[0], ps[1]), sel(even, ps[1], ps[0])
    x2, x3 = sel(even, ps[2], ps[3]), sel(even, ps[3], ps[2])
    return [sel(lo, x0, x2), sel(mid, x1, x3), sel(lo, x2, x0), sel(mid, x3, x1)]


def _ln(x, mode=0):
    m = jnp.sum(x, axis=-1, keepdims=True) * (1.0 / D)
    if mode == 0:
        e = x - m
        v = jnp.sum(e * e, axis=-1, keepdims=True) * (1.0 / D)
        return e * lax.rsqrt(v + 1e-5)
    c = _rb(m)
    e = x - c
    v = jnp.sum(e * e, axis=-1, keepdims=True) * (1.0 / D) - (m - c) * (m - c)
    w = _rb(_rb(jnp.maximum(v, 0.0)) + 1e-5)
    den = _rb(w * lax.rsqrt(w))
    if mode == 2:
        return _rb(_rb(e) / den)
    return e * (1.0 / den)


def _kernel(x_hbm, wq_hbm, wk_hbm, wv_hbm, wo_hbm, beta_hbm, wr_hbm, wg_hbm, wu_hbm, wd_hbm,
            out_hbm,
            x_ref, xn_ref, x1_ref, w_ref, wo_ref, wg_ref, wu_ref, wd_ref,
            beta_ref, wr_ref, wrf_ref, gate_ref, bias_ref, m_ref, r_ref, nd_ref,
            s0_ref, s1_ref, s2_ref, s3_ref, p0_ref, p1_ref, p2_ref, p3_ref, mx_ref, z_ref,
            qk0, vt0, qk1, vt1, oa_ref, ob_ref, sems):
    qkv = ((qk0, vt0), (qk1, vt1))
    o_refs = (oa_ref, ob_ref)
    s_refs = (s0_ref, s1_ref, s2_ref, s3_ref)
    p_refs = (p0_ref, p1_ref, p2_ref, p3_ref)
    xn_b = xn_ref.bitcast(bf16)
    w_u, wo_u, wg_u, wu_u, wd_u = (r.bitcast(u32) for r in (w_ref, wo_ref, wg_ref, wu_ref, wd_ref))

    def cp_x0():
        return pltpu.make_async_copy(x_hbm.at[0], x_ref.at[0], sems.at[SEM_X0])

    def cp_xr(g):
        r0 = pl.multiple_of(g * CH, CH)
        return pltpu.make_async_copy(x_hbm.at[1:NSEG, pl.ds(r0, CH), :],
                                     x_ref.at[1:NSEG, pl.ds(r0, CH), :], sems.at[SEM_XR + g])

    def cp_w(g, j):
        c0 = pl.multiple_of(g * 128, 128)
        src = (wq_hbm, wk_hbm, wv_hbm)[j]
        return pltpu.make_async_copy(src.at[:, pl.ds(c0, 128)], w_ref.at[3 * g + j], sems.at[SEM_W + 3 * g + j])

    def slabs(src, dst, n, sem):
        return [pltpu.make_async_copy(src.at[:, 128 * c:128 * c + 128], dst.at[c], sems.at[sem]) for c in range(n)]

    def cp_wo():
        return slabs(wo_hbm, wo_ref, NG, SEM_WO)

    def cp_small():
        return (pltpu.make_async_copy(beta_hbm, beta_ref, sems.at[SEM_SM]),
                pltpu.make_async_copy(wr_hbm, wr_ref, sems.at[SEM_SM + 1]))

    def cp_ff():
        return (slabs(wg_hbm, wg_ref, NF, SEM_FF) + slabs(wu_hbm, wu_ref, NF, SEM_FF + 1)
                + slabs(wd_hbm, wd_ref, NG, SEM_FF + 2))

    def cp_out_seg(s):
        return pltpu.make_async_copy(x_ref.at[s], out_hbm.at[s], sems.at[SEM_OUT + s])

    def after(x, tok, frac):
        if tok is None or not CFG['pace']:
            return x
        r = 8 * int(frac * tok.shape[0] // 8)
        t = pltpu.bitcast(tok[r:r + 8, 0:128], u32) & z_ref[...]
        return pltpu.bitcast(pltpu.bitcast(x, u32) | t, f32)

    def proj_items(seg, g, par):
        qk_r, vt_r = (r.bitcast(bf16) for r in qkv[par])
        part = {}

        def item(m, n, h):
            xn = _unpack(xn_ref[seg, 64 * m:64 * m + 64, 512 * h:512 * h + 512])
            y = _dot(xn, _unpack(w_u[3 * g + n, 256 * h:256 * h + 256, :]))
            if h == 0:
                part[m, n] = y
                return y
            y = y + part.pop((m, n))
            rows = slice(128 * m, 128 * m + 128)
            if n == 0:
                qk_r[rows, 0:128] = (y * QSCALE).astype(bf16)
                qk_r[rows, 128:256] = _phi(y).astype(bf16)
            elif n == 1:
                qk_r[rows, 256:384] = y.astype(bf16)
                qk_r[rows, 384:512] = _phi(y).astype(bf16)
            else:
                vt_r[0:128, rows] = y.T.astype(bf16)
            return y
        return item

    def attn_items(g, par, o_r, use_mem):
        qk_r, vt_r = qkv[par]
        st = {}

        def nd():
            ml = m_ref[g].astype(bf16)
            nd_ref[...] = lax.dot_general(ml, _unpack(qk_r[:, 128:256]), NT, preferred_element_type=f32)

        def upd():
            u = _dot(_unpack(vt_r[...]), _unpack(qk_r[:, 384:512]))
            r2 = lax.broadcasted_iota(i32, (144, 128), 0)
            c2 = lax.broadcasted_iota(i32, (144, 128), 1) >> 5
            keep = jnp.where(r2 < 128, r2 >> 5, r2 - 128) == c2
            u = jnp.where(keep, u, 0.0)
            m_ref[g] = (m_ref[g] + u) if use_mem else u

        def qk(i):
            lane = lax.broadcasted_iota(i32, (16, 128), 1) >> 5
            for be in (range(4) if i % 2 else range(3, -1, -1)):
                b = 4 * i + be
                n = 32 * (b + 1)
                qu = qk_r[16 * b:16 * b + 16, 0:128]
                wq = _unpack(jnp.concatenate(
                    [jnp.where(lane == (c - be) % 4, qu, jnp.uint32(0)) for c in range(4)], axis=0))
                s = lax.dot_general(_unpack(qk_r[0:n // 2, 256:384]), wq, NT, preferred_element_type=f32)
                cols = slice(128 * be, 128 * be + 128)
                if b > 0:
                    s_refs[i][0:n - 32, cols] = s[0:n - 32]
                s_refs[i][n - 32:n, cols] = s[n - 32:n] + bias_ref[...]

        def mx(i, mode='m'):
            for be in range(4):
                if mode == 'load':
                    st[i, 'm', be] = mx_ref[4 * i + be:4 * i + be + 1, :]
                    continue
                n = 32 * (4 * i + be + 1)
                sv = s_refs[i][0:n, 128 * be:128 * be + 128]
                m = jnp.max(jnp.max(sv.reshape(n // 8, 8, 128), axis=0), axis=0, keepdims=True)
                if mode == 'store':
                    mx_ref[4 * i + be:4 * i + be + 1, :] = m
                else:
                    st[i, 'm', be] = m

        def pr(i, t, tok):
            ps = []
            for be in range(4):
                n = 128 if t < i else 32 * (be + 1)
                m8 = after(jnp.broadcast_to(st[i, 'm', be], (8, 128)), tok, be / 4)
                p = jnp.exp2(s_refs[i][128 * t:128 * t + n, 128 * be:128 * be + 128].reshape(n // 8, 8, 128) - m8)
                ls = jnp.sum(p, axis=0)
                p = p.reshape(n, 128)
                st[i, 'l', be] = ls if t == 0 else st[i, 'l', be] + ls
                p_refs[i].bitcast(bf16)[128 * t:128 * t + n, 128 * be:128 * be + 128] = p.astype(bf16)

        def pv(i, t):
            ps = [p_refs[i][64 * t:64 * t + (64 if t < i else 16 * (be + 1)), 128 * be:128 * be + 128]
                  for be in range(4)]
            if t < i:
                ts = _unskew(ps)
            else:
                blk = [_unskew([ps[be][16 * u:16 * u + 16] if be >= u else None for be in range(4)])
                       for u in range(4)]
                ts = [jnp.concatenate([blk[u][j] for u in range(4)], axis=0) for j in range(4)]
            for j in range(4):
                o = _dot(_unpack(vt_r[16 * j:16 * j + 16, 128 * t:128 * t + 128]), _unpack(ts[j]))
                st[i, 'o', j] = o if t == 0 else st[i, 'o', j] + o

        def fin(i):
            ls = _unskew([jnp.sum(st.pop((i, 'l', be)), axis=0, keepdims=True) for be in range(4)])
            parts = []
            for j in range(4):
                gt = gate_ref[pl.ds(4 * g + j, 1), :]
                omg = gate_ref[pl.ds(32 + 4 * g + j, 1), :]
                o = st.pop((i, 'o', j)) * (omg / ls[j])
                if j > 0:
                    o = pltpu.roll(o, 128 - 32 * j, 1)
                if use_mem:
                    den = nd_ref[128 + j:129 + j, 128 * i:128 * i + 128] + 1e-6
                    o = o + nd_ref[32 * j:32 * j + 32, 128 * i:128 * i + 128] * (gt / den)
                parts.append(o)
            ot = jnp.concatenate(parts, axis=0)
            o_r.bitcast(bf16)[g // 2, 128 * i:128 * i + 128, 128 * par:128 * par + 128] = ot.T.astype(bf16)

        def ex(kind, i, t, tok):
            if kind in 'ep':
                pr(i, t, tok)
            if kind in 'ev':
                pv(i, t)
                if t == i:
                    fin(i)
        return nd, upd, qk, mx, ex

    def ln1(seg, r):
        r0 = pl.multiple_of(r * SUB, SUB)
        xn_b[seg, pl.ds(r0, SUB), :] = _ln(x_ref[seg, pl.ds(r0, SUB), :].astype(f32)).astype(bf16)

    def oproj(seg, r0, rows, n, o_r, k0=0, k1=NG):
        h0 = pl.multiple_of(r0 // 2, rows // 2)
        r0 = pl.multiple_of(r0, rows)
        lhs = _unpack(jnp.concatenate([o_r[p, pl.ds(h0, rows // 2), :] for p in range(k0 // 2, k1 // 2)], axis=1))
        y = _dot(lhs, _unpack(wo_u[n, 64 * k0:64 * k1, :]))
        cols = slice(128 * n, 128 * n + 128)
        if k0 > 0:
            y = y + x1_ref[seg, pl.ds(r0, rows), cols]
        if k1 == NG:
            y = _rb(x_ref[seg, pl.ds(r0, rows), cols].astype(f32) + y)
        x1_ref[seg, pl.ds(r0, rows), cols] = y
        return y

    def ln2(seg, c, t):
        r0 = pl.multiple_of(c * CH + t * SUB, SUB)
        lane = lax.broadcasted_iota(i32, (SUB, 128), 1)
        x1 = x1_ref[seg, pl.ds(r0, SUB), :]
        xn2 = _ln(x1, CFG['lnmode'])
        r = _rb(jnp.sum(xn2 * wrf_ref[...], axis=-1, keepdims=True))
        r_ref[SUB * t:SUB * t + SUB, :] = jnp.where(lane == seg * NG + c, r, r_ref[SUB * t:SUB * t + SUB, :])
        x_ref[seg, pl.ds(r0, SUB), :] = (x1 + xn2).astype(bf16)

    def group(s, g, par, last=False):
        nd, upd, qk, mx, ex = attn_items(g, par, o_refs[s % 2], s > 0)
        fill = []
        extra = []
        if s > 0:
            for n in range(NG):
                fill.append((128, lambda n=n: oproj(s - 1, g * CH, CH, n, o_refs[(s - 1) % 2])))
            extra = [lambda t=t: ln2(s - 1, g, t) for t in range(CH // SUB)]
        else:
            extra = [lambda seg=seg, t=t: ln1(seg, g * (CH // SUB) + t)
                     for seg in range(1, NSEG) for t in range(CH // SUB)]
        if not last:
            gn = g + 1
            pj = proj_items(s + gn // NG, gn % NG, 1 - par)
            for m, n in PORDER:
                for h in range(2):
                    fill.append((128, lambda m=m, n=n, h=h: pj(m, n, h)))
        else:
            for m in range(4):
                for n in range(NG):
                    fill.append((128, lambda m=m, n=n: oproj(s, 128 * m, 128, n, o_refs[s % 2], 0, 4)))
        sched = CFG['sched0' if s == 0 else 'schedL' if last else 'sched'].split()
        y = None
        for tok in sched:
            if tok == 'f':
                y = fill.pop(0)[1]()
            elif tok == 'F':
                while fill:
                    fill.pop(0)[1]()
            elif tok == 'x':
                extra.pop(0)()
            elif tok == 'n':
                nd()
            elif tok == 'u':
                if s < NSEG - 1:
                    upd()
            elif tok[0] == 'q':
                qk(int(tok[1]))
            elif tok[0] == 'Q':
                nxt = attn_items(None, 1 - par, None, None)
                nxt[2](int(tok[1]))
                nxt[3](int(tok[1]), 'store')
            elif tok[0] == 'M':
                mx(int(tok[1]), 'load')
            elif tok[0] == 'm':
                mx(int(tok[1]))
            else:
                ex(tok[0], int(tok[1]), int(tok[2]), y)
        for it in fill:
            it[1]()
        for e in extra:
            e()

    cp_x0().start()
    for j in range(3):
        cp_w(0, j).start()
    for cp in cp_small():
        cp.start()
    for j in range(3):
        cp_w(1, j).start()
    cp_xr(0).start()

    z_ref[...] = jnp.zeros((8, 128), u32)
    ones = jnp.full((8, 512), 0x3F803F80, u32)
    vt0[64:72, :] = ones
    vt1[64:72, :] = ones
    bias_ref[...] = jnp.where(lax.broadcasted_iota(i32, (32, 128), 0)
                              <= (lax.broadcasted_iota(i32, (32, 128), 1) & 31), 0.0, NEG)

    cp_x0().wait()
    for g in range(2, NG):
        for j in range(3):
            cp_w(g, j).start()
        cp_xr(g - 1).start()
    cp_xr(NG - 1).start()
    for cp in cp_wo():
        cp.start()

    def ln0_body(t, carry):
        ln1(0, t)
        return carry
    lax.fori_loop(0, L // SUB, ln0_body, 0, unroll=4)

    for cp in cp_small():
        cp.wait()
    wrf_ref[...] = wr_ref[...].astype(f32)
    gl = _rb(jax.nn.sigmoid(beta_ref[...].astype(f32)))
    hr = lax.broadcasted_iota(i32, (32, 32), 0)
    hc = lax.broadcasted_iota(i32, (32, 32), 1)
    gcol = jnp.sum(jnp.where(hr == hc, gl, 0.0), axis=1, keepdims=True)
    gate_ref[0:32, :] = jnp.broadcast_to(gcol, (32, 128))
    gate_ref[32:64, :] = jnp.broadcast_to(_rb(1.0 - gcol), (32, 128))
    for j in range(3):
        cp_w(0, j).wait()
    if CFG['prewait']:
        for g in range(NG):
            cp_xr(g).wait()
            for j in range(3 * (g > 0)):
                cp_w(g, j).wait()

    def layer(li, carry):
        first = li == 0
        r_ref[...] = jnp.full((CH, 128), -jnp.inf, f32)
        pj = proj_items(0, 0, 0)
        for m, n in PORDER:
            if True:
                pj(m, n, 0)
                pj(m, n, 1)
        for tok in CFG['pre'].split():
            nxt = attn_items(None, 0, None, None)
            nxt[2](int(tok[1]))
            nxt[3](int(tok[1]), 'store')

        for s in range(NSEG):
            def pair(p, c2, s=s, last=False):
                if s == 0 and not CFG['prewait']:
                    @pl.when(first)
                    def _():
                        for par in range(2):
                            g = 2 * p + par
                            cp_xr(g).wait()

                            @pl.when(g + 1 < NG)
                            def _():
                                gn = jnp.minimum(g + 1, NG - 1)
                                for j in range(3):
                                    cp_w(gn, j).wait()
                for par in range(2):
                    group(s, 2 * p + par, par, last and par == 1)
                return c2

            if s == 1:
                @pl.when(first)
                def _():
                    for cp in cp_wo():
                        cp.wait()
                    for cp in cp_ff():
                        cp.start()
            if s >= 2:
                @pl.when(li == CFG['nl'] - 1)
                def _():
                    cp_out_seg(s - 2).start()
            if s in (1, 2) and CFG['gp'] > 2:
                np_ = CFG['gp'] // 2

                def multi(p, c2, pair=pair):
                    for u in range(np_):
                        pair(np_ * p + u, c2)
                    return c2
                if np_ == NG // 2 and not CFG['rep']:
                    multi(0, 0)
                else:
                    _loop('s%d' % s, NG // 2 // np_, multi)
            elif s < NSEG - 1:
                _loop('s%d' % s, NG // 2, pair)
            else:
                _loop('s%d' % s, NG // 2 - 1, pair)
                pair(NG // 2 - 1, 0, last=True)

        s = NSEG - 1
        pend = []
        for m in (3, 2, 1, 0):
            for n in range(NG):
                oproj(s, 128 * m, 128, n, o_refs[s % 2], 4, NG)
                if pend:
                    pend.pop(0)()
            pend = [lambda c=c, t=t: ln2(s, c, t) for c in (2 * m, 2 * m + 1) for t in range(CH // SUB)]
        for e in pend:
            e()

        @pl.when(li == CFG['nl'] - 1)
        def _():
            cp_out_seg(NSEG - 2).start()
            cp_out_seg(NSEG - 1).start()

        rm = r_ref[...]
        idx = (lax.broadcasted_iota(i32, (CH, 128), 1) * CH + lax.broadcasted_iota(i32, (CH, 128), 0)).astype(f32)
        big = float(S)
        m1 = jnp.max(rm, axis=(0, 1), keepdims=True)
        i1 = jnp.min(jnp.where(rm == m1, idx, big), axis=(0, 1), keepdims=True)
        rm2 = jnp.where(idx == i1, -jnp.inf, rm)
        m2 = jnp.max(rm2, axis=(0, 1), keepdims=True)
        i2 = jnp.min(jnp.where(jnp.logical_and(rm2 == m2, idx != i1), idx, big), axis=(0, 1), keepdims=True)
        toks = [jnp.clip(jnp.max(iv).astype(i32), 0, S - 1) for iv in (i1, i2)]

        @pl.when(first)
        def _():
            for cp in cp_ff():
                cp.wait()

        row = lax.broadcasted_iota(i32, (SUB, D), 0)
        x1s = jnp.where(row == 0, x1_ref[toks[0] // L, pl.ds(toks[0] % L, 1), :],
                        jnp.where(row == 1, x1_ref[toks[1] // L, pl.ds(toks[1] % L, 1), :], 0.0))
        xs = _ln(x1s, 2 * CFG['lnmode']).astype(bf16)
        hs = []
        for c in range(NF):
            ga = _rb(_dot(xs, _unpack(wg_u[c])))
            up = _rb(_dot(xs, _unpack(wu_u[c])))
            hs.append((_rb(ga * _rb(jax.nn.sigmoid(ga))) * up).astype(bf16))
            ln1(0, c)
        hdn = jnp.concatenate(hs, axis=1)
        ys = []
        for c in range(NG):
            ys.append(_dot(hdn, _unpack(wd_u[c])))
            if NF + c < L // SUB:
                ln1(0, NF + c)
        y = _rb(jnp.concatenate(ys, axis=1))
        rsel = jnp.where(lax.broadcasted_iota(i32, (SUB, 1), 0) == 0, m1, m2)
        y = _rb(y * _rb(jax.nn.sigmoid(rsel)))
        x2s = _rb(x1s + _rb(xs.astype(f32) + y))
        xns = _ln(x2s)

        @pl.when(li == CFG['nl'] - 1)
        def _():
            for s in range(NSEG):
                cp_out_seg(s).wait()

        blks = []
        for n, t in enumerate(toks):
            sg = t // L
            b0 = pl.multiple_of((t % L) // SUB * SUB, SUB)
            hb = pl.multiple_of((t % L) // SUB * (SUB // 2), SUB // 2)
            hit = row == (t % SUB)
            old = x_ref[sg, pl.ds(b0, SUB), :].astype(f32)
            x_ref[sg, pl.ds(b0, SUB), :] = jnp.where(hit, x2s[n:n + 1], old).astype(bf16)
            oldn = _unpack(xn_ref[sg, pl.ds(hb, SUB // 2), :]).astype(f32)
            xn_ref[sg, pl.ds(hb, SUB // 2), :] = _pack(jnp.where(hit, xns[n:n + 1], oldn))
            blks.append((sg, b0))

        @pl.when(li == CFG['nl'] - 1)
        def _():
            def cp_fix(n):
                sg, b0 = blks[n]
                return pltpu.make_async_copy(x_ref.at[sg, pl.ds(b0, SUB), :],
                                             out_hbm.at[sg, pl.ds(b0, SUB), :], sems.at[SEM_FIX + n])
            differ = (toks[0] // SUB) != (toks[1] // SUB)
            cp_fix(0).start()

            @pl.when(differ)
            def _():
                cp_fix(1).start()
                cp_fix(1).wait()
            cp_fix(0).wait()
        return carry

    lax.fori_loop(0, CFG['nl'], layer, 0)


@jax.jit
def pallas_interleave_layers__memory_aug_infini_attn__moe_arch_mod__prompt_kernel(
    A_x: jax.Array,
    A_wq: jax.Array,
    A_wk: jax.Array,
    A_wv: jax.Array,
    A_wo: jax.Array,
    A_beta: jax.Array,
    B_x: jax.Array,
    B_w_r: jax.Array,
    B_w_gate: jax.Array,
    B_w_up: jax.Array,
    B_w_down: jax.Array,
):
    del B_x
    qkv_bufs = [pltpu.VMEM((L // 2, 512), u32), pltpu.VMEM((72, L), u32)]
    scratch = [
        pltpu.VMEM((NSEG, L, D), bf16),
        pltpu.VMEM((NSEG, L // 2, D), u32),
        pltpu.VMEM((NSEG, L, D), f32),
        pltpu.VMEM((3 * NG, D, 128), bf16),
        pltpu.VMEM((NG, D, 128), bf16),
        pltpu.VMEM((NF, D, 128), bf16),
        pltpu.VMEM((NF, D, 128), bf16),
        pltpu.VMEM((NG, F, 128), bf16),
        pltpu.VMEM((1, 32), bf16),
        pltpu.VMEM((1, D), bf16),
        pltpu.VMEM((1, D), f32),
        pltpu.VMEM((64, 128), f32),
        pltpu.VMEM((32, 128), f32),
        pltpu.VMEM((NG, 144, 128), f32),
        pltpu.VMEM((CH, 128), f32),
        pltpu.VMEM((144, L), f32),
        pltpu.VMEM((128, L), f32), pltpu.VMEM((256, L), f32),
        pltpu.VMEM((384, L), f32), pltpu.VMEM((512, L), f32),
        pltpu.VMEM((64, L), u32), pltpu.VMEM((128, L), u32),
        pltpu.VMEM((192, L), u32), pltpu.VMEM((256, L), u32),
        pltpu.VMEM((16, 128), f32),
        pltpu.VMEM((8, 128), u32),
        *qkv_bufs, *qkv_bufs,
        pltpu.VMEM((NG // 2, L // 2, 256), u32),
        pltpu.VMEM((NG // 2, L // 2, 256), u32),
        pltpu.SemaphoreType.DMA((NSEM,)),
    ]
    out = pl.pallas_call(
        _kernel,
        out_shape=jax.ShapeDtypeStruct((NSEG, L, D), bf16),
        in_specs=[pl.BlockSpec(memory_space=pl.ANY)] * 10,
        out_specs=pl.BlockSpec(memory_space=pl.ANY),
        scratch_shapes=scratch,
        compiler_params=pltpu.CompilerParams(vmem_limit_bytes=100 * 2 ** 20),
    )(A_x.reshape(NSEG, L, D), A_wq, A_wk, A_wv, A_wo, A_beta.reshape(1, 32), B_w_r.reshape(1, D),
      B_w_gate, B_w_up, B_w_down)
    return out.reshape(1, S, D)
```

```python
import jax
import jax.numpy as jnp
from jax import lax
import jax.experimental.pallas as pl
import jax.experimental.pallas.tpu as pltpu

bf16 = jnp.bfloat16
f32 = jnp.float32
u32 = jnp.uint32
i32 = jnp.int32

S = 2048
D = 1024
L = 512
NSEG = 4
NG = 8
F = 3584
CH = 64
SUB = 16
NEG = -1e30
QSCALE = (32 ** -0.5) * 1.4426950408889634
NT = (((1,), (1,)), ((), ()))

SEM_X0 = 0
SEM_XR = 1
SEM_W = 9
SEM_WO = 33
SEM_SM = 34
SEM_FF = 36
SEM_OUT = 39
SEM_FIX = 43
SEM_X1 = 45
SEM_XC = 46
NSEM = 50
NF = F // 128
PORDER = [(m, n) for m in range(4) for n in range(2)] + [(m, 2) for m in range(4)]

CFG = dict(
    rep={}, lnmode=0, nl=2, prewait=False, gp=2, pace=True, pace2=False, nb=3, chain=True, xfrac=0.0,
    pre='f ' * 16 + 'w x x x x Q3 ' + 'f x x x x ' * 7 + 'f',
    sched='M3 f p30 f n q2 v30 p31 f f v31 p32 f f m2 v32 p33 f f v33 p20 f f q1 v20 p21 f x f v21 p22 f x f '
          'm1 v22 p10 f x f q0 v10 p11 f x f u v11 m0 f p00 f f v00 F Q3',
    sched0='M3 f p30 f q2 v30 p31 f f v31 p32 f f x m2 v32 p33 f f x v33 p20 f f x q1 v20 p21 f f x '
           'v21 p22 f f x m1 v22 p10 f f x q0 v10 p11 f x f u v11 m0 f x p00 f f v00 F Q3',
    schedL='M3 f p30 f n q2 v30 p31 f f v31 p32 f f m2 v32 p33 f f v33 p20 f f q1 v20 p21 f x f v21 p22 f x f '
          'm1 v22 p10 f x f q0 v10 p11 f x f v11 m0 f p00 f f v00 F',
)


def _loop(name, n, body):
    rep = CFG['rep'].get(name, 1)
    if rep == 1:
        return lax.fori_loop(0, n, body, 0)
    return lax.fori_loop(0, n * rep, lambda i, c: body(i // rep, c), 0)


def _rb(x):
    return x.astype(bf16).astype(f32)


def _pack(x):
    return pltpu.bitcast(x.astype(bf16), u32)


def _unpack(u):
    return pltpu.bitcast(u, bf16)


def _phi(t):
    return jnp.where(t > 0, t + 1.0, jnp.exp(t))


def _dot(a, b):
    return jnp.dot(a, b, preferred_element_type=f32)


def _unskew(ps):
    shape, dt = next((p.shape, p.dtype) for p in ps if p is not None)
    c = lax.broadcasted_iota(i32, shape, 1) >> 5
    even = (c & 1) == 0
    lo = c < 2
    mid = jnp.logical_or(c == 1, c == 2)

    def sel(mask, a, b):
        if a is None and b is None:
            return None
        z = jnp.zeros(shape, dt)
        return jnp.where(mask, z if a is None else a, z if b is None else b)
    x0, x1 = sel(even, ps[0], ps[1]), sel(even, ps[1], ps[0])
    x2, x3 = sel(even, ps[2], ps[3]), sel(even, ps[3], ps[2])
    return [sel(lo, x0, x2), sel(mid, x1, x3), sel(lo, x2, x0), sel(mid, x3, x1)]


def _ln(x, mode=0):
    acc = x
    if CFG['chain']:
        acc = x[:, 0:128]
        for c in range(1, x.shape[1] // 128):
            acc = acc + x[:, 128 * c:128 * c + 128]
    m = jnp.sum(acc, axis=-1, keepdims=True) * (1.0 / D)
    if mode == 0:
        e = x - m
        v = jnp.sum(e * e, axis=-1, keepdims=True) * (1.0 / D)
        return e * lax.rsqrt(v + 1e-5)
    c = _rb(m)
    e = x - c
    v = jnp.sum(e * e, axis=-1, keepdims=True) * (1.0 / D) - (m - c) * (m - c)
    w = _rb(_rb(jnp.maximum(v, 0.0)) + 1e-5)
    den = _rb(w * lax.rsqrt(w))
    if mode == 2:
        return _rb(_rb(e) / den)
    return e * (1.0 / den)


def _kernel(x_hbm, wq_hbm, wk_hbm, wv_hbm, wo_hbm, beta_hbm, wr_hbm, wg_hbm, wu_hbm, wd_hbm,
            out_hbm,
            x_ref, xb_ref, x1_ref, w_ref, wo_ref, wg_ref, wu_ref, wd_ref,
            beta_ref, wr_ref, wrf_ref, gate_ref, bias_ref, m_ref, r_ref, nd_ref,
            s0_ref, s1_ref, s2_ref, s3_ref, p0_ref, p1_ref, p2_ref, p3_ref, mx_ref, z_ref,
            qk0, vt0, qk1, vt1, oa_ref, ob_ref, xa_ref, sems):
    qkv = ((qk0, vt0), (qk1, vt1))
    o_refs = (oa_ref, ob_ref)
    s_refs = (s0_ref, s1_ref, s2_ref, s3_ref)
    p_refs = (p0_ref, p1_ref, p2_ref, p3_ref)
    xa_b, xb_b = xa_ref.bitcast(bf16), xb_ref.bitcast(bf16)
    w_u, wo_u, wg_u, wu_u, wd_u = (r.bitcast(u32) for r in (w_ref, wo_ref, wg_ref, wu_ref, wd_ref))

    def cp_x0(c):
        rows = pl.ds(pl.multiple_of(128 * c, 128), 128)
        return pltpu.make_async_copy(x_hbm.at[0, rows], x_ref.at[0, rows], sems.at[SEM_XC + c])

    def cp_x1():
        return pltpu.make_async_copy(x_hbm.at[1], x_ref.at[1], sems.at[SEM_X1])

    def cp_xr(g):
        r0 = pl.multiple_of(g * CH, CH)
        return pltpu.make_async_copy(x_hbm.at[2:NSEG, pl.ds(r0, CH), :],
                                     x_ref.at[2:NSEG, pl.ds(r0, CH), :], sems.at[SEM_XR + g])

    def cp_w(g, j):
        c0 = pl.multiple_of(g * 128, 128)
        src = (wq_hbm, wk_hbm, wv_hbm)[j]
        return pltpu.make_async_copy(src.at[:, pl.ds(c0, 128)], w_ref.at[3 * g + j], sems.at[SEM_W + 3 * g + j])

    def slabs(src, dst, n, sem):
        return [pltpu.make_async_copy(src.at[:, 128 * c:128 * c + 128], dst.at[c], sems.at[sem]) for c in range(n)]

    def cp_wo():
        return slabs(wo_hbm, wo_ref, NG, SEM_WO)

    def cp_small():
        return (pltpu.make_async_copy(beta_hbm, beta_ref, sems.at[SEM_SM]),
                pltpu.make_async_copy(wr_hbm, wr_ref, sems.at[SEM_SM + 1]))

    def cp_ff():
        return (slabs(wg_hbm, wg_ref, NF, SEM_FF) + slabs(wu_hbm, wu_ref, NF, SEM_FF + 1)
                + slabs(wd_hbm, wd_ref, NG, SEM_FF + 2))

    def cp_out_seg(s):
        return pltpu.make_async_copy(x_ref.at[s], out_hbm.at[s], sems.at[SEM_OUT + s])

    def after(x, tok, frac):
        if tok is None or not CFG['pace']:
            return x
        r = 8 * int(frac * tok.shape[0] // 8)
        t = pltpu.bitcast(tok[r:r + 8, 0:128], u32) & z_ref[...]
        t = jnp.tile(t, (x.shape[0] // 8, x.shape[1] // 128))
        return pltpu.bitcast(pltpu.bitcast(x, u32) | t, x.dtype)

    def proj_items(s, nxt, g, par):
        xn_r, seg = (xa_ref, nxt) if s == 0 else (xb_ref, s - 1 + nxt)
        qk_r, vt_r = (r.bitcast(bf16) for r in qkv[par])
        part = {}

        def item(m, n, h):
            xn = _unpack(xn_r[seg, 64 * m:64 * m + 64, 512 * h:512 * h + 512])
            y = _dot(xn, _unpack(w_u[3 * g + n, 256 * h:256 * h + 256, :]))
            if h == 0:
                part[m, n] = y
                return y
            y = y + part.pop((m, n))
            rows = slice(128 * m, 128 * m + 128)
            if n == 0:
                qk_r[rows, 0:128] = (y * QSCALE).astype(bf16)
                qk_r[rows, 128:256] = _phi(y).astype(bf16)
            elif n == 1:
                qk_r[rows, 256:384] = y.astype(bf16)
                qk_r[rows, 384:512] = _phi(y).astype(bf16)
            else:
                vt_r[0:128, rows] = y.T.astype(bf16)
            return y
        return item

    def attn_items(g, par, o_r, use_mem):
        qk_r, vt_r = qkv[par]
        st = {}

        def nd():
            ml = m_ref[g].astype(bf16)
            nd_ref[...] = lax.dot_general(ml, _unpack(qk_r[:, 128:256]), NT, preferred_element_type=f32)

        def upd():
            u = _dot(_unpack(vt_r[...]), _unpack(qk_r[:, 384:512]))
            r2 = lax.broadcasted_iota(i32, (144, 128), 0)
            c2 = lax.broadcasted_iota(i32, (144, 128), 1) >> 5
            keep = jnp.where(r2 < 128, r2 >> 5, r2 - 128) == c2
            u = jnp.where(keep, u, 0.0)
            m_ref[g] = (m_ref[g] + u) if use_mem else u

        def qk(i):
            lane = lax.broadcasted_iota(i32, (16, 128), 1) >> 5
            for be in (range(4) if i % 2 else range(3, -1, -1)):
                b = 4 * i + be
                n = 32 * (b + 1)
                qu = qk_r[16 * b:16 * b + 16, 0:128]
                wq = _unpack(jnp.concatenate(
                    [jnp.where(lane == (c - be) % 4, qu, jnp.uint32(0)) for c in range(4)], axis=0))
                s = lax.dot_general(_unpack(qk_r[0:n // 2, 256:384]), wq, NT, preferred_element_type=f32)
                cols = slice(128 * be, 128 * be + 128)
                if b > 0:
                    s_refs[i][0:n - 32, cols] = s[0:n - 32]
                s_refs[i][n - 32:n, cols] = s[n - 32:n] + bias_ref[...]

        def mx(i, mode='m'):
            for be in range(4):
                if mode == 'load':
                    st[i, 'm', be] = mx_ref[4 * i + be:4 * i + be + 1, :]
                    continue
                n = 32 * (4 * i + be + 1)
                sv = s_refs[i][0:n, 128 * be:128 * be + 128]
                m = jnp.max(jnp.max(sv.reshape(n // 8, 8, 128), axis=0), axis=0, keepdims=True)
                if mode == 'store':
                    mx_ref[4 * i + be:4 * i + be + 1, :] = m
                else:
                    st[i, 'm', be] = m

        def pr(i, t, tok):
            ps = []
            for be in range(4):
                n = 128 if t < i else 32 * (be + 1)
                m8 = after(jnp.broadcast_to(st[i, 'm', be], (8, 128)), tok, be / 4)
                p = jnp.exp2(s_refs[i][128 * t:128 * t + n, 128 * be:128 * be + 128].reshape(n // 8, 8, 128) - m8)
                ls = jnp.sum(p, axis=0)
                p = p.reshape(n, 128)
                st[i, 'l', be] = ls if t == 0 else st[i, 'l', be] + ls
                p_refs[i].bitcast(bf16)[128 * t:128 * t + n, 128 * be:128 * be + 128] = p.astype(bf16)

        def pv(i, t):
            ps = [p_refs[i][64 * t:64 * t + (64 if t < i else 16 * (be + 1)), 128 * be:128 * be + 128]
                  for be in range(4)]
            if t < i:
                ts = _unskew(ps)
            else:
                blk = [_unskew([ps[be][16 * u:16 * u + 16] if be >= u else None for be in range(4)])
                       for u in range(4)]
                ts = [jnp.concatenate([blk[u][j] for u in range(4)], axis=0) for j in range(4)]
            for j in range(4):
                o = _dot(_unpack(vt_r[16 * j:16 * j + 16, 128 * t:128 * t + 128]), _unpack(ts[j]))
                st[i, 'o', j] = o if t == 0 else st[i, 'o', j] + o

        def fin(i):
            ls = _unskew([jnp.sum(st.pop((i, 'l', be)), axis=0, keepdims=True) for be in range(4)])
            parts = []
            for j in range(4):
                gt = gate_ref[pl.ds(4 * g + j, 1), :]
                omg = gate_ref[pl.ds(32 + 4 * g + j, 1), :]
                o = st.pop((i, 'o', j)) * (omg / ls[j])
                if j > 0:
                    o = pltpu.roll(o, 128 - 32 * j, 1)
                if use_mem:
                    den = nd_ref[128 + j:129 + j, 128 * i:128 * i + 128] + 1e-6
                    o = o + nd_ref[32 * j:32 * j + 32, 128 * i:128 * i + 128] * (gt / den)
                parts.append(o)
            ot = jnp.concatenate(parts, axis=0)
            o_r.bitcast(bf16)[g // 2, 128 * i:128 * i + 128, 128 * par:128 * par + 128] = ot.T.astype(bf16)

        def ex(kind, i, t, tok):
            if kind in 'ep':
                pr(i, t, tok)
            if kind in 'ev':
                pv(i, t)
                if t == i:
                    fin(i)
        return nd, upd, qk, mx, ex

    def ln1(seg, r, tok=None):
        r0 = pl.multiple_of(r * SUB, SUB)
        x = x_ref[seg, pl.ds(r0, SUB), :].astype(f32)
        if tok is not None:
            x = jnp.concatenate([after(x[:, 0:128], tok, CFG['xfrac']), x[:, 128:]], axis=1)
        xn = _ln(x).astype(bf16)
        if seg < 2:
            xa_b[seg, pl.ds(r0, SUB), :] = xn
        if seg > 0:
            xb_b[seg - 1, pl.ds(r0, SUB), :] = xn

    def oproj(seg, r0, rows, n, o_r, k0=0, k1=NG):
        h0 = pl.multiple_of(r0 // 2, rows // 2)
        r0 = pl.multiple_of(r0, rows)
        lhs = _unpack(jnp.concatenate([o_r[p, pl.ds(h0, rows // 2), :] for p in range(k0 // 2, k1 // 2)], axis=1))
        y = _dot(lhs, _unpack(wo_u[n, 64 * k0:64 * k1, :]))
        cols = slice(128 * n, 128 * n + 128)
        if k0 > 0:
            y = y + x1_ref[seg, pl.ds(r0, rows), cols]
        if k1 == NG:
            y = _rb(x_ref[seg, pl.ds(r0, rows), cols].astype(f32) + y)
        x1_ref[seg, pl.ds(r0, rows), cols] = y
        return y

    def ln2(seg, c, t, tok=None):
        r0 = pl.multiple_of(c * CH + t * SUB, SUB)
        lane = lax.broadcasted_iota(i32, (SUB, 128), 1)
        x1 = x1_ref[seg, pl.ds(r0, SUB), :]
        if tok is not None and CFG['pace2']:
            x1 = jnp.concatenate([after(x1[:, 0:128], tok, CFG['xfrac']), x1[:, 128:]], axis=1)
        xn2 = _ln(x1, CFG['lnmode'])
        r = _rb(jnp.sum(xn2 * wrf_ref[...], axis=-1, keepdims=True))
        r_ref[SUB * t:SUB * t + SUB, :] = jnp.where(lane == seg * NG + c, r, r_ref[SUB * t:SUB * t + SUB, :])
        x_ref[seg, pl.ds(r0, SUB), :] = (x1 + xn2).astype(bf16)

    def group(s, g, par, last=False):
        nd, upd, qk, mx, ex = attn_items(g, par, o_refs[s % 2], s > 0)
        fill = []
        extra = []
        if s > 0:
            for n in range(NG):
                fill.append((128, lambda n=n: oproj(s - 1, g * CH, CH, n, o_refs[(s - 1) % 2])))
            extra = [lambda tok, t=t: ln2(s - 1, g, t, tok) for t in range(CH // SUB)]
        else:
            extra = [lambda tok, seg=seg, t=t: ln1(seg, g * (CH // SUB) + t, tok)
                     for seg in range(2, NSEG) for t in range(CH // SUB)]
        if not last:
            gn = g + 1
            pj = proj_items(s, gn // NG, gn % NG, 1 - par)
            for m, n in PORDER:
                for h in range(2):
                    fill.append((128, lambda m=m, n=n, h=h: pj(m, n, h)))
        else:
            for m in range(4):
                for n in range(NG):
                    fill.append((128, lambda m=m, n=n: oproj(s, 128 * m, 128, n, o_refs[s % 2], 0, 4)))
        sched = CFG['sched0' if s == 0 else 'schedL' if last else 'sched'].split()
        y = None
        for tok in sched:
            if tok == 'f':
                y = fill.pop(0)[1]()
            elif tok == 'F':
                while fill:
                    fill.pop(0)[1]()
            elif tok == 'x':
                extra.pop(0)(y)
            elif tok == 'n':
                nd()
            elif tok == 'u':
                if s < NSEG - 1:
                    upd()
            elif tok[0] == 'q':
                qk(int(tok[1]))
            elif tok[0] == 'Q':
                nxt = attn_items(None, 1 - par, None, None)
                nxt[2](int(tok[1]))
                nxt[3](int(tok[1]), 'store')
            elif tok[0] == 'M':
                mx(int(tok[1]), 'load')
            elif tok[0] == 'm':
                mx(int(tok[1]))
            else:
                ex(tok[0], int(tok[1]), int(tok[2]), y)
        for it in fill:
            it[1]()
        for e in extra:
            e(None)

    for c in range(4):
        cp_x0(c).start()
    for j in range(3):
        cp_w(0, j).start()
    cp_x1().start()
    for cp in cp_small():
        cp.start()

    z_ref[...] = jnp.zeros((8, 128), u32)
    ones = jnp.full((8, 512), 0x3F803F80, u32)
    vt0[64:72, :] = ones
    vt1[64:72, :] = ones
    bias_ref[...] = jnp.where(lax.broadcasted_iota(i32, (32, 128), 0)
                              <= (lax.broadcasted_iota(i32, (32, 128), 1) & 31), 0.0, NEG)

    def ln0_body(c, carry):
        cp_x0(c).wait()
        for t in range(128 // SUB):
            ln1(0, c * (128 // SUB) + t)
        return carry
    lax.fori_loop(0, 4, ln0_body, 0)
    for g in range(1, NG):
        for j in range(3):
            cp_w(g, j).start()
        cp_xr(g - 1).start()
    cp_xr(NG - 1).start()
    for cp in cp_wo():
        cp.start()

    for cp in cp_small():
        cp.wait()
    wrf_ref[...] = wr_ref[...].astype(f32)
    gl = _rb(jax.nn.sigmoid(beta_ref[...].astype(f32)))
    hr = lax.broadcasted_iota(i32, (32, 32), 0)
    hc = lax.broadcasted_iota(i32, (32, 32), 1)
    gcol = jnp.sum(jnp.where(hr == hc, gl, 0.0), axis=1, keepdims=True)
    gate_ref[0:32, :] = jnp.broadcast_to(gcol, (32, 128))
    gate_ref[32:64, :] = jnp.broadcast_to(_rb(1.0 - gcol), (32, 128))
    for j in range(2):
        cp_w(0, j).wait()
    if CFG['prewait']:
        for g in range(NG):
            cp_xr(g).wait()
            for j in range(3 * (g > 0)):
                cp_w(g, j).wait()

    def layer(li, carry):
        first = li == 0
        r_ref[...] = jnp.full((CH, 128), -jnp.inf, f32)
        pj = proj_items(0, 0, 0, 0)
        fill = [(m, n, h) for m, n in PORDER for h in range(2)]
        extra = list(range(L // SUB))
        y = None
        for tok in CFG['pre'].split():
            if tok == 'f':
                y = pj(*fill.pop(0))
            elif tok == 'x':
                ln1(1, extra.pop(0), y)
            elif tok == 'w':
                @pl.when(first)
                def _():
                    cp_w(0, 2).wait()
                    cp_x1().wait()
                y = None
            else:
                nxt = attn_items(None, 0, None, None)
                nxt[2](int(tok[1]))
                nxt[3](int(tok[1]), 'store')
        assert not fill and not extra

        for s in range(NSEG):
            def pair(p, c2, s=s, last=False):
                if s == 0 and not CFG['prewait']:
                    @pl.when(first)
                    def _():
                        for par in range(2):
                            g = 2 * p + par
                            cp_xr(g).wait()

                            @pl.when(g + 1 < NG)
                            def _():
                                gn = jnp.minimum(g + 1, NG - 1)
                                for j in range(3):
                                    cp_w(gn, j).wait()
                for par in range(2):
                    group(s, 2 * p + par, par, last and par == 1)
                return c2

            if s == 1:
                @pl.when(first)
                def _():
                    for cp in cp_wo():
                        cp.wait()
                    for cp in cp_ff():
                        cp.start()
            if s >= 2:
                @pl.when(li == CFG['nl'] - 1)
                def _():
                    cp_out_seg(s - 2).start()
            if s in (1, 2) and CFG['gp'] > 2:
                np_ = CFG['gp'] // 2

                def multi(p, c2, pair=pair):
                    for u in range(np_):
                        pair(np_ * p + u, c2)
                    return c2
                if np_ == NG // 2 and not CFG['rep']:
                    multi(0, 0)
                else:
                    _loop('s%d' % s, NG // 2 // np_, multi)
            elif s < NSEG - 1:
                _loop('s%d' % s, NG // 2, pair)
            else:
                _loop('s%d' % s, NG // 2 - 1, pair)
                pair(NG // 2 - 1, 0, last=True)

        s = NSEG - 1
        pend = []
        for m in (3, 2, 1, 0):
            for n in range(NG):
                oproj(s, 128 * m, 128, n, o_refs[s % 2], 4, NG)
                if pend:
                    pend.pop(0)()
            pend = [lambda c=c, t=t: ln2(s, c, t) for c in (2 * m, 2 * m + 1) for t in range(CH // SUB)]
        for e in pend:
            e()

        @pl.when(li == CFG['nl'] - 1)
        def _():
            cp_out_seg(NSEG - 2).start()
            cp_out_seg(NSEG - 1).start()

        rm = r_ref[...]
        idx = (lax.broadcasted_iota(i32, (CH, 128), 1) * CH + lax.broadcasted_iota(i32, (CH, 128), 0)).astype(f32)
        big = float(S)
        m1 = jnp.max(rm, axis=(0, 1), keepdims=True)
        i1 = jnp.min(jnp.where(rm == m1, idx, big), axis=(0, 1), keepdims=True)
        rm2 = jnp.where(idx == i1, -jnp.inf, rm)
        m2 = jnp.max(rm2, axis=(0, 1), keepdims=True)
        i2 = jnp.min(jnp.where(jnp.logical_and(rm2 == m2, idx != i1), idx, big), axis=(0, 1), keepdims=True)
        toks = [jnp.clip(jnp.max(iv).astype(i32), 0, S - 1) for iv in (i1, i2)]

        @pl.when(first)
        def _():
            for cp in cp_ff():
                cp.wait()

        row = lax.broadcasted_iota(i32, (SUB, D), 0)
        x1s = jnp.where(row == 0, x1_ref[toks[0] // L, pl.ds(toks[0] % L, 1), :],
                        jnp.where(row == 1, x1_ref[toks[1] // L, pl.ds(toks[1] % L, 1), :], 0.0))
        xs = _ln(x1s, 2 * CFG['lnmode']).astype(bf16)
        hs = []
        for c in range(NF):
            ga = _rb(_dot(xs, _unpack(wg_u[c])))
            up = _rb(_dot(xs, _unpack(wu_u[c])))
            hs.append((_rb(ga * _rb(jax.nn.sigmoid(ga))) * up).astype(bf16))
            ln1(0, c)
        hdn = jnp.concatenate(hs, axis=1)
        ys = []
        for c in range(NG):
            ys.append(_dot(hdn, _unpack(wd_u[c])))
            if NF + c < L // SUB:
                ln1(0, NF + c)
        y = _rb(jnp.concatenate(ys, axis=1))
        rsel = jnp.where(lax.broadcasted_iota(i32, (SUB, 1), 0) == 0, m1, m2)
        y = _rb(y * _rb(jax.nn.sigmoid(rsel)))
        x2s = _rb(x1s + _rb(xs.astype(f32) + y))
        xns = _ln(x2s)

        @pl.when(li == CFG['nl'] - 1)
        def _():
            for s in range(NSEG):
                cp_out_seg(s).wait()

        blks = []
        for n, t in enumerate(toks):
            sg = t // L
            b0 = pl.multiple_of((t % L) // SUB * SUB, SUB)
            hb = pl.multiple_of((t % L) // SUB * (SUB // 2), SUB // 2)
            hit = row == (t % SUB)
            old = x_ref[sg, pl.ds(b0, SUB), :].astype(f32)
            x_ref[sg, pl.ds(b0, SUB), :] = jnp.where(hit, x2s[n:n + 1], old).astype(bf16)
            oldn = _unpack(xa_ref[0, pl.ds(hb, SUB // 2), :]).astype(f32)
            xa_ref[0, pl.ds(hb, SUB // 2), :] = _pack(jnp.where(row == t - b0, xns[n:n + 1], oldn))
            blks.append((sg, b0))

        @pl.when(li == CFG['nl'] - 1)
        def _():
            def cp_fix(n):
                sg, b0 = blks[n]
                return pltpu.make_async_copy(x_ref.at[sg, pl.ds(b0, SUB), :],
                                             out_hbm.at[sg, pl.ds(b0, SUB), :], sems.at[SEM_FIX + n])
            differ = (toks[0] // SUB) != (toks[1] // SUB)
            cp_fix(0).start()

            @pl.when(differ)
            def _():
                cp_fix(1).start()
                cp_fix(1).wait()
            cp_fix(0).wait()
        return carry

    lax.fori_loop(0, CFG['nl'], layer, 0)


@jax.jit
def pallas_interleave_layers__memory_aug_infini_attn__moe_arch_mod__prompt_kernel(
    A_x: jax.Array,
    A_wq: jax.Array,
    A_wk: jax.Array,
    A_wv: jax.Array,
    A_wo: jax.Array,
    A_beta: jax.Array,
    B_x: jax.Array,
    B_w_r: jax.Array,
    B_w_gate: jax.Array,
    B_w_up: jax.Array,
    B_w_down: jax.Array,
):
    del B_x
    qkv_bufs = [pltpu.VMEM((L // 2, 512), u32), pltpu.VMEM((72, L), u32)]
    scratch = [
        pltpu.VMEM((NSEG, L, D), bf16),
        pltpu.VMEM((CFG['nb'], L // 2, D), u32),
        pltpu.VMEM((NSEG, L, D), f32),
        pltpu.VMEM((3 * NG, D, 128), bf16),
        pltpu.VMEM((NG, D, 128), bf16),
        pltpu.VMEM((NF, D, 128), bf16),
        pltpu.VMEM((NF, D, 128), bf16),
        pltpu.VMEM((NG, F, 128), bf16),
        pltpu.VMEM((1, 32), bf16),
        pltpu.VMEM((1, D), bf16),
        pltpu.VMEM((1, D), f32),
        pltpu.VMEM((64, 128), f32),
        pltpu.VMEM((32, 128), f32),
        pltpu.VMEM((NG, 144, 128), f32),
        pltpu.VMEM((CH, 128), f32),
        pltpu.VMEM((144, L), f32),
        pltpu.VMEM((128, L), f32), pltpu.VMEM((256, L), f32),
        pltpu.VMEM((384, L), f32), pltpu.VMEM((512, L), f32),
        pltpu.VMEM((64, L), u32), pltpu.VMEM((128, L), u32),
        pltpu.VMEM((192, L), u32), pltpu.VMEM((256, L), u32),
        pltpu.VMEM((16, 128), f32),
        pltpu.VMEM((8, 128), u32),
        *qkv_bufs, *qkv_bufs,
        pltpu.VMEM((NG // 2, L // 2, 256), u32),
        pltpu.VMEM((NG // 2, L // 2, 256), u32),
        pltpu.VMEM((2, L // 2, D), u32),
        pltpu.SemaphoreType.DMA((NSEM,)),
    ]
    out = pl.pallas_call(
        _kernel,
        out_shape=jax.ShapeDtypeStruct((NSEG, L, D), bf16),
        in_specs=[pl.BlockSpec(memory_space=pl.ANY)] * 10,
        out_specs=pl.BlockSpec(memory_space=pl.ANY),
        scratch_shapes=scratch,
        compiler_params=pltpu.CompilerParams(vmem_limit_bytes=100 * 2 ** 20),
    )(A_x.reshape(NSEG, L, D), A_wq, A_wk, A_wv, A_wo, A_beta.reshape(1, 32), B_w_r.reshape(1, D),
      B_w_gate, B_w_up, B_w_down)
    return out.reshape(1, S, D)
```

```python
import jax
import jax.numpy as jnp
from jax import lax
import jax.experimental.pallas as pl
import jax.experimental.pallas.tpu as pltpu

bf16 = jnp.bfloat16
f32 = jnp.float32
u32 = jnp.uint32
i32 = jnp.int32

S = 2048
D = 1024
L = 512
NSEG = 4
NG = 8
F = 3584
CH = 64
SUB = 16
NEG = -1e30
QSCALE = (32 ** -0.5) * 1.4426950408889634
NT = (((1,), (1,)), ((), ()))

SEM_X0 = 0
SEM_XR = 1
SEM_W = 9
SEM_WO = 33
SEM_SM = 34
SEM_FF = 36
SEM_OUT = 39
SEM_FIX = 43
SEM_X1 = 45
SEM_XC = 46
SEM_XN = 50
NSEM = 51
NF = F // 128
PORDER = [(m, n) for m in range(4) for n in range(2)] + [(m, 2) for m in range(4)]

CFG = dict(
    rep={}, lnmode=0, nl=2, prewait=False, gp=2, pace=True, pace2=True, one=True, reload=True, chain=True, xfrac=0.0,
    pre='f ' * 16 + 'w x x x x Q3 ' + 'f x x x x ' * 7 + 'f',
    sched='M3 f p30 f n q2 v30 p31 f f v31 p32 f f m2 v32 p33 f f v33 p20 f f q1 v20 p21 f x f v21 p22 f x f '
          'm1 v22 p10 f x f q0 v10 p11 f x f u v11 m0 f p00 f f v00 F Q3',
    sched0='M3 f p30 f q2 v30 p31 f f v31 p32 f f x m2 v32 p33 f f x v33 p20 f f x q1 v20 p21 f f x '
           'v21 p22 f f x m1 v22 p10 f f x q0 v10 p11 f x f u v11 m0 f x p00 f f v00 F Q3',
    schedL='M3 f p30 f n q2 v30 p31 f f v31 p32 f f m2 v32 p33 f f v33 p20 f f q1 v20 p21 f x f v21 p22 f x f '
          'm1 v22 p10 f x f q0 v10 p11 f x f v11 m0 f p00 f f v00 F',
)


def _loop(name, n, body):
    rep = CFG['rep'].get(name, 1)
    if rep == 1:
        return lax.fori_loop(0, n, body, 0)
    return lax.fori_loop(0, n * rep, lambda i, c: body(i // rep, c), 0)


def _rb(x):
    return x.astype(bf16).astype(f32)


def _pack(x):
    return pltpu.bitcast(x.astype(bf16), u32)


def _unpack(u):
    return pltpu.bitcast(u, bf16)


def _phi(t):
    return jnp.where(t > 0, t + 1.0, jnp.exp(t))


def _dot(a, b):
    return jnp.dot(a, b, preferred_element_type=f32)


def _unskew(ps):
    shape, dt = next((p.shape, p.dtype) for p in ps if p is not None)
    c = lax.broadcasted_iota(i32, shape, 1) >> 5
    even = (c & 1) == 0
    lo = c < 2
    mid = jnp.logical_or(c == 1, c == 2)

    def sel(mask, a, b):
        if a is None and b is None:
            return None
        z = jnp.zeros(shape, dt)
        return jnp.where(mask, z if a is None else a, z if b is None else b)
    x0, x1 = sel(even, ps[0], ps[1]), sel(even, ps[1], ps[0])
    x2, x3 = sel(even, ps[2], ps[3]), sel(even, ps[3], ps[2])
    return [sel(lo, x0, x2), sel(mid, x1, x3), sel(lo, x2, x0), sel(mid, x3, x1)]


def _ln(x, mode=0):
    acc = x
    if CFG['chain']:
        acc = x[:, 0:128]
        for c in range(1, x.shape[1] // 128):
            acc = acc + x[:, 128 * c:128 * c + 128]
    m = jnp.sum(acc, axis=-1, keepdims=True) * (1.0 / D)
    if mode == 0:
        e = x - m
        v = jnp.sum(e * e, axis=-1, keepdims=True) * (1.0 / D)
        return e * lax.rsqrt(v + 1e-5)
    c = _rb(m)
    e = x - c
    v = jnp.sum(e * e, axis=-1, keepdims=True) * (1.0 / D) - (m - c) * (m - c)
    w = _rb(_rb(jnp.maximum(v, 0.0)) + 1e-5)
    den = _rb(w * lax.rsqrt(w))
    if mode == 2:
        return _rb(_rb(e) / den)
    return e * (1.0 / den)


def _rowsum(x, first=None):
    acc = x[:, 0:128] if first is None else first
    for c in range(1, x.shape[1] // 128):
        acc = acc + x[:, 128 * c:128 * c + 128]
    return jnp.sum(acc, axis=-1, keepdims=True)


def _stats(x):
    m = _rowsum(x) * (1.0 / D)
    v = jnp.maximum(_rowsum(x * x) * (1.0 / D) - m * m, 0.0)
    return m, lax.rsqrt(v + 1e-5)


def _kernel(x_hbm, wq_hbm, wk_hbm, wv_hbm, wo_hbm, beta_hbm, wr_hbm, wg_hbm, wu_hbm, wd_hbm,
            out_hbm,
            x_ref, xb_ref, x1_ref, w_ref, wo_ref, wg_ref, wu_ref, wd_ref,
            gate_ref, bias_ref, m_ref, r_ref, nd_ref,
            s0_ref, s1_ref, s2_ref, s3_ref, p0_ref, p1_ref, p2_ref, p3_ref,
            qk0, vt0, qk1, vt1, oa_ref, ob_ref, xa_ref, mx_ref, z_ref, wrf_ref, wr_ref, beta_ref, sems):
    qkv = ((qk0, vt0), (qk1, vt1))
    o_refs = (oa_ref, ob_ref)
    s_refs = (s0_ref, s1_ref, s2_ref, s3_ref)
    p_refs = (p0_ref, p1_ref, p2_ref, p3_ref)
    xa_b, xb_b = xa_ref.bitcast(bf16), xb_ref.bitcast(bf16)
    w_u, wo_u, wg_u, wu_u, wd_u = (r.bitcast(u32) for r in (w_ref, wo_ref, wg_ref, wu_ref, wd_ref))

    def cp_x0(c):
        rows = pl.ds(pl.multiple_of(128 * c, 128), 128)
        return pltpu.make_async_copy(x_hbm.at[0, rows], x_ref.at[0, rows], sems.at[SEM_XC + c])

    def cp_x1():
        return pltpu.make_async_copy(x_hbm.at[1], x_ref.at[1], sems.at[SEM_X1])

    def cp_xn():
        return pltpu.make_async_copy(xa_ref.at[L // 2:L], xb_ref.at[0:L // 2], sems.at[SEM_XN])

    def cp_xr(g):
        r0 = pl.multiple_of(g * CH, CH)
        return pltpu.make_async_copy(x_hbm.at[2:NSEG, pl.ds(r0, CH), :],
                                     x_ref.at[2:NSEG, pl.ds(r0, CH), :], sems.at[SEM_XR + g])

    def cp_w(g, j):
        c0 = pl.multiple_of(g * 128, 128)
        src = (wq_hbm, wk_hbm, wv_hbm)[j]
        return pltpu.make_async_copy(src.at[:, pl.ds(c0, 128)], w_ref.at[3 * g + j], sems.at[SEM_W + 3 * g + j])

    def slabs(src, dst, n, sem):
        return [pltpu.make_async_copy(src.at[:, 128 * c:128 * c + 128], dst.at[c], sems.at[sem]) for c in range(n)]

    def cp_wo():
        return slabs(wo_hbm, wo_ref, NG, SEM_WO)

    def cp_small():
        return (pltpu.make_async_copy(beta_hbm, beta_ref, sems.at[SEM_SM]),
                pltpu.make_async_copy(wr_hbm, wr_ref, sems.at[SEM_SM + 1]))

    def cp_ff():
        return (slabs(wg_hbm, wg_ref, NF, SEM_FF) + slabs(wu_hbm, wu_ref, NF, SEM_FF + 1)
                + slabs(wd_hbm, wd_ref, NG, SEM_FF + 2))

    def cp_out_seg(s):
        return pltpu.make_async_copy(x_ref.at[s], out_hbm.at[s], sems.at[SEM_OUT + s])

    def after(x, tok, frac):
        if tok is None or not CFG['pace']:
            return x
        r = 8 * int(frac * tok.shape[0] // 8)
        t = pltpu.bitcast(tok[r:r + 8, 0:128], u32) & z_ref[...]
        t = jnp.tile(t, (x.shape[0] // 8, x.shape[1] // 128))
        return pltpu.bitcast(pltpu.bitcast(x, u32) | t, x.dtype)

    def proj_items(s, nxt, g, par):
        xn_r, seg = (xa_ref, nxt) if s == 0 else (xb_ref, s - 1 + nxt)
        qk_r, vt_r = (r.bitcast(bf16) for r in qkv[par])
        part = {}

        def item(m, n, h):
            xn = _unpack(xn_r[pl.ds(pl.multiple_of(seg * (L // 2) + 64 * m, 64), 64), 512 * h:512 * h + 512])
            y = _dot(xn, _unpack(w_u[3 * g + n, 256 * h:256 * h + 256, :]))
            if h == 0:
                part[m, n] = y
                return y
            y = y + part.pop((m, n))
            rows = slice(128 * m, 128 * m + 128)
            if n == 0:
                qk_r[rows, 0:128] = (y * QSCALE).astype(bf16)
                qk_r[rows, 128:256] = _phi(y).astype(bf16)
            elif n == 1:
                qk_r[rows, 256:384] = y.astype(bf16)
                qk_r[rows, 384:512] = _phi(y).astype(bf16)
            else:
                vt_r[0:128, rows] = y.T.astype(bf16)
            return y
        return item

    def attn_items(g, par, o_r, use_mem):
        qk_r, vt_r = qkv[par]
        st = {}

        def nd():
            ml = m_ref[g].astype(bf16)
            nd_ref[...] = lax.dot_general(ml, _unpack(qk_r[:, 128:256]), NT, preferred_element_type=f32)

        def upd():
            u = _dot(_unpack(vt_r[...]), _unpack(qk_r[:, 384:512]))
            r2 = lax.broadcasted_iota(i32, (144, 128), 0)
            c2 = lax.broadcasted_iota(i32, (144, 128), 1) >> 5
            keep = jnp.where(r2 < 128, r2 >> 5, r2 - 128) == c2
            u = jnp.where(keep, u, 0.0)
            m_ref[g] = (m_ref[g] + u) if use_mem else u

        def qk(i):
            lane = lax.broadcasted_iota(i32, (16, 128), 1) >> 5
            for be in (range(4) if i % 2 else range(3, -1, -1)):
                b = 4 * i + be
                n = 32 * (b + 1)
                qu = qk_r[16 * b:16 * b + 16, 0:128]
                wq = _unpack(jnp.concatenate(
                    [jnp.where(lane == (c - be) % 4, qu, jnp.uint32(0)) for c in range(4)], axis=0))
                s = lax.dot_general(_unpack(qk_r[0:n // 2, 256:384]), wq, NT, preferred_element_type=f32)
                cols = slice(128 * be, 128 * be + 128)
                if b > 0:
                    s_refs[i][0:n - 32, cols] = s[0:n - 32]
                s_refs[i][n - 32:n, cols] = s[n - 32:n] + bias_ref[...]

        def mx(i, mode='m'):
            for be in range(4):
                if mode == 'load':
                    st[i, 'm', be] = mx_ref[4 * i + be:4 * i + be + 1, :]
                    continue
                n = 32 * (4 * i + be + 1)
                sv = s_refs[i][0:n, 128 * be:128 * be + 128]
                m = jnp.max(jnp.max(sv.reshape(n // 8, 8, 128), axis=0), axis=0, keepdims=True)
                if mode == 'store':
                    mx_ref[4 * i + be:4 * i + be + 1, :] = m
                else:
                    st[i, 'm', be] = m

        def pr(i, t, tok):
            ps = []
            for be in range(4):
                n = 128 if t < i else 32 * (be + 1)
                m8 = after(jnp.broadcast_to(st[i, 'm', be], (8, 128)), tok, be / 4)
                p = jnp.exp2(s_refs[i][128 * t:128 * t + n, 128 * be:128 * be + 128].reshape(n // 8, 8, 128) - m8)
                ls = jnp.sum(p, axis=0)
                p = p.reshape(n, 128)
                st[i, 'l', be] = ls if t == 0 else st[i, 'l', be] + ls
                p_refs[i].bitcast(bf16)[128 * t:128 * t + n, 128 * be:128 * be + 128] = p.astype(bf16)

        def pv(i, t):
            ps = [p_refs[i][64 * t:64 * t + (64 if t < i else 16 * (be + 1)), 128 * be:128 * be + 128]
                  for be in range(4)]
            if t < i:
                ts = _unskew(ps)
            else:
                blk = [_unskew([ps[be][16 * u:16 * u + 16] if be >= u else None for be in range(4)])
                       for u in range(4)]
                ts = [jnp.concatenate([blk[u][j] for u in range(4)], axis=0) for j in range(4)]
            for j in range(4):
                o = _dot(_unpack(vt_r[16 * j:16 * j + 16, 128 * t:128 * t + 128]), _unpack(ts[j]))
                st[i, 'o', j] = o if t == 0 else st[i, 'o', j] + o

        def fin(i):
            ls = _unskew([jnp.sum(st.pop((i, 'l', be)), axis=0, keepdims=True) for be in range(4)])
            parts = []
            for j in range(4):
                gt = gate_ref[pl.ds(4 * g + j, 1), :]
                omg = gate_ref[pl.ds(32 + 4 * g + j, 1), :]
                o = st.pop((i, 'o', j)) * (omg / ls[j])
                if j > 0:
                    o = pltpu.roll(o, 128 - 32 * j, 1)
                if use_mem:
                    den = nd_ref[128 + j:129 + j, 128 * i:128 * i + 128] + 1e-6
                    o = o + nd_ref[32 * j:32 * j + 32, 128 * i:128 * i + 128] * (gt / den)
                parts.append(o)
            ot = jnp.concatenate(parts, axis=0)
            o_r.bitcast(bf16)[pl.ds(pl.multiple_of(g // 2 * L + 128 * i, 128), 128),
                              128 * par:128 * par + 128] = ot.T.astype(bf16)

        def ex(kind, i, t, tok):
            if kind in 'ep':
                pr(i, t, tok)
            if kind in 'ev':
                pv(i, t)
                if t == i:
                    fin(i)
        return nd, upd, qk, mx, ex

    def ln1(seg, r, tok=None):
        r0 = pl.multiple_of(r * SUB, SUB)
        x = x_ref[seg, pl.ds(r0, SUB), :].astype(f32)
        if tok is not None:
            x = jnp.concatenate([after(x[:, 0:128], tok, CFG['xfrac']), x[:, 128:]], axis=1)
        if CFG['one']:
            m, rs = _stats(x)
            if CFG['reload']:
                mx_ref[16:24, :] = jnp.broadcast_to(m[0:8], (8, 128))
                x = x_ref[seg, pl.ds(r0, SUB), :].astype(f32)
            xn = ((x - m) * rs).astype(bf16)
        else:
            xn = _ln(x).astype(bf16)
        if seg < 2:
            xa_b[pl.ds(pl.multiple_of(seg * L + r0, SUB), SUB), :] = xn
        else:
            xb_b[pl.ds(pl.multiple_of((seg - 1) * L + r0, SUB), SUB), :] = xn

    def oproj(seg, r0, rows, n, o_r, k0=0, k1=NG):
        h0 = pl.multiple_of(r0 // 2, rows // 2)
        r0 = pl.multiple_of(r0, rows)
        lhs = _unpack(jnp.concatenate([o_r[pl.ds(pl.multiple_of(p * (L // 2) + h0, rows // 2), rows // 2), :]
                                       for p in range(k0 // 2, k1 // 2)], axis=1))
        y = _dot(lhs, _unpack(wo_u[n, 64 * k0:64 * k1, :]))
        cols = slice(128 * n, 128 * n + 128)
        if k0 > 0:
            y = y + x1_ref[seg, pl.ds(r0, rows), cols]
        if k1 == NG:
            y = _rb(x_ref[seg, pl.ds(r0, rows), cols].astype(f32) + y)
        x1_ref[seg, pl.ds(r0, rows), cols] = y
        return y

    def ln2(seg, c, t, tok=None):
        r0 = pl.multiple_of(c * CH + t * SUB, SUB)
        lane = lax.broadcasted_iota(i32, (SUB, 128), 1)
        x1 = x1_ref[seg, pl.ds(r0, SUB), :]
        if tok is not None and CFG['pace2']:
            x1 = jnp.concatenate([after(x1[:, 0:128], tok, CFG['xfrac']), x1[:, 128:]], axis=1)
        if CFG['one']:
            m, rs = _stats(x1)
            r = _rb((_rowsum(x1 * wrf_ref[0:1, :]) - m * wrf_ref[1:2, 0:128]) * rs)
        else:
            xn2 = _ln(x1, CFG['lnmode'])
            r = _rb(jnp.sum(xn2 * wrf_ref[0:1, :], axis=-1, keepdims=True))
        r_ref[SUB * t:SUB * t + SUB, :] = jnp.where(lane == seg * NG + c, r, r_ref[SUB * t:SUB * t + SUB, :])
        if CFG['one']:
            if CFG['reload']:
                x1 = x1_ref[seg, pl.ds(r0, SUB), :]
            x2 = x1 * (1.0 + rs) - m * rs
        else:
            x2 = x1 + xn2
        x_ref[seg, pl.ds(r0, SUB), :] = x2.astype(bf16)

    def group(s, g, par, last=False):
        nd, upd, qk, mx, ex = attn_items(g, par, o_refs[s % 2], s > 0)
        fill = []
        extra = []
        if s > 0:
            for n in range(NG):
                fill.append((128, lambda n=n: oproj(s - 1, g * CH, CH, n, o_refs[(s - 1) % 2])))
            extra = [lambda tok, t=t: ln2(s - 1, g, t, tok) for t in range(CH // SUB)]
        else:
            extra = [lambda tok, seg=seg, t=t: ln1(seg, g * (CH // SUB) + t, tok)
                     for seg in range(2, NSEG) for t in range(CH // SUB)]
        if not last:
            gn = g + 1
            pj = proj_items(s, gn // NG, gn % NG, 1 - par)
            for m, n in PORDER:
                for h in range(2):
                    fill.append((128, lambda m=m, n=n, h=h: pj(m, n, h)))
        else:
            for m in range(4):
                for n in range(NG):
                    fill.append((128, lambda m=m, n=n: oproj(s, 128 * m, 128, n, o_refs[s % 2], 0, 4)))
        sched = CFG['sched0' if s == 0 else 'schedL' if last else 'sched'].split()
        y = None
        for tok in sched:
            if tok == 'f':
                y = fill.pop(0)[1]()
            elif tok == 'F':
                while fill:
                    fill.pop(0)[1]()
            elif tok == 'x':
                extra.pop(0)(y)
            elif tok == 'n':
                nd()
            elif tok == 'u':
                if s < NSEG - 1:
                    upd()
            elif tok[0] == 'q':
                qk(int(tok[1]))
            elif tok[0] == 'Q':
                nxt = attn_items(None, 1 - par, None, None)
                nxt[2](int(tok[1]))
                nxt[3](int(tok[1]), 'store')
            elif tok[0] == 'M':
                mx(int(tok[1]), 'load')
            elif tok[0] == 'm':
                mx(int(tok[1]))
            else:
                ex(tok[0], int(tok[1]), int(tok[2]), y)
        for it in fill:
            it[1]()
        for e in extra:
            e(None)

    for c in range(4):
        cp_x0(c).start()
    for j in range(3):
        cp_w(0, j).start()
    cp_x1().start()
    for cp in cp_small():
        cp.start()

    z_ref[...] = jnp.zeros((8, 128), u32)
    ones = jnp.full((8, 512), 0x3F803F80, u32)
    vt0[64:72, :] = ones
    vt1[64:72, :] = ones
    bias_ref[...] = jnp.where(lax.broadcasted_iota(i32, (32, 128), 0)
                              <= (lax.broadcasted_iota(i32, (32, 128), 1) & 31), 0.0, NEG)

    def ln0_body(c, carry):
        cp_x0(c).wait()
        for t in range(128 // SUB):
            ln1(0, c * (128 // SUB) + t)
        return carry
    lax.fori_loop(0, 4, ln0_body, 0)
    for g in range(1, NG):
        for j in range(3):
            cp_w(g, j).start()
        cp_xr(g - 1).start()
    cp_xr(NG - 1).start()
    for cp in cp_wo():
        cp.start()

    for cp in cp_small():
        cp.wait()
    wr = wr_ref[...].astype(f32)
    wrf_ref[0:1, :] = wr
    wrf_ref[1:2, :] = jnp.broadcast_to(jnp.sum(wr, axis=-1, keepdims=True), (1, D))
    gl = _rb(jax.nn.sigmoid(beta_ref[...].astype(f32)))
    hr = lax.broadcasted_iota(i32, (32, 32), 0)
    hc = lax.broadcasted_iota(i32, (32, 32), 1)
    gcol = jnp.sum(jnp.where(hr == hc, gl, 0.0), axis=1, keepdims=True)
    gate_ref[0:32, :] = jnp.broadcast_to(gcol, (32, 128))
    gate_ref[32:64, :] = jnp.broadcast_to(_rb(1.0 - gcol), (32, 128))
    for j in range(2):
        cp_w(0, j).wait()
    if CFG['prewait']:
        for g in range(NG):
            cp_xr(g).wait()
            for j in range(3 * (g > 0)):
                cp_w(g, j).wait()

    def layer(li, carry):
        first = li == 0
        r_ref[...] = jnp.full((CH, 128), -jnp.inf, f32)
        pj = proj_items(0, 0, 0, 0)
        fill = [(m, n, h) for m, n in PORDER for h in range(2)]
        extra = list(range(L // SUB))
        y = None
        for tok in CFG['pre'].split():
            if tok == 'f':
                y = pj(*fill.pop(0))
            elif tok == 'x':
                ln1(1, extra.pop(0), y)
            elif tok == 'w':
                @pl.when(first)
                def _():
                    cp_w(0, 2).wait()
                    cp_x1().wait()
                y = None
            else:
                nxt = attn_items(None, 0, None, None)
                nxt[2](int(tok[1]))
                nxt[3](int(tok[1]), 'store')
        assert not fill and not extra
        cp_xn().start()

        for s in range(NSEG):
            def pair(p, c2, s=s, last=False):
                if s == 0 and not CFG['prewait']:
                    @pl.when(first)
                    def _():
                        for par in range(2):
                            g = 2 * p + par
                            cp_xr(g).wait()

                            @pl.when(g + 1 < NG)
                            def _():
                                gn = jnp.minimum(g + 1, NG - 1)
                                for j in range(3):
                                    cp_w(gn, j).wait()
                for par in range(2):
                    group(s, 2 * p + par, par, last and par == 1)
                return c2

            if s == 1:
                cp_xn().wait()

                @pl.when(first)
                def _():
                    for cp in cp_wo():
                        cp.wait()
                    for cp in cp_ff():
                        cp.start()
            if s >= 2:
                @pl.when(li == CFG['nl'] - 1)
                def _():
                    cp_out_seg(s - 2).start()
            if s in (1, 2) and CFG['gp'] > 2:
                np_ = CFG['gp'] // 2

                def multi(p, c2, pair=pair):
                    for u in range(np_):
                        pair(np_ * p + u, c2)
                    return c2
                if np_ == NG // 2 and not CFG['rep']:
                    multi(0, 0)
                else:
                    _loop('s%d' % s, NG // 2 // np_, multi)
            elif s < NSEG - 1:
                _loop('s%d' % s, NG // 2, pair)
            else:
                _loop('s%d' % s, NG // 2 - 1, pair)
                pair(NG // 2 - 1, 0, last=True)

        s = NSEG - 1
        pend = []
        for m in (3, 2, 1, 0):
            for n in range(NG):
                oproj(s, 128 * m, 128, n, o_refs[s % 2], 4, NG)
                if pend:
                    pend.pop(0)()
            pend = [lambda c=c, t=t: ln2(s, c, t) for c in (2 * m, 2 * m + 1) for t in range(CH // SUB)]
        for e in pend:
            e()

        @pl.when(li == CFG['nl'] - 1)
        def _():
            cp_out_seg(NSEG - 2).start()
            cp_out_seg(NSEG - 1).start()

        rm = r_ref[...]
        idx = (lax.broadcasted_iota(i32, (CH, 128), 1) * CH + lax.broadcasted_iota(i32, (CH, 128), 0)).astype(f32)
        big = float(S)
        m1 = jnp.max(rm, axis=(0, 1), keepdims=True)
        i1 = jnp.min(jnp.where(rm == m1, idx, big), axis=(0, 1), keepdims=True)
        rm2 = jnp.where(idx == i1, -jnp.inf, rm)
        m2 = jnp.max(rm2, axis=(0, 1), keepdims=True)
        i2 = jnp.min(jnp.where(jnp.logical_and(rm2 == m2, idx != i1), idx, big), axis=(0, 1), keepdims=True)
        toks = [jnp.clip(jnp.max(iv).astype(i32), 0, S - 1) for iv in (i1, i2)]

        @pl.when(first)
        def _():
            for cp in cp_ff():
                cp.wait()

        row = lax.broadcasted_iota(i32, (SUB, D), 0)
        x1s = jnp.where(row == 0, x1_ref[toks[0] // L, pl.ds(toks[0] % L, 1), :],
                        jnp.where(row == 1, x1_ref[toks[1] // L, pl.ds(toks[1] % L, 1), :], 0.0))
        xs = _ln(x1s, 2 * CFG['lnmode']).astype(bf16)
        hs = []
        for c in range(NF):
            ga = _rb(_dot(xs, _unpack(wg_u[c])))
            up = _rb(_dot(xs, _unpack(wu_u[c])))
            hs.append((_rb(ga * _rb(jax.nn.sigmoid(ga))) * up).astype(bf16))
            ln1(0, c)
        hdn = jnp.concatenate(hs, axis=1)
        ys = []
        for c in range(NG):
            ys.append(_dot(hdn, _unpack(wd_u[c])))
            if NF + c < L // SUB:
                ln1(0, NF + c)
        y = _rb(jnp.concatenate(ys, axis=1))
        rsel = jnp.where(lax.broadcasted_iota(i32, (SUB, 1), 0) == 0, m1, m2)
        y = _rb(y * _rb(jax.nn.sigmoid(rsel)))
        x2s = _rb(x1s + _rb(xs.astype(f32) + y))
        xns = _ln(x2s)

        @pl.when(li == CFG['nl'] - 1)
        def _():
            for s in range(NSEG):
                cp_out_seg(s).wait()

        blks = []
        for n, t in enumerate(toks):
            sg = t // L
            b0 = pl.multiple_of((t % L) // SUB * SUB, SUB)
            hb = pl.multiple_of((t % L) // SUB * (SUB // 2), SUB // 2)
            hit = row == (t % SUB)
            old = x_ref[sg, pl.ds(b0, SUB), :].astype(f32)
            x_ref[sg, pl.ds(b0, SUB), :] = jnp.where(hit, x2s[n:n + 1], old).astype(bf16)
            oldn = _unpack(xa_ref[pl.ds(hb, SUB // 2), :]).astype(f32)
            xa_ref[pl.ds(hb, SUB // 2), :] = _pack(jnp.where(row == t - b0, xns[n:n + 1], oldn))
            blks.append((sg, b0))

        @pl.when(li == CFG['nl'] - 1)
        def _():
            def cp_fix(n):
                sg, b0 = blks[n]
                return pltpu.make_async_copy(x_ref.at[sg, pl.ds(b0, SUB), :],
                                             out_hbm.at[sg, pl.ds(b0, SUB), :], sems.at[SEM_FIX + n])
            differ = (toks[0] // SUB) != (toks[1] // SUB)
            cp_fix(0).start()

            @pl.when(differ)
            def _():
                cp_fix(1).start()
                cp_fix(1).wait()
            cp_fix(0).wait()
        return carry

    lax.fori_loop(0, CFG['nl'], layer, 0)


@jax.jit
def pallas_interleave_layers__memory_aug_infini_attn__moe_arch_mod__prompt_kernel(
    A_x: jax.Array,
    A_wq: jax.Array,
    A_wk: jax.Array,
    A_wv: jax.Array,
    A_wo: jax.Array,
    A_beta: jax.Array,
    B_x: jax.Array,
    B_w_r: jax.Array,
    B_w_gate: jax.Array,
    B_w_up: jax.Array,
    B_w_down: jax.Array,
):
    del B_x
    qkv_bufs = [pltpu.VMEM((L // 2, 512), u32), pltpu.VMEM((72, L), u32)]
    scratch = [
        pltpu.VMEM((NSEG, L, D), bf16),
        pltpu.VMEM((3 * L // 2, D), u32),
        pltpu.VMEM((NSEG, L, D), f32),
        pltpu.VMEM((3 * NG, D, 128), bf16),
        pltpu.VMEM((NG, D, 128), bf16),
        pltpu.VMEM((NF, D, 128), bf16),
        pltpu.VMEM((NF, D, 128), bf16),
        pltpu.VMEM((NG, F, 128), bf16),
        pltpu.VMEM((64, 128), f32),
        pltpu.VMEM((32, 128), f32),
        pltpu.VMEM((NG, 144, 128), f32),
        pltpu.VMEM((CH, 128), f32),
        pltpu.VMEM((144, L), f32),
        pltpu.VMEM((128, L), f32), pltpu.VMEM((256, L), f32),
        pltpu.VMEM((384, L), f32), pltpu.VMEM((512, L), f32),
        pltpu.VMEM((64, L), u32), pltpu.VMEM((128, L), u32),
        pltpu.VMEM((192, L), u32), pltpu.VMEM((256, L), u32),
        *qkv_bufs, *qkv_bufs,
        pltpu.VMEM((NG // 2 * L // 2, 256), u32),
        pltpu.VMEM((NG // 2 * L // 2, 256), u32),
        pltpu.VMEM((L, D), u32),
        pltpu.VMEM((24, 128), f32),
        pltpu.VMEM((8, 128), u32),
        pltpu.VMEM((2, D), f32),
        pltpu.VMEM((1, D), bf16),
        pltpu.VMEM((1, 32), bf16),
        pltpu.SemaphoreType.DMA((NSEM,)),
    ]
    out = pl.pallas_call(
        _kernel,
        out_shape=jax.ShapeDtypeStruct((NSEG, L, D), bf16),
        in_specs=[pl.BlockSpec(memory_space=pl.ANY)] * 10,
        out_specs=pl.BlockSpec(memory_space=pl.ANY),
        scratch_shapes=scratch,
        compiler_params=pltpu.CompilerParams(vmem_limit_bytes=100 * 2 ** 20),
    )(A_x.reshape(NSEG, L, D), A_wq, A_wk, A_wv, A_wo, A_beta.reshape(1, 32), B_w_r.reshape(1, D),
      B_w_gate, B_w_up, B_w_down)
    return out.reshape(1, S, D)
```

```python
import jax
import jax.numpy as jnp
from jax import lax
import jax.experimental.pallas as pl
import jax.experimental.pallas.tpu as pltpu

bf16 = jnp.bfloat16
f32 = jnp.float32
u32 = jnp.uint32
i32 = jnp.int32

S = 2048
D = 1024
L = 512
NSEG = 4
NG = 8
F = 3584
CH = 64
SUB = 16
NEG = -1e30
QSCALE = (32 ** -0.5) * 1.4426950408889634
NT = (((1,), (1,)), ((), ()))

SEM_XC = 0
SEM_W0 = 4
SEM_X1 = 5
SEM_SM = 6
SEM_P = 7
NSEM = 11
SEM_OUT, SEM_FIX, SEM_FF, SEM_XN = 0, 1, 2, 3
NF = F // 128
PORDER = [(m, n) for m in range(4) for n in range(2)] + [(m, 2) for m in range(4)]

CFG = dict(
    rep={}, cnt={}, lnmode=0, nl=2, prewait=False, gp=2, pace=True, pace2=True, one=True, reload=True, chain=True, xfrac=0.0, freload=False, lag=0, fskip=0,
    pre='f ' * 16 + 'w x x x x Q3 ' + 'f x x x x ' * 7 + 'f',
    sched='M3 f p30 f n q2 v30 p31 f f v31 p32 f f m2 v32 p33 f f v33 p20 f f q1 v20 p21 f x f v21 p22 f x f '
          'm1 v22 p10 f x f q0 v10 p11 f x f u v11 m0 f p00 f f v00 F Q3',
    sched0='M3 f p30 f q2 v30 p31 f f v31 p32 f f x m2 v32 p33 f f x v33 p20 f f x q1 v20 p21 f f x '
           'v21 p22 f f x m1 v22 p10 f f x q0 v10 p11 f x f u v11 m0 f x p00 f f v00 F Q3',
    schedL='M3 f p30 f n q2 v30 p31 f f v31 p32 f f m2 v32 p33 f f v33 p20 f f q1 v20 p21 f x f v21 p22 f x f '
          'm1 v22 p10 f x f q0 v10 p11 f x f v11 m0 f p00 f f v00 F',
)


def _loop(name, n, body):
    rep = CFG['rep'].get(name, 1)
    n = CFG['cnt'].get(name, n)
    if n == 0:
        return 0
    if rep == 1:
        return lax.fori_loop(0, n, body, 0)
    return lax.fori_loop(0, n * rep, lambda i, c: body(i // rep, c), 0)


def _rb(x):
    return x.astype(bf16).astype(f32)


def _pack(x):
    return pltpu.bitcast(x.astype(bf16), u32)


def _unpack(u):
    return pltpu.bitcast(u, bf16)


def _phi(t):
    return jnp.where(t > 0, t + 1.0, jnp.exp(t))


def _dot(a, b):
    return jnp.dot(a, b, preferred_element_type=f32)


def _unskew(ps):
    shape, dt = next((p.shape, p.dtype) for p in ps if p is not None)
    c = lax.broadcasted_iota(i32, shape, 1) >> 5
    even = (c & 1) == 0
    lo = c < 2
    mid = jnp.logical_or(c == 1, c == 2)

    def sel(mask, a, b):
        if a is None and b is None:
            return None
        z = jnp.zeros(shape, dt)
        return jnp.where(mask, z if a is None else a, z if b is None else b)
    x0, x1 = sel(even, ps[0], ps[1]), sel(even, ps[1], ps[0])
    x2, x3 = sel(even, ps[2], ps[3]), sel(even, ps[3], ps[2])
    return [sel(lo, x0, x2), sel(mid, x1, x3), sel(lo, x2, x0), sel(mid, x3, x1)]


def _ln(x, mode=0):
    acc = x
    if CFG['chain']:
        acc = x[:, 0:128]
        for c in range(1, x.shape[1] // 128):
            acc = acc + x[:, 128 * c:128 * c + 128]
    m = jnp.sum(acc, axis=-1, keepdims=True) * (1.0 / D)
    if mode == 0:
        e = x - m
        v = jnp.sum(e * e, axis=-1, keepdims=True) * (1.0 / D)
        return e * lax.rsqrt(v + 1e-5)
    c = _rb(m)
    e = x - c
    v = jnp.sum(e * e, axis=-1, keepdims=True) * (1.0 / D) - (m - c) * (m - c)
    w = _rb(_rb(jnp.maximum(v, 0.0)) + 1e-5)
    den = _rb(w * lax.rsqrt(w))
    if mode == 2:
        return _rb(_rb(e) / den)
    return e * (1.0 / den)


def _rowsum(x, first=None):
    acc = x[:, 0:128] if first is None else first
    for c in range(1, x.shape[1] // 128):
        acc = acc + x[:, 128 * c:128 * c + 128]
    return jnp.sum(acc, axis=-1, keepdims=True)


def _stats(x):
    m = _rowsum(x) * (1.0 / D)
    v = jnp.maximum(_rowsum(x * x) * (1.0 / D) - m * m, 0.0)
    return m, lax.rsqrt(v + 1e-5)


def _kernel(x_hbm, wq_hbm, wk_hbm, wv_hbm, wo_hbm, beta_hbm, wr_hbm, wg_hbm, wu_hbm, wd_hbm,
            out_hbm,
            x_ref, xb_ref, x1_ref, w_ref, wo_ref, wg_ref, wu_ref, wd_ref,
            gate_ref, bias_ref, m_ref, r_ref, nd_ref,
            s0_ref, s1_ref, s2_ref, s3_ref, p0_ref, p1_ref, p2_ref, p3_ref,
            qk0, vt0, qk1, vt1, o_ref, xa_ref, mx_ref, z_ref, wrf_ref, wr_ref, beta_ref, sems):
    qkv = ((qk0, vt0), (qk1, vt1))
    s_refs = (s0_ref, s1_ref, s2_ref, s3_ref)
    p_refs = (p0_ref, p1_ref, p2_ref, p3_ref)
    xa_b, xb_b = xa_ref.bitcast(bf16), xb_ref.bitcast(bf16)
    w_u, wo_u, wg_u, wu_u, wd_u = (r.bitcast(u32) for r in (w_ref, wo_ref, wg_ref, wu_ref, wd_ref))

    def cp_x0(c):
        rows = pl.ds(pl.multiple_of(128 * c, 128), 128)
        return pltpu.make_async_copy(x_hbm.at[0, rows], x_ref.at[0, rows], sems.at[SEM_XC + c])

    def cp_x1():
        return pltpu.make_async_copy(x_hbm.at[1], x_ref.at[1], sems.at[SEM_X1])

    def cp_xn():
        return pltpu.make_async_copy(xa_ref.at[L // 2:L], xb_ref.at[0:L // 2], sems.at[SEM_XN])

    def cp_xr(g):
        r0 = pl.multiple_of(g * CH, CH)
        return pltpu.make_async_copy(x_hbm.at[2:NSEG, pl.ds(r0, CH), :],
                                     x_ref.at[2:NSEG, pl.ds(r0, CH), :], sems.at[SEM_P + g // 2])

    def cp_w(g, j):
        c0 = pl.multiple_of(g * 128, 128)
        src = (wq_hbm, wk_hbm, wv_hbm)[j]
        sem = (SEM_W0 + j // 2) if isinstance(g, int) and g == 0 else SEM_P + (g - 1) // 2
        return pltpu.make_async_copy(src.at[:, pl.ds(c0, 128)], w_ref.at[3 * g + j], sems.at[sem])

    def slabs(src, dst, n, sem):
        return [pltpu.make_async_copy(src.at[:, 128 * c:128 * c + 128], dst.at[c], sems.at[sem]) for c in range(n)]

    def cp_wo():
        return slabs(wo_hbm, wo_ref, NG, SEM_P + 3)

    def cp_small():
        return (pltpu.make_async_copy(beta_hbm, beta_ref, sems.at[SEM_SM]),
                pltpu.make_async_copy(wr_hbm, wr_ref, sems.at[SEM_SM]))

    def cp_ff():
        return (slabs(wg_hbm, wg_ref, NF, SEM_FF) + slabs(wu_hbm, wu_ref, NF, SEM_FF)
                + slabs(wd_hbm, wd_ref, NG, SEM_FF))

    def cp_out_seg(s):
        return pltpu.make_async_copy(x_ref.at[s], out_hbm.at[s], sems.at[SEM_OUT])

    def after(x, tok, frac):
        if tok is None or not CFG['pace']:
            return x
        r = 8 * int(frac * tok.shape[0] // 8)
        t = pltpu.bitcast(tok[r:r + 8, 0:128], u32) & z_ref[...]
        t = jnp.tile(t, (x.shape[0] // 8, x.shape[1] // 128))
        return pltpu.bitcast(pltpu.bitcast(x, u32) | t, x.dtype)

    def proj_items(s, nxt, g, par):
        xn_r, seg = (xa_ref, nxt) if isinstance(s, int) and s == 0 else (xb_ref, s - 1 + nxt)
        qk_r, vt_r = (r.bitcast(bf16) for r in qkv[par])
        part = {}

        def item(m, n, h):
            xn = _unpack(xn_r[pl.ds(pl.multiple_of(seg * (L // 2) + 64 * m, 64), 64), 512 * h:512 * h + 512])
            y = _dot(xn, _unpack(w_u[3 * g + n, 256 * h:256 * h + 256, :]))
            if h == 0:
                part[m, n] = y
                return y
            y = y + part.pop((m, n))
            rows = slice(128 * m, 128 * m + 128)
            if n == 0:
                qk_r[rows, 0:128] = (y * QSCALE).astype(bf16)
                qk_r[rows, 128:256] = _phi(y).astype(bf16)
            elif n == 1:
                qk_r[rows, 256:384] = y.astype(bf16)
                qk_r[rows, 384:512] = _phi(y).astype(bf16)
            else:
                vt_r[0:128, rows] = y.T.astype(bf16)
            return y
        return item

    def attn_items(g, par, seg, use_mem):
        qk_r, vt_r = qkv[par]
        st = {}

        def nd():
            ml = m_ref[g].astype(bf16)
            nd_ref[...] = lax.dot_general(ml, _unpack(qk_r[:, 128:256]), NT, preferred_element_type=f32)

        def upd():
            u = _dot(_unpack(vt_r[...]), _unpack(qk_r[:, 384:512]))
            r2 = lax.broadcasted_iota(i32, (144, 128), 0)
            c2 = lax.broadcasted_iota(i32, (144, 128), 1) >> 5
            keep = jnp.where(r2 < 128, r2 >> 5, r2 - 128) == c2
            u = jnp.where(keep, u, 0.0)
            m_ref[g] = (m_ref[g] + u) if use_mem else u

        def qk(i):
            lane = lax.broadcasted_iota(i32, (16, 128), 1) >> 5
            for be in (range(4) if i % 2 else range(3, -1, -1)):
                b = 4 * i + be
                n = 32 * (b + 1)
                qu = qk_r[16 * b:16 * b + 16, 0:128]
                wq = _unpack(jnp.concatenate(
                    [jnp.where(lane == (c - be) % 4, qu, jnp.uint32(0)) for c in range(4)], axis=0))
                s = lax.dot_general(_unpack(qk_r[0:n // 2, 256:384]), wq, NT, preferred_element_type=f32)
                cols = slice(128 * be, 128 * be + 128)
                if b > 0:
                    s_refs[i][0:n - 32, cols] = s[0:n - 32]
                s_refs[i][n - 32:n, cols] = s[n - 32:n] + bias_ref[...]

        def mx(i, mode='m'):
            for be in range(4):
                if mode == 'load':
                    st[i, 'm', be] = mx_ref[4 * i + be:4 * i + be + 1, :]
                    continue
                n = 32 * (4 * i + be + 1)
                sv = s_refs[i][0:n, 128 * be:128 * be + 128]
                m = jnp.max(jnp.max(sv.reshape(n // 8, 8, 128), axis=0), axis=0, keepdims=True)
                if mode == 'store':
                    mx_ref[4 * i + be:4 * i + be + 1, :] = m
                else:
                    st[i, 'm', be] = m

        def pr(i, t, tok):
            ps = []
            for be in range(4):
                n = 128 if t < i else 32 * (be + 1)
                m8 = after(jnp.broadcast_to(st[i, 'm', be], (8, 128)), tok, be / 4)
                p = jnp.exp2(s_refs[i][128 * t:128 * t + n, 128 * be:128 * be + 128].reshape(n // 8, 8, 128) - m8)
                ls = jnp.sum(p, axis=0)
                p = p.reshape(n, 128)
                st[i, 'l', be] = ls if t == 0 else st[i, 'l', be] + ls
                p_refs[i].bitcast(bf16)[128 * t:128 * t + n, 128 * be:128 * be + 128] = p.astype(bf16)

        def pv(i, t):
            ps = [p_refs[i][64 * t:64 * t + (64 if t < i else 16 * (be + 1)), 128 * be:128 * be + 128]
                  for be in range(4)]
            if t < i:
                ts = _unskew(ps)
            else:
                blk = [_unskew([ps[be][16 * u:16 * u + 16] if be >= u else None for be in range(4)])
                       for u in range(4)]
                ts = [jnp.concatenate([blk[u][j] for u in range(4)], axis=0) for j in range(4)]
            for j in range(4):
                o = _dot(_unpack(vt_r[16 * j:16 * j + 16, 128 * t:128 * t + 128]), _unpack(ts[j]))
                st[i, 'o', j] = o if t == 0 else st[i, 'o', j] + o

        def fin(i):
            ls = _unskew([jnp.sum(st.pop((i, 'l', be)), axis=0, keepdims=True) for be in range(4)])
            parts = []
            for j in range(4):
                gt = gate_ref[pl.ds(4 * g + j, 1), :]
                omg = gate_ref[pl.ds(32 + 4 * g + j, 1), :]
                o = st.pop((i, 'o', j)) * (omg / ls[j])
                if j > 0:
                    o = pltpu.roll(o, 128 - 32 * j, 1)
                if use_mem:
                    den = nd_ref[128 + j:129 + j, 128 * i:128 * i + 128] + 1e-6
                    o = o + nd_ref[32 * j:32 * j + 32, 128 * i:128 * i + 128] * (gt / den)
                parts.append(o)
            ot = jnp.concatenate(parts, axis=0)
            o_ref.bitcast(bf16)[pl.ds(pl.multiple_of((seg % 2 * 4 + g // 2) * L + 128 * i, 128), 128),
                                128 * par:128 * par + 128] = ot.T.astype(bf16)

        def ex(kind, i, t, tok):
            if kind in 'ep':
                pr(i, t, tok)
            if kind in 'ev':
                pv(i, t)
                if t == i:
                    fin(i)
        return nd, upd, qk, mx, ex

    def ln1(seg, r, tok=None, reload=True):
        r0 = pl.multiple_of(r * SUB, SUB)
        x = x_ref[seg, pl.ds(r0, SUB), :].astype(f32)
        if tok is not None:
            x = jnp.concatenate([after(x[:, 0:128], tok, CFG['xfrac']), x[:, 128:]], axis=1)
        if CFG['one']:
            m, rs = _stats(x)
            if CFG['reload'] and reload:
                mx_ref[16:24, :] = jnp.broadcast_to(m[0:8], (8, 128))
                x = x_ref[seg, pl.ds(r0, SUB), :].astype(f32)
            xn = ((x - m) * rs).astype(bf16)
        else:
            xn = _ln(x).astype(bf16)
        if seg < 2:
            xa_b[pl.ds(pl.multiple_of(seg * L + r0, SUB), SUB), :] = xn
        else:
            xb_b[pl.ds(pl.multiple_of((seg - 1) * L + r0, SUB), SUB), :] = xn
        return xn

    def oproj(seg, r0, rows, n, k0=0, k1=NG):
        h0 = pl.multiple_of(r0 // 2, rows // 2)
        r0 = pl.multiple_of(r0, rows)
        lhs = _unpack(jnp.concatenate(
            [o_ref[pl.ds(pl.multiple_of((seg % 2 * 4 + p) * (L // 2) + h0, rows // 2), rows // 2), :]
             for p in range(k0 // 2, k1 // 2)], axis=1))
        y = _dot(lhs, _unpack(wo_u[n, 64 * k0:64 * k1, :]))
        cols = slice(128 * n, 128 * n + 128)
        if k0 > 0:
            y = y + x1_ref[seg, pl.ds(r0, rows), cols]
        if k1 == NG:
            y = _rb(x_ref[seg, pl.ds(r0, rows), cols].astype(f32) + y)
        x1_ref[seg, pl.ds(r0, rows), cols] = y
        return y

    def ln2(seg, c, t, tok=None):
        r0 = pl.multiple_of(c * CH + t * SUB, SUB)
        lane = lax.broadcasted_iota(i32, (SUB, 128), 1)
        x1 = x1_ref[seg, pl.ds(r0, SUB), :]
        if tok is not None and CFG['pace2']:
            x1 = jnp.concatenate([after(x1[:, 0:128], tok, CFG['xfrac']), x1[:, 128:]], axis=1)
        if CFG['one']:
            m, rs = _stats(x1)
            r = _rb((_rowsum(x1 * wrf_ref[0:1, :]) - m * wrf_ref[1:2, 0:128]) * rs)
        else:
            xn2 = _ln(x1, CFG['lnmode'])
            r = _rb(jnp.sum(xn2 * wrf_ref[0:1, :], axis=-1, keepdims=True))
        r_ref[SUB * t:SUB * t + SUB, :] = jnp.where(lane == seg * NG + c, r, r_ref[SUB * t:SUB * t + SUB, :])
        if CFG['one']:
            if CFG['reload']:
                x1 = x1_ref[seg, pl.ds(r0, SUB), :]
            x2 = x1 * (1.0 + rs) - m * rs
        else:
            x2 = x1 + xn2
        x_ref[seg, pl.ds(r0, SUB), :] = x2.astype(bf16)

    def group(s, g, par, last=False):
        kind = s if isinstance(s, int) else 1
        nd, upd, qk, mx, ex = attn_items(g, par, s, kind > 0)
        fill = []
        extra = []
        if kind > 0:
            for n in range(NG):
                fill.append((128, lambda n=n: oproj(s - 1, g * CH, CH, n)))
            extra = [lambda tok, t=t: ln2(s - 1, g, t, tok) for t in range(CH // SUB)]
        else:
            extra = [lambda tok, seg=seg, t=t: ln1(seg, g * (CH // SUB) + t, tok)
                     for seg in range(2, NSEG) for t in range(CH // SUB)]
        if not last:
            gn = g + 1
            pj = proj_items(s, gn // NG, gn % NG, 1 - par)
            for m, n in PORDER:
                for h in range(2):
                    fill.append((128, lambda m=m, n=n, h=h: pj(m, n, h)))
        else:
            for m in range(4):
                for n in range(NG):
                    fill.append((128, lambda m=m, n=n: oproj(s, 128 * m, 128, n, 0, 4)))
        sched = CFG['sched0' if kind == 0 else 'schedL' if last else 'sched'].split()
        y = None
        for tok in sched:
            if tok == 'f':
                y = fill.pop(0)[1]()
            elif tok == 'F':
                while fill:
                    fill.pop(0)[1]()
            elif tok == 'x':
                extra.pop(0)(y)
            elif tok == 'n':
                nd()
            elif tok == 'u':
                if kind < NSEG - 1:
                    upd()
            elif tok[0] == 'q':
                qk(int(tok[1]))
            elif tok[0] == 'Q':
                nxt = attn_items(None, 1 - par, None, None)
                nxt[2](int(tok[1]))
                nxt[3](int(tok[1]), 'store')
            elif tok[0] == 'M':
                mx(int(tok[1]), 'load')
            elif tok[0] == 'm':
                mx(int(tok[1]))
            else:
                ex(tok[0], int(tok[1]), int(tok[2]), y)
        for it in fill:
            it[1]()
        for e in extra:
            e(None)

    for c in range(4):
        cp_x0(c).start()
    for j in range(3):
        cp_w(0, j).start()
    cp_x1().start()
    for cp in cp_small():
        cp.start()

    z_ref[...] = jnp.zeros((8, 128), u32)
    ones = jnp.full((8, 512), 0x3F803F80, u32)
    vt0[64:72, :] = ones
    vt1[64:72, :] = ones
    bias_ref[...] = jnp.where(lax.broadcasted_iota(i32, (32, 128), 0)
                              <= (lax.broadcasted_iota(i32, (32, 128), 1) & 31), 0.0, NEG)

    def ln0_body(c, carry):
        cp_x0(c).wait()
        for t in range(128 // SUB):
            ln1(0, c * (128 // SUB) + t)
        return carry
    lax.fori_loop(0, 4, ln0_body, 0)
    for g in range(1, NG):
        for j in range(3):
            cp_w(g, j).start()
        cp_xr(g - 1).start()
    cp_xr(NG - 1).start()
    for cp in cp_wo():
        cp.start()

    for cp in cp_small():
        cp.wait()
    wr = wr_ref[...].astype(f32)
    wrf_ref[0:1, :] = wr
    wrf_ref[1:2, :] = jnp.broadcast_to(jnp.sum(wr, axis=-1, keepdims=True), (1, D))
    gl = _rb(jax.nn.sigmoid(beta_ref[...].astype(f32)))
    hr = lax.broadcasted_iota(i32, (32, 32), 0)
    hc = lax.broadcasted_iota(i32, (32, 32), 1)
    gcol = jnp.sum(jnp.where(hr == hc, gl, 0.0), axis=1, keepdims=True)
    gate_ref[0:32, :] = jnp.broadcast_to(gcol, (32, 128))
    gate_ref[32:64, :] = jnp.broadcast_to(_rb(1.0 - gcol), (32, 128))
    for j in range(2):
        cp_w(0, j).wait()
    if CFG['prewait']:
        for g in range(NG):
            cp_xr(g).wait()
            for j in range(3 * (g > 0)):
                cp_w(g, j).wait()
        for cp in cp_wo():
            cp.wait()

    def layer(li, carry):
        first = li == 0
        r_ref[...] = jnp.full((CH, 128), -jnp.inf, f32)
        pj = proj_items(0, 0, 0, 0)
        fill = [(m, n, h) for m, n in PORDER for h in range(2)]
        extra = list(range(L // SUB))
        y = None
        for tok in CFG['pre'].split():
            if tok == 'f':
                y = pj(*fill.pop(0))
            elif tok == 'x':
                ln1(1, extra.pop(0), y)
            elif tok == 'w':
                @pl.when(first)
                def _():
                    cp_w(0, 2).wait()
                    cp_x1().wait()
                y = None
            else:
                nxt = attn_items(None, 0, None, None)
                nxt[2](int(tok[1]))
                nxt[3](int(tok[1]), 'store')
        assert not fill and not extra
        cp_xn().start()

        def pair(s, p, last=False):
            for par in range(2):
                group(s, 2 * p + par, par, last and par == 1)

        def seg0(p, c2):
            if not CFG['prewait']:
                @pl.when(first)
                def _():
                    for par in range(2):
                        cp_xr(2 * p + par).wait()
                    for j in range(3):
                        cp_w(2 * p + 1, j).wait()

                    @pl.when(p < NG // 2 - 1)
                    def _():
                        for j in range(3):
                            cp_w(jnp.minimum(2 * p + 2, NG - 2), j).wait()

                    @pl.when(p == NG // 2 - 1)
                    def _():
                        for cp in cp_wo():
                            cp.wait()
            pair(0, p)
            return c2
        _loop('s0', NG // 2, seg0)
        cp_xn().wait()

        @pl.when(first)
        def _():
            for cp in cp_ff():
                cp.start()

        def mid(t, c2):
            pair(1 + t // (NG // 2), t % (NG // 2))
            return c2
        _loop('s1', NG, mid)

        @pl.when(li == CFG['nl'] - 1)
        def _():
            cp_out_seg(0).start()
            cp_out_seg(1).start()

        def seg3(p, c2):
            pair(NSEG - 1, p)
            return c2
        _loop('s3', NG // 2 - 1, seg3)
        pair(NSEG - 1, NG // 2 - 1, last=True)

        s = NSEG - 1
        pend = []
        for m in (3, 2, 1, 0):
            for n in range(NG):
                oproj(s, 128 * m, 128, n, 4, NG)
                if pend:
                    pend.pop(0)()
            pend = [lambda c=c, t=t: ln2(s, c, t) for c in (2 * m, 2 * m + 1) for t in range(CH // SUB)]
        for e in pend:
            e()

        @pl.when(li == CFG['nl'] - 1)
        def _():
            cp_out_seg(NSEG - 2).start()
            cp_out_seg(NSEG - 1).start()

        rm = r_ref[...]
        idx = (lax.broadcasted_iota(i32, (CH, 128), 1) * CH + lax.broadcasted_iota(i32, (CH, 128), 0)).astype(f32)
        big = float(S)
        m1 = jnp.max(rm, axis=(0, 1), keepdims=True)
        i1 = jnp.min(jnp.where(rm == m1, idx, big), axis=(0, 1), keepdims=True)
        rm2 = jnp.where(idx == i1, -jnp.inf, rm)
        m2 = jnp.max(rm2, axis=(0, 1), keepdims=True)
        i2 = jnp.min(jnp.where(jnp.logical_and(rm2 == m2, idx != i1), idx, big), axis=(0, 1), keepdims=True)
        toks = [jnp.clip(jnp.max(iv).astype(i32), 0, S - 1) for iv in (i1, i2)]

        @pl.when(first)
        def _():
            for cp in cp_ff():
                cp.wait()

        row = lax.broadcasted_iota(i32, (SUB, D), 0)
        x1s = jnp.where(row == 0, x1_ref[toks[0] // L, pl.ds(toks[0] % L, 1), :],
                        jnp.where(row == 1, x1_ref[toks[1] // L, pl.ds(toks[1] % L, 1), :], 0.0))
        xs = _ln(x1s, 2 * CFG['lnmode']).astype(bf16)
        lag, due = CFG['lag'], []

        def gated(lhs, c):
            u = pltpu.bitcast(lhs, u32)
            if c < lag or lag == 0:
                return lhs
            t = u[:, 0:128]
            for d in due[c - lag]:
                t = t | (pltpu.bitcast(d[:, d.shape[1] - 128:], u32) & z_ref[...])
            return pltpu.bitcast(jnp.concatenate([t, u[:, 128:]], axis=1), bf16)
        hs = []
        for c in range(NF):
            xc = gated(xs, c)
            if c >= NF - CFG['fskip']:
                hs.append(hs[0])
                due.append([ln1(0, c, ga, CFG['freload'])])
                continue
            ga = _rb(_dot(xc, _unpack(wg_u[c])))
            up = _rb(_dot(xc, _unpack(wu_u[c])))
            hs.append((_rb(ga * _rb(jax.nn.sigmoid(ga))) * up).astype(bf16))
            due.append([hs[-1], ln1(0, c, ga, CFG['freload'])])
        hdn = jnp.concatenate(hs, axis=1)
        ys = []
        for c in range(NG):
            ys.append(_dot(gated(hdn, NF + c), _unpack(wd_u[c])))
            due.append([ln1(0, NF + c, ys[-1], CFG['freload'])] if NF + c < L // SUB else [])
        y = _rb(jnp.concatenate(ys, axis=1))
        rsel = jnp.where(lax.broadcasted_iota(i32, (SUB, 1), 0) == 0, m1, m2)
        y = _rb(y * _rb(jax.nn.sigmoid(rsel)))
        x2s = _rb(x1s + _rb(xs.astype(f32) + y))
        xns = _ln(x2s)

        @pl.when(li == CFG['nl'] - 1)
        def _():
            for s in range(NSEG):
                cp_out_seg(s).wait()

        blks = []
        for n, t in enumerate(toks):
            sg = t // L
            b0 = pl.multiple_of((t % L) // SUB * SUB, SUB)
            hb = pl.multiple_of((t % L) // SUB * (SUB // 2), SUB // 2)
            hit = row == (t % SUB)
            old = x_ref[sg, pl.ds(b0, SUB), :].astype(f32)
            x_ref[sg, pl.ds(b0, SUB), :] = jnp.where(hit, x2s[n:n + 1], old).astype(bf16)
            oldn = _unpack(xa_ref[pl.ds(hb, SUB // 2), :]).astype(f32)
            xa_ref[pl.ds(hb, SUB // 2), :] = _pack(jnp.where(row == t - b0, xns[n:n + 1], oldn))
            blks.append((sg, b0))

        @pl.when(li == CFG['nl'] - 1)
        def _():
            def cp_fix(n):
                sg, b0 = blks[n]
                return pltpu.make_async_copy(x_ref.at[sg, pl.ds(b0, SUB), :],
                                             out_hbm.at[sg, pl.ds(b0, SUB), :], sems.at[SEM_FIX])
            differ = (toks[0] // SUB) != (toks[1] // SUB)
            cp_fix(0).start()

            @pl.when(differ)
            def _():
                cp_fix(1).start()
                cp_fix(1).wait()
            cp_fix(0).wait()
        return carry

    lax.fori_loop(0, CFG['nl'], layer, 0)


@jax.jit
def pallas_interleave_layers__memory_aug_infini_attn__moe_arch_mod__prompt_kernel(
    A_x: jax.Array,
    A_wq: jax.Array,
    A_wk: jax.Array,
    A_wv: jax.Array,
    A_wo: jax.Array,
    A_beta: jax.Array,
    B_x: jax.Array,
    B_w_r: jax.Array,
    B_w_gate: jax.Array,
    B_w_up: jax.Array,
    B_w_down: jax.Array,
):
    del B_x
    qkv_bufs = [pltpu.VMEM((L // 2, 512), u32), pltpu.VMEM((72, L), u32)]
    scratch = [
        pltpu.VMEM((NSEG, L, D), bf16),
        pltpu.VMEM((3 * L // 2, D), u32),
        pltpu.VMEM((NSEG, L, D), f32),
        pltpu.VMEM((3 * NG, D, 128), bf16),
        pltpu.VMEM((NG, D, 128), bf16),
        pltpu.VMEM((NF, D, 128), bf16),
        pltpu.VMEM((NF, D, 128), bf16),
        pltpu.VMEM((NG, F, 128), bf16),
        pltpu.VMEM((64, 128), f32),
        pltpu.VMEM((32, 128), f32),
        pltpu.VMEM((NG, 144, 128), f32),
        pltpu.VMEM((CH, 128), f32),
        pltpu.VMEM((144, L), f32),
        pltpu.VMEM((128, L), f32), pltpu.VMEM((256, L), f32),
        pltpu.VMEM((384, L), f32), pltpu.VMEM((512, L), f32),
        pltpu.VMEM((64, L), u32), pltpu.VMEM((128, L), u32),
        pltpu.VMEM((192, L), u32), pltpu.VMEM((256, L), u32),
        *qkv_bufs, *qkv_bufs,
        pltpu.VMEM((NG * L // 2, 256), u32),
        pltpu.VMEM((L, D), u32),
        pltpu.VMEM((24, 128), f32),
        pltpu.VMEM((8, 128), u32),
        pltpu.VMEM((2, D), f32),
        pltpu.VMEM((1, D), bf16),
        pltpu.VMEM((1, 32), bf16),
        pltpu.SemaphoreType.DMA((NSEM,)),
    ]
    out = pl.pallas_call(
        _kernel,
        out_shape=jax.ShapeDtypeStruct((NSEG, L, D), bf16),
        in_specs=[pl.BlockSpec(memory_space=pl.ANY)] * 10,
        out_specs=pl.BlockSpec(memory_space=pl.ANY),
        scratch_shapes=scratch,
        compiler_params=pltpu.CompilerParams(vmem_limit_bytes=100 * 2 ** 20),
    )(A_x.reshape(NSEG, L, D), A_wq, A_wk, A_wv, A_wo, A_beta.reshape(1, 32), B_w_r.reshape(1, D),
      B_w_gate, B_w_up, B_w_down)
    return out.reshape(1, S, D)
```

```python
import jax
import jax.numpy as jnp
from jax import lax
import jax.experimental.pallas as pl
import jax.experimental.pallas.tpu as pltpu

bf16 = jnp.bfloat16
f32 = jnp.float32
u32 = jnp.uint32
i32 = jnp.int32

S = 2048
D = 1024
L = 512
NSEG = 4
NG = 8
F = 3584
CH = 64
SUB = 16
NEG = -1e30
QSCALE = (32 ** -0.5) * 1.4426950408889634
NT = (((1,), (1,)), ((), ()))

SEM_XC = 0
SEM_W0 = 4
SEM_X1 = 5
SEM_SM = 6
SEM_P = 7
NSEM = 11
SEM_OUT, SEM_FIX, SEM_FF, SEM_XN = 0, 1, 2, 3
NF = F // 128
PORDER = [(m, n) for m in range(4) for n in range(2)] + [(m, 2) for m in range(4)]

CFG = dict(
    rep={}, cnt={}, merge3=0, zpad=3, issue='abcdqksr vx', lnmode=0, nl=2, prewait=False, gp=2, pace=True, pace2=True, one=True, reload=True, chain=True, xfrac=0.0, freload=False, lag=0, fskip=0,
    pre='f ' * 16 + 'w x x x x Q3 ' + 'f x x x x ' * 7 + 'f',
    sched='M3 f p30 f n q2 v30 p31 f f v31 p32 f f m2 v32 p33 f f v33 p20 f f q1 v20 p21 f x f v21 p22 f x f '
          'm1 v22 p10 f x f q0 v10 p11 f x f u v11 m0 f p00 f f v00 F Q3',
    sched0='M3 f p30 f q2 v30 p31 f f v31 p32 f f x m2 v32 p33 f f x v33 p20 f f x q1 v20 p21 f f x '
           'v21 p22 f f x m1 v22 p10 f f x q0 v10 p11 f x f u v11 m0 f x p00 f f v00 F Q3',
    schedL='M3 f p30 f n q2 v30 p31 f f v31 p32 f f m2 v32 p33 f f v33 p20 f f q1 v20 p21 f x f v21 p22 f x f '
          'm1 v22 p10 f x f q0 v10 p11 f x f v11 m0 f p00 f f v00 F',
)


def _loop(name, n, body):
    rep = CFG['rep'].get(name, 1)
    n = CFG['cnt'].get(name, n)
    if n == 0:
        return 0
    if rep == 1:
        return lax.fori_loop(0, n, body, 0)
    return lax.fori_loop(0, n * rep, lambda i, c: body(i // rep, c), 0)


def _rb(x):
    return x.astype(bf16).astype(f32)


def _pack(x):
    return pltpu.bitcast(x.astype(bf16), u32)


def _unpack(u):
    return pltpu.bitcast(u, bf16)


def _phi(t):
    return jnp.where(t > 0, t + 1.0, jnp.exp(t))


def _dot(a, b):
    return jnp.dot(a, b, preferred_element_type=f32)


def _unskew(ps):
    shape, dt = next((p.shape, p.dtype) for p in ps if p is not None)
    c = lax.broadcasted_iota(i32, shape, 1) >> 5
    even = (c & 1) == 0
    lo = c < 2
    mid = jnp.logical_or(c == 1, c == 2)

    def sel(mask, a, b):
        if a is None and b is None:
            return None
        z = jnp.zeros(shape, dt)
        return jnp.where(mask, z if a is None else a, z if b is None else b)
    x0, x1 = sel(even, ps[0], ps[1]), sel(even, ps[1], ps[0])
    x2, x3 = sel(even, ps[2], ps[3]), sel(even, ps[3], ps[2])
    return [sel(lo, x0, x2), sel(mid, x1, x3), sel(lo, x2, x0), sel(mid, x3, x1)]


def _ln(x, mode=0):
    acc = x
    if CFG['chain']:
        acc = x[:, 0:128]
        for c in range(1, x.shape[1] // 128):
            acc = acc + x[:, 128 * c:128 * c + 128]
    m = jnp.sum(acc, axis=-1, keepdims=True) * (1.0 / D)
    if mode == 0:
        e = x - m
        v = jnp.sum(e * e, axis=-1, keepdims=True) * (1.0 / D)
        return e * lax.rsqrt(v + 1e-5)
    c = _rb(m)
    e = x - c
    v = jnp.sum(e * e, axis=-1, keepdims=True) * (1.0 / D) - (m - c) * (m - c)
    w = _rb(_rb(jnp.maximum(v, 0.0)) + 1e-5)
    den = _rb(w * lax.rsqrt(w))
    if mode == 2:
        return _rb(_rb(e) / den)
    return e * (1.0 / den)


def _rowsum(x, first=None):
    acc = x[:, 0:128] if first is None else first
    for c in range(1, x.shape[1] // 128):
        acc = acc + x[:, 128 * c:128 * c + 128]
    return jnp.sum(acc, axis=-1, keepdims=True)


def _stats(x):
    m = _rowsum(x) * (1.0 / D)
    v = jnp.maximum(_rowsum(x * x) * (1.0 / D) - m * m, 0.0)
    return m, lax.rsqrt(v + 1e-5)


def _kernel(x_hbm, wq_hbm, wk_hbm, wv_hbm, wo_hbm, beta_hbm, wr_hbm, wg_hbm, wu_hbm, wd_hbm,
            out_hbm,
            z_ref, x_ref, xb_ref, x1_ref, w_ref, wo_ref, wg_ref, wu_ref, wd_ref,
            gate_ref, bias_ref, m_ref, r_ref, nd_ref,
            s0_ref, s1_ref, s2_ref, s3_ref, p0_ref, p1_ref, p2_ref, p3_ref,
            qk0, vt0, qk1, vt1, o_ref, xa_ref, mx_ref, wrf_ref, wr_ref, beta_ref, sems):
    qkv = ((qk0, vt0), (qk1, vt1))
    s_refs = (s0_ref, s1_ref, s2_ref, s3_ref)
    p_refs = (p0_ref, p1_ref, p2_ref, p3_ref)
    xa_b, xb_b = xa_ref.bitcast(bf16), xb_ref.bitcast(bf16)
    w_u, wo_u, wg_u, wu_u, wd_u = (r.bitcast(u32) for r in (w_ref, wo_ref, wg_ref, wu_ref, wd_ref))

    def cp_x0(c):
        rows = pl.ds(pl.multiple_of(128 * c, 128), 128)
        return pltpu.make_async_copy(x_hbm.at[0, rows], x_ref.at[0, rows], sems.at[SEM_XC + c])

    def cp_x1():
        return pltpu.make_async_copy(x_hbm.at[1], x_ref.at[1], sems.at[SEM_X1])

    def cp_xn():
        return pltpu.make_async_copy(xa_ref.at[L // 2:L], xb_ref.at[0:L // 2], sems.at[SEM_XN])

    def cp_xr(g):
        r0 = pl.multiple_of(g * CH, CH)
        return pltpu.make_async_copy(x_hbm.at[2:NSEG, pl.ds(r0, CH), :],
                                     x_ref.at[2:NSEG, pl.ds(r0, CH), :], sems.at[SEM_P + g // 2])

    def cp_w(g, j):
        c0 = pl.multiple_of(g * 128, 128)
        src = (wq_hbm, wk_hbm, wv_hbm)[j]
        sem = (SEM_W0 + j // 2) if isinstance(g, int) and g == 0 else SEM_P + (g - 1) // 2
        return pltpu.make_async_copy(src.at[:, pl.ds(c0, 128)], w_ref.at[3 * g + j], sems.at[sem])

    def slabs(src, dst, n, sem):
        return [pltpu.make_async_copy(src.at[:, 128 * c:128 * c + 128], dst.at[c], sems.at[sem]) for c in range(n)]

    def cp_wo():
        return slabs(wo_hbm, wo_ref, NG, SEM_P + 3)

    def cp_small():
        return (pltpu.make_async_copy(beta_hbm, beta_ref, sems.at[SEM_SM]),
                pltpu.make_async_copy(wr_hbm, wr_ref, sems.at[SEM_SM]))

    def cp_ff():
        return (slabs(wg_hbm, wg_ref, NF, SEM_FF) + slabs(wu_hbm, wu_ref, NF, SEM_FF)
                + slabs(wd_hbm, wd_ref, NG, SEM_FF))

    def cp_out_seg(s):
        return pltpu.make_async_copy(x_ref.at[s], out_hbm.at[s], sems.at[SEM_OUT])

    def after(x, tok, frac):
        if tok is None or not CFG['pace']:
            return x
        r = 8 * int(frac * tok.shape[0] // 8)
        t = pltpu.bitcast(tok[r:r + 8, 0:128], u32) & z_ref[0:8, :]
        t = jnp.tile(t, (x.shape[0] // 8, x.shape[1] // 128))
        return pltpu.bitcast(pltpu.bitcast(x, u32) | t, x.dtype)

    def proj_items(s, nxt, g, par):
        xn_r, seg = (xa_ref, nxt) if isinstance(s, int) and s == 0 else (xb_ref, s - 1 + nxt)
        qk_r, vt_r = (r.bitcast(bf16) for r in qkv[par])
        part = {}

        def item(m, n, h):
            xn = _unpack(xn_r[pl.ds(pl.multiple_of(seg * (L // 2) + 64 * m, 64), 64), 512 * h:512 * h + 512])
            y = _dot(xn, _unpack(w_u[3 * g + n, 256 * h:256 * h + 256, :]))
            if h == 0:
                part[m, n] = y
                return y
            y = y + part.pop((m, n))
            rows = slice(128 * m, 128 * m + 128)
            if n == 0:
                qk_r[rows, 0:128] = (y * QSCALE).astype(bf16)
                qk_r[rows, 128:256] = _phi(y).astype(bf16)
            elif n == 1:
                qk_r[rows, 256:384] = y.astype(bf16)
                qk_r[rows, 384:512] = _phi(y).astype(bf16)
            else:
                vt_r[0:128, rows] = y.T.astype(bf16)
            return y
        return item

    def attn_items(g, par, seg, use_mem):
        qk_r, vt_r = qkv[par]
        st = {}

        def nd():
            ml = m_ref[g].astype(bf16)
            nd_ref[...] = lax.dot_general(ml, _unpack(qk_r[:, 128:256]), NT, preferred_element_type=f32)

        def upd():
            u = _dot(_unpack(vt_r[...]), _unpack(qk_r[:, 384:512]))
            r2 = lax.broadcasted_iota(i32, (144, 128), 0)
            c2 = lax.broadcasted_iota(i32, (144, 128), 1) >> 5
            keep = jnp.where(r2 < 128, r2 >> 5, r2 - 128) == c2
            u = jnp.where(keep, u, 0.0)
            m_ref[g] = (m_ref[g] + u) if use_mem else u

        def qk(i):
            lane = lax.broadcasted_iota(i32, (16, 128), 1) >> 5
            for be in (range(4) if i % 2 else range(3, -1, -1)):
                b = 4 * i + be
                n = 32 * (b + 1)
                qu = qk_r[16 * b:16 * b + 16, 0:128]
                wq = _unpack(jnp.concatenate(
                    [jnp.where(lane == (c - be) % 4, qu, jnp.uint32(0)) for c in range(4)], axis=0))
                s = lax.dot_general(_unpack(qk_r[0:n // 2, 256:384]), wq, NT, preferred_element_type=f32)
                cols = slice(128 * be, 128 * be + 128)
                if b > 0:
                    s_refs[i][0:n - 32, cols] = s[0:n - 32]
                s_refs[i][n - 32:n, cols] = s[n - 32:n] + bias_ref[...]

        def mx(i, mode='m'):
            for be in range(4):
                if mode == 'load':
                    st[i, 'm', be] = mx_ref[4 * i + be:4 * i + be + 1, :]
                    continue
                n = 32 * (4 * i + be + 1)
                sv = s_refs[i][0:n, 128 * be:128 * be + 128]
                m = jnp.max(jnp.max(sv.reshape(n // 8, 8, 128), axis=0), axis=0, keepdims=True)
                if mode == 'store':
                    mx_ref[4 * i + be:4 * i + be + 1, :] = m
                else:
                    st[i, 'm', be] = m

        def pr(i, t, tok):
            ps = []
            for be in range(4):
                n = 128 if t < i else 32 * (be + 1)
                m8 = after(jnp.broadcast_to(st[i, 'm', be], (8, 128)), tok, be / 4)
                p = jnp.exp2(s_refs[i][128 * t:128 * t + n, 128 * be:128 * be + 128].reshape(n // 8, 8, 128) - m8)
                ls = jnp.sum(p, axis=0)
                p = p.reshape(n, 128)
                st[i, 'l', be] = ls if t == 0 else st[i, 'l', be] + ls
                p_refs[i].bitcast(bf16)[128 * t:128 * t + n, 128 * be:128 * be + 128] = p.astype(bf16)

        def pv(i, t):
            ps = [p_refs[i][64 * t:64 * t + (64 if t < i else 16 * (be + 1)), 128 * be:128 * be + 128]
                  for be in range(4)]
            if t < i:
                ts = _unskew(ps)
            else:
                blk = [_unskew([ps[be][16 * u:16 * u + 16] if be >= u else None for be in range(4)])
                       for u in range(4)]
                ts = [jnp.concatenate([blk[u][j] for u in range(4)], axis=0) for j in range(4)]
            for j in range(4):
                o = _dot(_unpack(vt_r[16 * j:16 * j + 16, 128 * t:128 * t + 128]), _unpack(ts[j]))
                st[i, 'o', j] = o if t == 0 else st[i, 'o', j] + o

        def fin(i):
            ls = _unskew([jnp.sum(st.pop((i, 'l', be)), axis=0, keepdims=True) for be in range(4)])
            parts = []
            for j in range(4):
                gt = gate_ref[pl.ds(4 * g + j, 1), :]
                omg = gate_ref[pl.ds(32 + 4 * g + j, 1), :]
                o = st.pop((i, 'o', j)) * (omg / ls[j])
                if j > 0:
                    o = pltpu.roll(o, 128 - 32 * j, 1)
                if use_mem:
                    den = nd_ref[128 + j:129 + j, 128 * i:128 * i + 128] + 1e-6
                    o = o + nd_ref[32 * j:32 * j + 32, 128 * i:128 * i + 128] * (gt / den)
                parts.append(o)
            ot = jnp.concatenate(parts, axis=0)
            o_ref.bitcast(bf16)[pl.ds(pl.multiple_of((seg % 2 * 4 + g // 2) * L + 128 * i, 128), 128),
                                128 * par:128 * par + 128] = ot.T.astype(bf16)

        def ex(kind, i, t, tok):
            if kind in 'ep':
                pr(i, t, tok)
            if kind in 'ev':
                pv(i, t)
                if t == i:
                    fin(i)
        return nd, upd, qk, mx, ex

    def ln1(seg, r, tok=None, reload=True):
        r0 = pl.multiple_of(r * SUB, SUB)
        x = x_ref[seg, pl.ds(r0, SUB), :].astype(f32)
        if tok is not None:
            x = jnp.concatenate([after(x[:, 0:128], tok, CFG['xfrac']), x[:, 128:]], axis=1)
        if CFG['one']:
            m, rs = _stats(x)
            if CFG['reload'] and reload:
                mx_ref[16:24, :] = jnp.broadcast_to(m[0:8], (8, 128))
                x = x_ref[seg, pl.ds(r0, SUB), :].astype(f32)
            xn = ((x - m) * rs).astype(bf16)
        else:
            xn = _ln(x).astype(bf16)
        if seg < 2:
            xa_b[pl.ds(pl.multiple_of(seg * L + r0, SUB), SUB), :] = xn
        else:
            xb_b[pl.ds(pl.multiple_of((seg - 1) * L + r0, SUB), SUB), :] = xn
        return xn

    def oproj(seg, r0, rows, n, k0=0, k1=NG):
        h0 = pl.multiple_of(r0 // 2, rows // 2)
        r0 = pl.multiple_of(r0, rows)
        lhs = _unpack(jnp.concatenate(
            [o_ref[pl.ds(pl.multiple_of((seg % 2 * 4 + p) * (L // 2) + h0, rows // 2), rows // 2), :]
             for p in range(k0 // 2, k1 // 2)], axis=1))
        y = _dot(lhs, _unpack(wo_u[n, 64 * k0:64 * k1, :]))
        cols = slice(128 * n, 128 * n + 128)
        if k0 > 0:
            y = y + x1_ref[seg, pl.ds(r0, rows), cols]
        if k1 == NG:
            y = _rb(x_ref[seg, pl.ds(r0, rows), cols].astype(f32) + y)
        x1_ref[seg, pl.ds(r0, rows), cols] = y
        return y

    def ln2(seg, c, t, tok=None):
        r0 = pl.multiple_of(c * CH + t * SUB, SUB)
        lane = lax.broadcasted_iota(i32, (SUB, 128), 1)
        x1 = x1_ref[seg, pl.ds(r0, SUB), :]
        if tok is not None and CFG['pace2']:
            x1 = jnp.concatenate([after(x1[:, 0:128], tok, CFG['xfrac']), x1[:, 128:]], axis=1)
        if CFG['one']:
            m, rs = _stats(x1)
            r = _rb((_rowsum(x1 * wrf_ref[0:1, :]) - m * wrf_ref[1:2, 0:128]) * rs)
        else:
            xn2 = _ln(x1, CFG['lnmode'])
            r = _rb(jnp.sum(xn2 * wrf_ref[0:1, :], axis=-1, keepdims=True))
        r_ref[SUB * t:SUB * t + SUB, :] = jnp.where(lane == seg * NG + c, r, r_ref[SUB * t:SUB * t + SUB, :])
        if CFG['one']:
            if CFG['reload']:
                x1 = x1_ref[seg, pl.ds(r0, SUB), :]
            x2 = x1 * (1.0 + rs) - m * rs
        else:
            x2 = x1 + xn2
        x_ref[seg, pl.ds(r0, SUB), :] = x2.astype(bf16)

    def group(s, g, par, last=False):
        kind = s if isinstance(s, int) else 1
        nd, upd, qk, mx, ex = attn_items(g, par, s, kind > 0)
        fill = []
        extra = []
        if kind > 0:
            for n in range(NG):
                fill.append((128, lambda n=n: oproj(s - 1, g * CH, CH, n)))
            extra = [lambda tok, t=t: ln2(s - 1, g, t, tok) for t in range(CH // SUB)]
        else:
            extra = [lambda tok, seg=seg, t=t: ln1(seg, g * (CH // SUB) + t, tok)
                     for seg in range(2, NSEG) for t in range(CH // SUB)]
        if not last:
            gn = g + 1
            pj = proj_items(s, gn // NG, gn % NG, 1 - par)
            for m, n in PORDER:
                for h in range(2):
                    fill.append((128, lambda m=m, n=n, h=h: pj(m, n, h)))
        else:
            for m in range(4):
                for n in range(NG):
                    fill.append((128, lambda m=m, n=n: oproj(s, 128 * m, 128, n, 0, 4)))
        sched = CFG['sched0' if kind == 0 else 'schedL' if last else 'sched'].split()
        y = None
        for tok in sched:
            if tok == 'f':
                y = fill.pop(0)[1]()
            elif tok == 'F':
                while fill:
                    fill.pop(0)[1]()
            elif tok == 'x':
                extra.pop(0)(y)
            elif tok == 'n':
                nd()
            elif tok == 'u':
                if kind < NSEG - 1:
                    upd()
            elif tok[0] == 'q':
                qk(int(tok[1]))
            elif tok[0] == 'Q':
                nxt = attn_items(None, 1 - par, None, None)
                nxt[2](int(tok[1]))
                nxt[3](int(tok[1]), 'store')
            elif tok[0] == 'M':
                mx(int(tok[1]), 'load')
            elif tok[0] == 'm':
                mx(int(tok[1]))
            else:
                ex(tok[0], int(tok[1]), int(tok[2]), y)
        for it in fill:
            it[1]()
        for e in extra:
            e(None)

    early = {'a': cp_x0(0), 'b': cp_x0(1), 'c': cp_x0(2), 'd': cp_x0(3), 'q': cp_w(0, 0), 'k': cp_w(0, 1),
             'v': cp_w(0, 2), 'x': cp_x1(), 's': cp_small()[0], 'r': cp_small()[1]}
    issue = CFG['issue'].split()
    for k in issue[0]:
        early[k].start()

    z_ref[0:8, :] = jnp.zeros((8, 128), u32)
    ones = jnp.full((8, 512), 0x3F803F80, u32)
    vt0[64:72, :] = ones
    vt1[64:72, :] = ones
    bias_ref[...] = jnp.where(lax.broadcasted_iota(i32, (32, 128), 0)
                              <= (lax.broadcasted_iota(i32, (32, 128), 1) & 31), 0.0, NEG)

    def ln0_body(c, carry):
        cp_x0(c).wait()
        for n in range(1, len(issue)):
            @pl.when(c == n - 1)
            def _():
                for k in issue[n].strip('-'):
                    early[k].start()
        for t in range(128 // SUB):
            ln1(0, c * (128 // SUB) + t)
        return carry
    lax.fori_loop(0, 4, ln0_body, 0)
    for g in range(1, NG):
        for j in range(3):
            cp_w(g, j).start()
        cp_xr(g - 1).start()
    cp_xr(NG - 1).start()
    for cp in cp_wo():
        cp.start()

    for cp in cp_small():
        cp.wait()
    wr = wr_ref[...].astype(f32)
    for c in range(D // 128):
        wrf_ref[0:1, 128 * c:128 * c + 128] = wr[c:c + 1, :]
    wrf_ref[1:2, :] = jnp.broadcast_to(jnp.sum(wr, axis=(0, 1), keepdims=True), (1, D))
    gl = _rb(jax.nn.sigmoid(beta_ref[...].astype(f32)))
    hr = lax.broadcasted_iota(i32, (32, 32), 0)
    hc = lax.broadcasted_iota(i32, (32, 32), 1)
    gcol = jnp.sum(jnp.where(hr == hc, gl, 0.0), axis=1, keepdims=True)
    gate_ref[0:32, :] = jnp.broadcast_to(gcol, (32, 128))
    gate_ref[32:64, :] = jnp.broadcast_to(_rb(1.0 - gcol), (32, 128))
    for j in range(2):
        cp_w(0, j).wait()
    if CFG['prewait']:
        for g in range(NG):
            cp_xr(g).wait()
            for j in range(3 * (g > 0)):
                cp_w(g, j).wait()
        for cp in cp_wo():
            cp.wait()

    def layer(li, carry):
        first = li == 0
        r_ref[...] = jnp.full((CH, 128), -jnp.inf, f32)
        pj = proj_items(0, 0, 0, 0)
        fill = [(m, n, h) for m, n in PORDER for h in range(2)]
        extra = list(range(L // SUB))
        y = None
        for tok in CFG['pre'].split():
            if tok == 'f':
                y = pj(*fill.pop(0))
            elif tok == 'x':
                ln1(1, extra.pop(0), y)
            elif tok == 'w':
                @pl.when(first)
                def _():
                    cp_w(0, 2).wait()
                    cp_x1().wait()
                y = None
            else:
                nxt = attn_items(None, 0, None, None)
                nxt[2](int(tok[1]))
                nxt[3](int(tok[1]), 'store')
        assert not fill and not extra
        cp_xn().start()

        def pair(s, p, last=False):
            for par in range(2):
                group(s, 2 * p + par, par, last and par == 1)

        def seg0(p, c2):
            if not CFG['prewait']:
                @pl.when(first)
                def _():
                    for par in range(2):
                        cp_xr(2 * p + par).wait()
                    for j in range(3):
                        cp_w(2 * p + 1, j).wait()

                    @pl.when(p < NG // 2 - 1)
                    def _():
                        for j in range(3):
                            cp_w(jnp.minimum(2 * p + 2, NG - 2), j).wait()

                    @pl.when(p == NG // 2 - 1)
                    def _():
                        for cp in cp_wo():
                            cp.wait()
            pair(0, p)
            return c2
        _loop('s0', NG // 2, seg0)
        cp_xn().wait()

        @pl.when(first)
        def _():
            for cp in cp_ff():
                cp.start()

        def mid(t, c2):
            pair(1 + t // (NG // 2), t % (NG // 2))
            return c2
        _loop('s1', NG + (NG // 2 - 1) * CFG['merge3'], mid)

        @pl.when(li == CFG['nl'] - 1)
        def _():
            cp_out_seg(0).start()
            cp_out_seg(1).start()

        def seg3(p, c2):
            pair(NSEG - 1, p)
            return c2
        if not CFG['merge3']:
            _loop('s3', NG // 2 - 1, seg3)
        pair(NSEG - 1, NG // 2 - 1, last=True)

        s = NSEG - 1
        pend = []
        for m in (3, 2, 1, 0):
            for n in range(NG):
                oproj(s, 128 * m, 128, n, 4, NG)
                if pend:
                    pend.pop(0)()
            pend = [lambda c=c, t=t: ln2(s, c, t) for c in (2 * m, 2 * m + 1) for t in range(CH // SUB)]
        for e in pend:
            e()

        @pl.when(li == CFG['nl'] - 1)
        def _():
            cp_out_seg(NSEG - 2).start()
            cp_out_seg(NSEG - 1).start()

        rm = r_ref[...]
        idx = (lax.broadcasted_iota(i32, (CH, 128), 1) * CH + lax.broadcasted_iota(i32, (CH, 128), 0)).astype(f32)
        big = float(S)
        m1 = jnp.max(rm, axis=(0, 1), keepdims=True)
        i1 = jnp.min(jnp.where(rm == m1, idx, big), axis=(0, 1), keepdims=True)
        rm2 = jnp.where(idx == i1, -jnp.inf, rm)
        m2 = jnp.max(rm2, axis=(0, 1), keepdims=True)
        i2 = jnp.min(jnp.where(jnp.logical_and(rm2 == m2, idx != i1), idx, big), axis=(0, 1), keepdims=True)
        toks = [jnp.clip(jnp.max(iv).astype(i32), 0, S - 1) for iv in (i1, i2)]

        @pl.when(first)
        def _():
            for cp in cp_ff():
                cp.wait()

        row = lax.broadcasted_iota(i32, (SUB, D), 0)
        x1s = jnp.where(row == 0, x1_ref[toks[0] // L, pl.ds(toks[0] % L, 1), :],
                        jnp.where(row == 1, x1_ref[toks[1] // L, pl.ds(toks[1] % L, 1), :], 0.0))
        xs = _ln(x1s, 2 * CFG['lnmode']).astype(bf16)
        lag, due = CFG['lag'], []

        def gated(lhs, c):
            u = pltpu.bitcast(lhs, u32)
            if c < lag or lag == 0:
                return lhs
            t = u[:, 0:128]
            for d in due[c - lag]:
                t = t | (pltpu.bitcast(d[:, d.shape[1] - 128:], u32) & z_ref[0:8, :])
            return pltpu.bitcast(jnp.concatenate([t, u[:, 128:]], axis=1), bf16)
        hs = []
        for c in range(NF):
            xc = gated(xs, c)
            if c >= NF - CFG['fskip']:
                hs.append(hs[0])
                due.append([ln1(0, c, ga, CFG['freload'])])
                continue
            ga = _rb(_dot(xc, _unpack(wg_u[c])))
            up = _rb(_dot(xc, _unpack(wu_u[c])))
            hs.append((_rb(ga * _rb(jax.nn.sigmoid(ga))) * up).astype(bf16))
            due.append([hs[-1], ln1(0, c, ga, CFG['freload'])])
        hdn = jnp.concatenate(hs, axis=1)
        ys = []
        for c in range(NG):
            ys.append(_dot(gated(hdn, NF + c), _unpack(wd_u[c])))
            due.append([ln1(0, NF + c, ys[-1], CFG['freload'])] if NF + c < L // SUB else [])
        y = _rb(jnp.concatenate(ys, axis=1))
        rsel = jnp.where(lax.broadcasted_iota(i32, (SUB, 1), 0) == 0, m1, m2)
        y = _rb(y * _rb(jax.nn.sigmoid(rsel)))
        x2s = _rb(x1s + _rb(xs.astype(f32) + y))
        xns = _ln(x2s)

        @pl.when(li == CFG['nl'] - 1)
        def _():
            for s in range(NSEG):
                cp_out_seg(s).wait()

        blks = []
        for n, t in enumerate(toks):
            sg = t // L
            b0 = pl.multiple_of((t % L) // SUB * SUB, SUB)
            hb = pl.multiple_of((t % L) // SUB * (SUB // 2), SUB // 2)
            hit = row == (t % SUB)
            old = x_ref[sg, pl.ds(b0, SUB), :].astype(f32)
            x_ref[sg, pl.ds(b0, SUB), :] = jnp.where(hit, x2s[n:n + 1], old).astype(bf16)
            oldn = _unpack(xa_ref[pl.ds(hb, SUB // 2), :]).astype(f32)
            xa_ref[pl.ds(hb, SUB // 2), :] = _pack(jnp.where(row == t - b0, xns[n:n + 1], oldn))
            blks.append((sg, b0))

        @pl.when(li == CFG['nl'] - 1)
        def _():
            def cp_fix(n):
                sg, b0 = blks[n]
                return pltpu.make_async_copy(x_ref.at[sg, pl.ds(b0, SUB), :],
                                             out_hbm.at[sg, pl.ds(b0, SUB), :], sems.at[SEM_FIX])
            differ = (toks[0] // SUB) != (toks[1] // SUB)
            cp_fix(0).start()

            @pl.when(differ)
            def _():
                cp_fix(1).start()
                cp_fix(1).wait()
            cp_fix(0).wait()
        return carry

    lax.fori_loop(0, CFG['nl'], layer, 0)


@jax.jit
def pallas_interleave_layers__memory_aug_infini_attn__moe_arch_mod__prompt_kernel(
    A_x: jax.Array,
    A_wq: jax.Array,
    A_wk: jax.Array,
    A_wv: jax.Array,
    A_wo: jax.Array,
    A_beta: jax.Array,
    B_x: jax.Array,
    B_w_r: jax.Array,
    B_w_gate: jax.Array,
    B_w_up: jax.Array,
    B_w_down: jax.Array,
):
    del B_x
    qkv_bufs = [pltpu.VMEM((L // 2, 512), u32), pltpu.VMEM((72, L), u32)]
    scratch = [
        pltpu.VMEM((8 * CFG['zpad'], 128), u32),
        pltpu.VMEM((NSEG, L, D), bf16),
        pltpu.VMEM((3 * L // 2, D), u32),
        pltpu.VMEM((NSEG, L, D), f32),
        pltpu.VMEM((3 * NG, D, 128), bf16),
        pltpu.VMEM((NG, D, 128), bf16),
        pltpu.VMEM((NF, D, 128), bf16),
        pltpu.VMEM((NF, D, 128), bf16),
        pltpu.VMEM((NG, F, 128), bf16),
        pltpu.VMEM((64, 128), f32),
        pltpu.VMEM((32, 128), f32),
        pltpu.VMEM((NG, 144, 128), f32),
        pltpu.VMEM((CH, 128), f32),
        pltpu.VMEM((144, L), f32),
        pltpu.VMEM((128, L), f32), pltpu.VMEM((256, L), f32),
        pltpu.VMEM((384, L), f32), pltpu.VMEM((512, L), f32),
        pltpu.VMEM((64, L), u32), pltpu.VMEM((128, L), u32),
        pltpu.VMEM((192, L), u32), pltpu.VMEM((256, L), u32),
        *qkv_bufs, *qkv_bufs,
        pltpu.VMEM((NG * L // 2, 256), u32),
        pltpu.VMEM((L, D), u32),
        pltpu.VMEM((24, 128), f32),
        pltpu.VMEM((2, D), f32),
        pltpu.VMEM((8, 128), bf16),
        pltpu.VMEM((1, 32), bf16),
        pltpu.SemaphoreType.DMA((NSEM,)),
    ]
    out = pl.pallas_call(
        _kernel,
        out_shape=jax.ShapeDtypeStruct((NSEG, L, D), bf16),
        in_specs=[pl.BlockSpec(memory_space=pl.ANY)] * 10,
        out_specs=pl.BlockSpec(memory_space=pl.ANY),
        scratch_shapes=scratch,
        compiler_params=pltpu.CompilerParams(vmem_limit_bytes=100 * 2 ** 20),
    )(A_x.reshape(NSEG, L, D), A_wq, A_wk, A_wv, A_wo, A_beta.reshape(1, 32), B_w_r.reshape(8, 128),
      B_w_gate, B_w_up, B_w_down)
    return out.reshape(1, S, D)
```

```python
import jax
import jax.numpy as jnp
from jax import lax
import jax.experimental.pallas as pl
import jax.experimental.pallas.tpu as pltpu

bf16 = jnp.bfloat16
f32 = jnp.float32
u32 = jnp.uint32
i32 = jnp.int32

S = 2048
D = 1024
L = 512
NSEG = 4
NG = 8
F = 3584
CH = 64
SUB = 16
NEG = -1e30
QSCALE = (32 ** -0.5) * 1.4426950408889634
NT = (((1,), (1,)), ((), ()))

SEM_XC = 0
SEM_W0 = 4
SEM_X1 = 5
SEM_SM = 6
SEM_P = 7
NSEM = 11
SEM_OUT, SEM_FIX, SEM_FF, SEM_XN = 0, 1, 2, 3
NF = F // 128
PORDER = [(m, n) for m in range(4) for n in range(2)] + [(m, 2) for m in range(4)]

CFG = dict(
    tail=(128, 128, 128, 64, 32, 32), defer=128, mpad=2, glag=(0, 0, 0, 0, 0, 0), ffearly=1, pace3=1, rep={}, cnt={}, merge3=0, zpad=4, issue='abcdqksr vx', lnmode=0, nl=2, prewait=False, gp=2, pace=True, pace2=True, one=True, reload=True, chain=True, xfrac=0.0, freload=False, lag=0, fskip=0,
    pre='f ' * 16 + 'w x x x x Q3 ' + 'f x x x x ' * 7 + 'f',
    sched='M3 f p30 f n q2 v30 p31 f f v31 p32 f f m2 v32 p33 f f v33 p20 f f q1 v20 p21 f x f v21 p22 f x f '
          'm1 v22 p10 f x f q0 v10 p11 f x f u v11 m0 f p00 f f v00 F Q3',
    sched0='M3 f p30 f q2 v30 p31 f f v31 p32 f f x m2 v32 p33 f f x v33 p20 f f x q1 v20 p21 f f x '
           'v21 p22 f f x m1 v22 p10 f f x q0 v10 p11 f x f u v11 m0 f x p00 f f v00 F Q3',
    schedL='M3 f p30 f n q2 v30 p31 f f v31 p32 f f m2 v32 p33 f f v33 p20 f f q1 v20 p21 f x f v21 p22 f x f '
          'm1 v22 p10 f x f q0 v10 p11 f x f v11 m0 f p00 f f v00 F',
)


def _loop(name, n, body):
    rep = CFG['rep'].get(name, 1)
    n = CFG['cnt'].get(name, n)
    if n == 0:
        return 0
    if rep == 1:
        return lax.fori_loop(0, n, body, 0)
    return lax.fori_loop(0, n * rep, lambda i, c: body(i // rep, c), 0)


def _rb(x):
    return x.astype(bf16).astype(f32)


def _pack(x):
    return pltpu.bitcast(x.astype(bf16), u32)


def _unpack(u):
    return pltpu.bitcast(u, bf16)


def _phi(t):
    return jnp.where(t > 0, t + 1.0, jnp.exp(t))


def _dot(a, b):
    return jnp.dot(a, b, preferred_element_type=f32)


def _unskew(ps):
    shape, dt = next((p.shape, p.dtype) for p in ps if p is not None)
    c = lax.broadcasted_iota(i32, shape, 1) >> 5
    even = (c & 1) == 0
    lo = c < 2
    mid = jnp.logical_or(c == 1, c == 2)

    def sel(mask, a, b):
        if a is None and b is None:
            return None
        z = jnp.zeros(shape, dt)
        return jnp.where(mask, z if a is None else a, z if b is None else b)
    x0, x1 = sel(even, ps[0], ps[1]), sel(even, ps[1], ps[0])
    x2, x3 = sel(even, ps[2], ps[3]), sel(even, ps[3], ps[2])
    return [sel(lo, x0, x2), sel(mid, x1, x3), sel(lo, x2, x0), sel(mid, x3, x1)]


def _ln(x, mode=0):
    acc = x
    if CFG['chain']:
        acc = x[:, 0:128]
        for c in range(1, x.shape[1] // 128):
            acc = acc + x[:, 128 * c:128 * c + 128]
    m = jnp.sum(acc, axis=-1, keepdims=True) * (1.0 / D)
    if mode == 0:
        e = x - m
        v = jnp.sum(e * e, axis=-1, keepdims=True) * (1.0 / D)
        return e * lax.rsqrt(v + 1e-5)
    c = _rb(m)
    e = x - c
    v = jnp.sum(e * e, axis=-1, keepdims=True) * (1.0 / D) - (m - c) * (m - c)
    w = _rb(_rb(jnp.maximum(v, 0.0)) + 1e-5)
    den = _rb(w * lax.rsqrt(w))
    if mode == 2:
        return _rb(_rb(e) / den)
    return e * (1.0 / den)


def _rowsum(x, first=None):
    acc = x[:, 0:128] if first is None else first
    for c in range(1, x.shape[1] // 128):
        acc = acc + x[:, 128 * c:128 * c + 128]
    return jnp.sum(acc, axis=-1, keepdims=True)


def _stats(x):
    m = _rowsum(x) * (1.0 / D)
    v = jnp.maximum(_rowsum(x * x) * (1.0 / D) - m * m, 0.0)
    return m, lax.rsqrt(v + 1e-5)


def _kernel(x_hbm, wq_hbm, wk_hbm, wv_hbm, wo_hbm, beta_hbm, wr_hbm, wg_hbm, wu_hbm, wd_hbm,
            out_hbm,
            z_ref, x_ref, xb_ref, x1_ref, w_ref, wo_ref, wg_ref, wu_ref, wd_ref,
            gate_ref, bias_ref, m_ref, r_ref, nd_ref,
            s0_ref, s1_ref, s2_ref, s3_ref, p0_ref, p1_ref, p2_ref, p3_ref,
            qk0, vt0, qk1, vt1, o_ref, xa_ref, wrf_ref, mx_ref, wr_ref, beta_ref, sems):
    qkv = ((qk0, vt0), (qk1, vt1))
    s_refs = (s0_ref, s1_ref, s2_ref, s3_ref)
    p_refs = (p0_ref, p1_ref, p2_ref, p3_ref)
    xa_b, xb_b = xa_ref.bitcast(bf16), xb_ref.bitcast(bf16)
    w_u, wo_u, wg_u, wu_u, wd_u = (r.bitcast(u32) for r in (w_ref, wo_ref, wg_ref, wu_ref, wd_ref))

    def cp_x0(c):
        rows = pl.ds(pl.multiple_of(128 * c, 128), 128)
        return pltpu.make_async_copy(x_hbm.at[0, rows], x_ref.at[0, rows], sems.at[SEM_XC + c])

    def cp_x1():
        return pltpu.make_async_copy(x_hbm.at[1], x_ref.at[1], sems.at[SEM_X1])

    def cp_xn():
        return pltpu.make_async_copy(xa_ref.at[L // 2:L], xb_ref.at[0:L // 2], sems.at[SEM_XN])

    def cp_xr(g):
        r0 = pl.multiple_of(g * CH, CH)
        return pltpu.make_async_copy(x_hbm.at[2:NSEG, pl.ds(r0, CH), :],
                                     x_ref.at[2:NSEG, pl.ds(r0, CH), :], sems.at[SEM_P + g // 2])

    def cp_w(g, j):
        c0 = pl.multiple_of(g * 128, 128)
        src = (wq_hbm, wk_hbm, wv_hbm)[j]
        sem = (SEM_W0 + j // 2) if isinstance(g, int) and g == 0 else SEM_P + (g - 1) // 2
        return pltpu.make_async_copy(src.at[:, pl.ds(c0, 128)], w_ref.at[3 * g + j], sems.at[sem])

    def slabs(src, dst, n, sem):
        return [pltpu.make_async_copy(src.at[:, 128 * c:128 * c + 128], dst.at[c], sems.at[sem]) for c in range(n)]

    def cp_wo():
        return slabs(wo_hbm, wo_ref, NG, SEM_P + 3)

    def cp_small():
        return (pltpu.make_async_copy(beta_hbm, beta_ref, sems.at[SEM_SM]),
                pltpu.make_async_copy(wr_hbm, wr_ref, sems.at[SEM_SM]))

    def cp_ff():
        return (slabs(wg_hbm, wg_ref, NF, SEM_FF) + slabs(wu_hbm, wu_ref, NF, SEM_FF)
                + slabs(wd_hbm, wd_ref, NG, SEM_FF))

    def cp_out_seg(s):
        return pltpu.make_async_copy(x_ref.at[s], out_hbm.at[s], sems.at[SEM_OUT])

    def after(x, tok, frac):
        if tok is None or not CFG['pace']:
            return x
        r = 8 * int(frac * tok.shape[0] // 8)
        t = pltpu.bitcast(tok[r:r + 8, 0:128], u32) & z_ref[0:8, :]
        t = jnp.tile(t, (x.shape[0] // 8, x.shape[1] // 128))
        return pltpu.bitcast(pltpu.bitcast(x, u32) | t, x.dtype)

    def proj_items(s, nxt, g, par):
        xn_r, seg = (xa_ref, nxt) if isinstance(s, int) and s == 0 else (xb_ref, s - 1 + nxt)
        qk_r, vt_r = (r.bitcast(bf16) for r in qkv[par])
        part = {}

        def item(m, n, h):
            xn = _unpack(xn_r[pl.ds(pl.multiple_of(seg * (L // 2) + 64 * m, 64), 64), 512 * h:512 * h + 512])
            y = _dot(xn, _unpack(w_u[3 * g + n, 256 * h:256 * h + 256, :]))
            if h == 0:
                part[m, n] = y
                return y
            y = y + part.pop((m, n))
            rows = slice(128 * m, 128 * m + 128)
            if n == 0:
                qk_r[rows, 0:128] = (y * QSCALE).astype(bf16)
                qk_r[rows, 128:256] = _phi(y).astype(bf16)
            elif n == 1:
                qk_r[rows, 256:384] = y.astype(bf16)
                qk_r[rows, 384:512] = _phi(y).astype(bf16)
            else:
                vt_r[0:128, rows] = y.T.astype(bf16)
            return y
        return item

    def attn_items(g, par, seg, use_mem):
        qk_r, vt_r = qkv[par]
        st = {}

        def nd():
            ml = m_ref[g].astype(bf16)
            nd_ref[...] = lax.dot_general(ml, _unpack(qk_r[:, 128:256]), NT, preferred_element_type=f32)

        def upd():
            u = _dot(_unpack(vt_r[...]), _unpack(qk_r[:, 384:512]))
            r2 = lax.broadcasted_iota(i32, (144, 128), 0)
            c2 = lax.broadcasted_iota(i32, (144, 128), 1) >> 5
            keep = jnp.where(r2 < 128, r2 >> 5, r2 - 128) == c2
            u = jnp.where(keep, u, 0.0)
            m_ref[g] = (m_ref[g] + u) if use_mem else u

        def qk(i):
            lane = lax.broadcasted_iota(i32, (16, 128), 1) >> 5
            for be in (range(4) if i % 2 else range(3, -1, -1)):
                b = 4 * i + be
                n = 32 * (b + 1)
                qu = qk_r[16 * b:16 * b + 16, 0:128]
                wq = _unpack(jnp.concatenate(
                    [jnp.where(lane == (c - be) % 4, qu, jnp.uint32(0)) for c in range(4)], axis=0))
                s = lax.dot_general(_unpack(qk_r[0:n // 2, 256:384]), wq, NT, preferred_element_type=f32)
                cols = slice(128 * be, 128 * be + 128)
                if b > 0:
                    s_refs[i][0:n - 32, cols] = s[0:n - 32]
                s_refs[i][n - 32:n, cols] = s[n - 32:n] + bias_ref[...]

        def mx(i, mode='m'):
            for be in range(4):
                if mode == 'load':
                    st[i, 'm', be] = mx_ref[4 * i + be:4 * i + be + 1, :]
                    continue
                n = 32 * (4 * i + be + 1)
                sv = s_refs[i][0:n, 128 * be:128 * be + 128]
                m = jnp.max(jnp.max(sv.reshape(n // 8, 8, 128), axis=0), axis=0, keepdims=True)
                if mode == 'store':
                    mx_ref[4 * i + be:4 * i + be + 1, :] = m
                else:
                    st[i, 'm', be] = m

        def pr(i, t, tok):
            ps = []
            for be in range(4):
                n = 128 if t < i else 32 * (be + 1)
                m8 = after(jnp.broadcast_to(st[i, 'm', be], (8, 128)), tok, be / 4)
                p = jnp.exp2(s_refs[i][128 * t:128 * t + n, 128 * be:128 * be + 128].reshape(n // 8, 8, 128) - m8)
                ls = jnp.sum(p, axis=0)
                p = p.reshape(n, 128)
                st[i, 'l', be] = ls if t == 0 else st[i, 'l', be] + ls
                p_refs[i].bitcast(bf16)[128 * t:128 * t + n, 128 * be:128 * be + 128] = p.astype(bf16)

        def pv(i, t):
            ps = [p_refs[i][64 * t:64 * t + (64 if t < i else 16 * (be + 1)), 128 * be:128 * be + 128]
                  for be in range(4)]
            if t < i:
                ts = _unskew(ps)
            else:
                blk = [_unskew([ps[be][16 * u:16 * u + 16] if be >= u else None for be in range(4)])
                       for u in range(4)]
                ts = [jnp.concatenate([blk[u][j] for u in range(4)], axis=0) for j in range(4)]
            for j in range(4):
                o = _dot(_unpack(vt_r[16 * j:16 * j + 16, 128 * t:128 * t + 128]), _unpack(ts[j]))
                st[i, 'o', j] = o if t == 0 else st[i, 'o', j] + o

        def fin(i):
            ls = _unskew([jnp.sum(st.pop((i, 'l', be)), axis=0, keepdims=True) for be in range(4)])
            parts = []
            for j in range(4):
                gt = gate_ref[pl.ds(4 * g + j, 1), :]
                omg = gate_ref[pl.ds(32 + 4 * g + j, 1), :]
                o = st.pop((i, 'o', j)) * (omg / ls[j])
                if j > 0:
                    o = pltpu.roll(o, 128 - 32 * j, 1)
                if use_mem:
                    den = nd_ref[128 + j:129 + j, 128 * i:128 * i + 128] + 1e-6
                    o = o + nd_ref[32 * j:32 * j + 32, 128 * i:128 * i + 128] * (gt / den)
                parts.append(o)
            ot = jnp.concatenate(parts, axis=0)
            o_ref.bitcast(bf16)[pl.ds(pl.multiple_of((seg % 2 * 4 + g // 2) * L + 128 * i, 128), 128),
                                128 * par:128 * par + 128] = ot.T.astype(bf16)

        def ex(kind, i, t, tok):
            if kind in 'ep':
                pr(i, t, tok)
            if kind in 'ev':
                pv(i, t)
                if t == i:
                    fin(i)
        return nd, upd, qk, mx, ex

    def ln1(seg, r, tok=None, reload=True):
        r0 = pl.multiple_of(r * SUB, SUB)
        x = x_ref[seg, pl.ds(r0, SUB), :].astype(f32)
        if tok is not None:
            x = jnp.concatenate([after(x[:, 0:128], tok, CFG['xfrac']), x[:, 128:]], axis=1)
        if CFG['one']:
            m, rs = _stats(x)
            if CFG['reload'] and reload:
                mx_ref[16:24, :] = jnp.broadcast_to(m[0:8], (8, 128))
                x = x_ref[seg, pl.ds(r0, SUB), :].astype(f32)
            xn = ((x - m) * rs).astype(bf16)
        else:
            xn = _ln(x).astype(bf16)
        if seg < 2:
            xa_b[pl.ds(pl.multiple_of(seg * L + r0, SUB), SUB), :] = xn
        else:
            xb_b[pl.ds(pl.multiple_of((seg - 1) * L + r0, SUB), SUB), :] = xn
        return xn

    def oproj(seg, r0, rows, n, k0=0, k1=NG, deps=()):
        h0 = pl.multiple_of(r0 // 2, rows // 2)
        r0 = pl.multiple_of(r0, rows)
        lhs = jnp.concatenate(
            [o_ref[pl.ds(pl.multiple_of((seg % 2 * 4 + p) * (L // 2) + h0, rows // 2), rows // 2), :]
             for p in range(k0 // 2, k1 // 2)], axis=1)
        for d in deps:
            top = jnp.concatenate([after(lhs[0:8, 0:128], d, 0.0), lhs[0:8, 128:]], axis=1)
            lhs = jnp.concatenate([top, lhs[8:]], axis=0)
        lhs = _unpack(lhs)
        y = _dot(lhs, _unpack(wo_u[n, 64 * k0:64 * k1, :]))
        cols = slice(128 * n, 128 * n + 128)
        if k0 > 0:
            y = y + x1_ref[seg, pl.ds(r0, rows), cols]
        if k1 == NG:
            y = _rb(x_ref[seg, pl.ds(r0, rows), cols].astype(f32) + y)
        x1_ref[seg, pl.ds(r0, rows), cols] = y
        return y

    def ln2(seg, c, t, tok=None, defer=False):
        r0 = pl.multiple_of(c * CH + t * SUB, SUB)
        lane = lax.broadcasted_iota(i32, (SUB, 128), 1)
        x1 = x1_ref[seg, pl.ds(r0, SUB), :]
        if tok is not None and CFG['pace2']:
            x1 = jnp.concatenate([after(x1[:, 0:128], tok, CFG['xfrac']), x1[:, 128:]], axis=1)
        if CFG['one']:
            m, rs = _stats(x1)
            r = _rb((_rowsum(x1 * jnp.tile(wrf_ref[0:8, :], (2, 1))) - m * jnp.tile(wrf_ref[8:16, 0:128], (2, 1))) * rs)
        else:
            xn2 = _ln(x1, CFG['lnmode'])
            r = _rb(jnp.sum(xn2 * wrf_ref[0:1, :], axis=-1, keepdims=True))
        r_ref[SUB * t:SUB * t + SUB, :] = jnp.where(lane == seg * NG + c, r, r_ref[SUB * t:SUB * t + SUB, :])

        def fin(tok2=None):
            if CFG['one']:
                xr = x1_ref[seg, pl.ds(r0, SUB), :] if CFG['reload'] else x1
                if tok2 is not None:
                    xr = jnp.concatenate([after(xr[:, 0:128], tok2, CFG['xfrac']), xr[:, 128:]], axis=1)
                x2 = xr * (1.0 + rs) - m * rs
            else:
                x2 = x1 + xn2
            x_ref[seg, pl.ds(r0, SUB), :] = x2.astype(bf16)
        if defer:
            return r, fin
        fin()
        return r, None

    def group(s, g, par, last=False):
        kind = s if isinstance(s, int) else 1
        nd, upd, qk, mx, ex = attn_items(g, par, s, kind > 0)
        fill = []
        extra = []
        if kind > 0:
            for n in range(NG):
                fill.append((128, lambda n=n: oproj(s - 1, g * CH, CH, n)))
            extra = [lambda tok, t=t: ln2(s - 1, g, t, tok) for t in range(CH // SUB)]
        else:
            extra = [lambda tok, seg=seg, t=t: ln1(seg, g * (CH // SUB) + t, tok)
                     for seg in range(2, NSEG) for t in range(CH // SUB)]
        if not last:
            gn = g + 1
            pj = proj_items(s, gn // NG, gn % NG, 1 - par)
            for m, n in PORDER:
                for h in range(2):
                    fill.append((128, lambda m=m, n=n, h=h: pj(m, n, h)))
        else:
            for m in range(4):
                for n in range(NG):
                    fill.append((128, lambda m=m, n=n: oproj(s, 128 * m, 128, n, 0, 4)))
        sched = CFG['sched0' if kind == 0 else 'schedL' if last else 'sched'].split()
        y = None
        for tok in sched:
            if tok == 'f':
                y = fill.pop(0)[1]()
            elif tok == 'F':
                while fill:
                    fill.pop(0)[1]()
            elif tok == 'x':
                extra.pop(0)(y)
            elif tok == 'n':
                nd()
            elif tok == 'u':
                if kind < NSEG - 1:
                    upd()
            elif tok[0] == 'q':
                qk(int(tok[1]))
            elif tok[0] == 'Q':
                nxt = attn_items(None, 1 - par, None, None)
                nxt[2](int(tok[1]))
                nxt[3](int(tok[1]), 'store')
            elif tok[0] == 'M':
                mx(int(tok[1]), 'load')
            elif tok[0] == 'm':
                mx(int(tok[1]))
            else:
                ex(tok[0], int(tok[1]), int(tok[2]), y)
        for it in fill:
            it[1]()
        for e in extra:
            e(None)

    early = {'a': cp_x0(0), 'b': cp_x0(1), 'c': cp_x0(2), 'd': cp_x0(3), 'q': cp_w(0, 0), 'k': cp_w(0, 1),
             'v': cp_w(0, 2), 'x': cp_x1(), 's': cp_small()[0], 'r': cp_small()[1]}
    issue = CFG['issue'].split()
    for k in issue[0]:
        early[k].start()

    z_ref[0:8, :] = jnp.zeros((8, 128), u32)
    ones = jnp.full((8, 512), 0x3F803F80, u32)
    vt0[64:72, :] = ones
    vt1[64:72, :] = ones
    bias_ref[...] = jnp.where(lax.broadcasted_iota(i32, (32, 128), 0)
                              <= (lax.broadcasted_iota(i32, (32, 128), 1) & 31), 0.0, NEG)

    def ln0_body(c, carry):
        cp_x0(c).wait()
        for n in range(1, len(issue)):
            @pl.when(c == n - 1)
            def _():
                for k in issue[n].strip('-'):
                    early[k].start()
        for t in range(128 // SUB):
            ln1(0, c * (128 // SUB) + t)
        return carry
    lax.fori_loop(0, 4, ln0_body, 0)
    for g in range(1, NG):
        for j in range(3):
            cp_w(g, j).start()
        cp_xr(g - 1).start()
    cp_xr(NG - 1).start()
    for cp in cp_wo():
        cp.start()

    for cp in cp_small():
        cp.wait()
    wr = wr_ref[...].astype(f32)
    for c in range(D // 128):
        wrf_ref[0:8, 128 * c:128 * c + 128] = jnp.broadcast_to(wr[c:c + 1, :], (8, 128))
    wrf_ref[8:16, :] = jnp.broadcast_to(jnp.sum(wr, axis=(0, 1), keepdims=True), (8, D))
    gl = _rb(jax.nn.sigmoid(beta_ref[...].astype(f32)))
    hr = lax.broadcasted_iota(i32, (32, 32), 0)
    hc = lax.broadcasted_iota(i32, (32, 32), 1)
    gcol = jnp.sum(jnp.where(hr == hc, gl, 0.0), axis=1, keepdims=True)
    gate_ref[0:32, :] = jnp.broadcast_to(gcol, (32, 128))
    gate_ref[32:64, :] = jnp.broadcast_to(_rb(1.0 - gcol), (32, 128))
    for j in range(2):
        cp_w(0, j).wait()
    if CFG['prewait']:
        for g in range(NG):
            cp_xr(g).wait()
            for j in range(3 * (g > 0)):
                cp_w(g, j).wait()
        for cp in cp_wo():
            cp.wait()

    def layer(li, carry):
        first = li == 0
        r_ref[...] = jnp.full((CH, 128), -jnp.inf, f32)
        pj = proj_items(0, 0, 0, 0)
        fill = [(m, n, h) for m, n in PORDER for h in range(2)]
        extra = list(range(L // SUB))
        y = None
        for tok in CFG['pre'].split():
            if tok == 'f':
                y = pj(*fill.pop(0))
            elif tok == 'x':
                ln1(1, extra.pop(0), y)
            elif tok == 'w':
                @pl.when(first)
                def _():
                    cp_w(0, 2).wait()
                    cp_x1().wait()
                y = None
            else:
                nxt = attn_items(None, 0, None, None)
                nxt[2](int(tok[1]))
                nxt[3](int(tok[1]), 'store')
        assert not fill and not extra
        cp_xn().start()

        def pair(s, p, last=False):
            for par in range(2):
                group(s, 2 * p + par, par, last and par == 1)

        def seg0(p, c2):
            if not CFG['prewait']:
                @pl.when(first)
                def _():
                    for par in range(2):
                        cp_xr(2 * p + par).wait()
                    for j in range(3):
                        cp_w(2 * p + 1, j).wait()

                    @pl.when(p < NG // 2 - 1)
                    def _():
                        for j in range(3):
                            cp_w(jnp.minimum(2 * p + 2, NG - 2), j).wait()

                    @pl.when(p == NG // 2 - 1)
                    def _():
                        for cp in cp_wo():
                            cp.wait()
            pair(0, p)
            return c2
        _loop('s0', NG // 2, seg0)
        cp_xn().wait()

        @pl.when(first)
        def _():
            for cp in cp_ff():
                cp.start()

        def mid(t, c2):
            pair(1 + t // (NG // 2), t % (NG // 2))
            return c2
        _loop('s1', NG + (NG // 2 - 1) * CFG['merge3'], mid)

        def wait_ff():
            @pl.when(first)
            def _():
                for cp in cp_ff():
                    cp.wait()

        @pl.when(li == CFG['nl'] - 1)
        def _():
            cp_out_seg(0).start()
            cp_out_seg(1).start()

        def seg3(p, c2):
            pair(NSEG - 1, p)
            return c2
        if not CFG['merge3']:
            _loop('s3', NG // 2 - 1, seg3)
        if CFG['ffearly']:
            wait_ff()
        pair(NSEG - 1, NG // 2 - 1, last=True)

        s = NSEG - 1
        pend = []
        r0 = L
        late, gate, step, glag = [], {}, 0, 0
        for rows, nlag in zip(CFG['tail'], CFG['glag']):
            r0 -= rows
            for n in range(NG):
                y = oproj(s, r0, rows, n, 4, NG, gate.pop(step, ()))
                if pend:
                    r, fin = pend.pop(0)(y)
                    late.append(fin)
                    if glag:
                        gate.setdefault(step + glag, []).append(r)
                step += 1
            pend = [lambda tok, r=r: ln2(s, r // CH, r % CH // SUB, tok, r < CFG['defer'])
                    for r in range(r0, r0 + rows, SUB)]
            glag = nlag
        assert r0 == 0
        late = [e for e in late + [e(None)[1] for e in pend] if e is not None]

        def start_out():
            cp_out_seg(NSEG - 2).start()
            cp_out_seg(NSEG - 1).start()
        if not late:
            start_out()

        rm = r_ref[...]
        rb = pltpu.bitcast(jnp.where(rm == 0.0, 0.0, rm), i32)
        lane = lax.broadcasted_iota(i32, (CH, 128), 1)
        base = jnp.where(lane < S // CH, (1 << 29) + S - 1 - lane * CH - lax.broadcasted_iota(i32, (CH, 128), 0), 0)
        mono = rb ^ ((rb >> 31) | jnp.int32(-2 ** 31))
        key = pltpu.bitcast(base + (lax.shift_right_logical(mono, 5) & 0x07FFF800), f32)
        k1 = jnp.max(key, axis=(0, 1), keepdims=True)
        k2 = jnp.max(jnp.where(key == k1, 0.0, key), axis=(0, 1), keepdims=True)
        toks = [jnp.clip(jnp.max((S - 1 - (pltpu.bitcast(k, i32) & (S - 1))).astype(f32)).astype(i32), 0, S - 1)
                for k in (k1, k2)]

        if not CFG['ffearly']:
            wait_ff()

        row = lax.broadcasted_iota(i32, (SUB, D), 0)
        x1s = jnp.concatenate([x1_ref[t >> 9, pl.ds(pl.multiple_of(t & (L - 8), 8), 8), :] for t in toks], axis=0)
        ms, rss = _stats(x1s)
        xs = ((x1s - ms) * rss).astype(bf16)
        lag, due = CFG['lag'], []

        def gated(lhs, c):
            u = pltpu.bitcast(lhs, u32)
            if c < lag or lag == 0:
                return lhs
            t = u[:, 0:128]
            for d in due[c - lag]:
                t = t | (pltpu.bitcast(d[:, d.shape[1] - 128:], u32) & z_ref[0:8, :])
            return pltpu.bitcast(jnp.concatenate([t, u[:, 128:]], axis=1), bf16)
        hs = []
        for c in range(NF):
            xc = gated(xs, c)
            if c >= NF - CFG['fskip']:
                hs.append(hs[0])
                due.append([ln1(0, c, ga, CFG['freload'])])
                continue
            ga = _rb(_dot(xc, _unpack(wg_u[c])))
            up = _rb(_dot(xc, _unpack(wu_u[c])))
            hs.append((_rb(ga * _rb(jax.nn.sigmoid(ga))) * up).astype(bf16))
            due.append([hs[-1], ln1(0, c, ga, CFG['freload'])])
            if late:
                late.pop(0)(ga)
                if not late:
                    start_out()
        hdn = jnp.concatenate(hs, axis=1)
        ys = []
        for c in range(NG):
            ys.append(_dot(gated(hdn, NF + c), _unpack(wd_u[c])))
            due.append([ln1(0, NF + c, ys[-1], CFG['freload'])] if NF + c < L // SUB else [])
        y = _rb(jnp.concatenate(ys, axis=1))
        ksel = pltpu.bitcast(jnp.where(lax.broadcasted_iota(i32, (SUB, 128), 0) < 8, k1, k2), i32)
        hi = (ksel << 5) & -65536
        rsel = pltpu.bitcast(jnp.where(hi < 0, hi ^ jnp.int32(-2 ** 31), ~hi & -65536), f32)[:, 0:1]
        y = _rb(y * _rb(jax.nn.sigmoid(rsel)))
        x2s = _rb(x1s + _rb(xs.astype(f32) + y))
        ms, rss = _stats(x2s)
        xns = (x2s - ms) * rss

        @pl.when(li == CFG['nl'] - 1)
        def _():
            for s in range(NSEG - 2):
                cp_out_seg(s).wait()
        for s in range(NSEG - 2, NSEG):
            cp_out_seg(s).wait()

        blks = []
        for n, t in enumerate(toks):
            sg = t >> 9
            b0 = pl.multiple_of(t & (L - SUB), SUB)
            hb = pl.multiple_of((t & (L - SUB)) >> 1, SUB // 2)
            hit = row == (t & (SUB - 1))
            old = x_ref[sg, pl.ds(b0, SUB), :].astype(f32)
            x_ref[sg, pl.ds(b0, SUB), :] = jnp.where(hit, jnp.tile(x2s[8 * n:8 * n + 8], (2, 1)), old).astype(bf16)
            oldn = _unpack(xa_ref[pl.ds(hb, SUB // 2), :]).astype(f32)
            xa_ref[pl.ds(hb, SUB // 2), :] = _pack(jnp.where(row == t - b0, jnp.tile(xns[8 * n:8 * n + 8], (2, 1)), oldn))
            blks.append((sg, b0))

        @pl.when(li == CFG['nl'] - 1)
        def _():
            def cp_fix(n):
                sg, b0 = blks[n]
                return pltpu.make_async_copy(x_ref.at[sg, pl.ds(b0, SUB), :],
                                             out_hbm.at[sg, pl.ds(b0, SUB), :], sems.at[SEM_FIX])
            differ = (toks[0] >> 4) != (toks[1] >> 4)
            cp_fix(0).start()

            @pl.when(differ)
            def _():
                cp_fix(1).start()
                cp_fix(1).wait()
            cp_fix(0).wait()
        return carry

    lax.fori_loop(0, CFG['nl'], layer, 0)


@jax.jit
def pallas_interleave_layers__memory_aug_infini_attn__moe_arch_mod__prompt_kernel(
    A_x: jax.Array,
    A_wq: jax.Array,
    A_wk: jax.Array,
    A_wv: jax.Array,
    A_wo: jax.Array,
    A_beta: jax.Array,
    B_x: jax.Array,
    B_w_r: jax.Array,
    B_w_gate: jax.Array,
    B_w_up: jax.Array,
    B_w_down: jax.Array,
):
    del B_x
    qkv_bufs = [pltpu.VMEM((L // 2, 512), u32), pltpu.VMEM((72, L), u32)]
    scratch = [
        pltpu.VMEM((8 * CFG['zpad'], 128), u32),
        pltpu.VMEM((NSEG, L, D), bf16),
        pltpu.VMEM((3 * L // 2, D), u32),
        pltpu.VMEM((NSEG, L, D), f32),
        pltpu.VMEM((3 * NG, D, 128), bf16),
        pltpu.VMEM((NG, D, 128), bf16),
        pltpu.VMEM((NF, D, 128), bf16),
        pltpu.VMEM((NF, D, 128), bf16),
        pltpu.VMEM((NG, F, 128), bf16),
        pltpu.VMEM((64, 128), f32),
        pltpu.VMEM((32, 128), f32),
        pltpu.VMEM((NG, 144, 128), f32),
        pltpu.VMEM((CH, 128), f32),
        pltpu.VMEM((144, L), f32),
        pltpu.VMEM((128, L), f32), pltpu.VMEM((256, L), f32),
        pltpu.VMEM((384, L), f32), pltpu.VMEM((512, L), f32),
        pltpu.VMEM((64, L), u32), pltpu.VMEM((128, L), u32),
        pltpu.VMEM((192, L), u32), pltpu.VMEM((256, L), u32),
        *qkv_bufs, *qkv_bufs,
        pltpu.VMEM((NG * L // 2, 256), u32),
        pltpu.VMEM((L, D), u32),
        pltpu.VMEM((16, D), f32),
        pltpu.VMEM((24 + 8 * CFG['mpad'], 128), f32),
        pltpu.VMEM((8, 128), bf16),
        pltpu.VMEM((1, 32), bf16),
        pltpu.SemaphoreType.DMA((NSEM,)),
    ]
    out = pl.pallas_call(
        _kernel,
        out_shape=jax.ShapeDtypeStruct((NSEG, L, D), bf16),
        in_specs=[pl.BlockSpec(memory_space=pl.ANY)] * 10,
        out_specs=pl.BlockSpec(memory_space=pl.ANY),
        scratch_shapes=scratch,
        compiler_params=pltpu.CompilerParams(vmem_limit_bytes=100 * 2 ** 20),
    )(A_x.reshape(NSEG, L, D), A_wq, A_wk, A_wv, A_wo, A_beta.reshape(1, 32), B_w_r.reshape(8, 128),
      B_w_gate, B_w_up, B_w_down)
    return out.reshape(1, S, D)
```

```python
import jax
import jax.numpy as jnp
from jax import lax
import jax.experimental.pallas as pl
import jax.experimental.pallas.tpu as pltpu

bf16 = jnp.bfloat16
f32 = jnp.float32
u32 = jnp.uint32
i32 = jnp.int32

S = 2048
D = 1024
L = 512
NSEG = 4
NG = 8
F = 3584
CH = 64
SUB = 16
NEG = -1e30
QSCALE = (32 ** -0.5) * 1.4426950408889634
NT = (((1,), (1,)), ((), ()))

SEM_XC = 0
SEM_W0 = 4
SEM_X1 = 5
SEM_SM = 6
SEM_P = 7
NSEM = 11
SEM_OUT, SEM_FIX, SEM_FF, SEM_XN = 0, 1, 2, 3
NF = F // 128
PORDER = [(m, n) for m in range(4) for n in range(2)] + [(m, 2) for m in range(4)]

CFG = dict(
    tail=(128, 128, 128, 64, 32, 32), defer=128, dlag=2, kc=4, xln=8, alag=0, n1=32, vearly=1, mpad=2, glag=(0, 0, 0, 0, 0, 0), ffearly=1, pace3=1, rep={}, cnt={}, merge3=0, zpad=4, issue='abcdqkvsr x', lnmode=0, nl=2, prewait=False, gp=2, pace=True, pace2=True, one=True, reload=True, chain=True, xfrac=0.0, freload=False, lag=0, fskip=0,
    pre='f ' * 18 + 'Q3 ' + 'f ' * 6 + 'W',
    sched='M3 f p30 f n q2 v30 p31 f f v31 p32 f f m2 v32 p33 f f v33 p20 f f q1 v20 p21 f x f v21 p22 f x f '
          'm1 v22 p10 f x f q0 v10 p11 f x f u v11 m0 f p00 f f v00 F Q3',
    sched0='M3 f p30 f q2 v30 p31 f f v31 p32 f f x m2 v32 p33 f f x v33 p20 f f x q1 v20 p21 f f x '
           'v21 p22 f f x m1 v22 p10 f f x q0 v10 p11 f x f u v11 m0 f x p00 f f v00 F Q3',
    schedL='M3 f p30 f n q2 v30 p31 f f v31 p32 f f m2 v32 p33 f f v33 p20 f f q1 v20 p21 f x f v21 p22 f x f '
          'm1 v22 p10 f x f q0 v10 p11 f x f v11 m0 f p00 f f v00 F',
)


def _loop(name, n, body):
    rep = CFG['rep'].get(name, 1)
    n = CFG['cnt'].get(name, n)
    if n == 0:
        return 0
    if rep == 1:
        return lax.fori_loop(0, n, body, 0)
    return lax.fori_loop(0, n * rep, lambda i, c: body(i // rep, c), 0)


def _rb(x):
    return x.astype(bf16).astype(f32)


def _pack(x):
    return pltpu.bitcast(x.astype(bf16), u32)


def _unpack(u):
    return pltpu.bitcast(u, bf16)


def _phi(t):
    return jnp.where(t > 0, t + 1.0, jnp.exp(t))


def _dot(a, b):
    return jnp.dot(a, b, preferred_element_type=f32)


def _unskew(ps):
    shape, dt = next((p.shape, p.dtype) for p in ps if p is not None)
    c = lax.broadcasted_iota(i32, shape, 1) >> 5
    even = (c & 1) == 0
    lo = c < 2
    mid = jnp.logical_or(c == 1, c == 2)

    def sel(mask, a, b):
        if a is None and b is None:
            return None
        z = jnp.zeros(shape, dt)
        return jnp.where(mask, z if a is None else a, z if b is None else b)
    x0, x1 = sel(even, ps[0], ps[1]), sel(even, ps[1], ps[0])
    x2, x3 = sel(even, ps[2], ps[3]), sel(even, ps[3], ps[2])
    return [sel(lo, x0, x2), sel(mid, x1, x3), sel(lo, x2, x0), sel(mid, x3, x1)]


def _ln(x, mode=0):
    acc = x
    if CFG['chain']:
        acc = x[:, 0:128]
        for c in range(1, x.shape[1] // 128):
            acc = acc + x[:, 128 * c:128 * c + 128]
    m = jnp.sum(acc, axis=-1, keepdims=True) * (1.0 / D)
    if mode == 0:
        e = x - m
        v = jnp.sum(e * e, axis=-1, keepdims=True) * (1.0 / D)
        return e * lax.rsqrt(v + 1e-5)
    c = _rb(m)
    e = x - c
    v = jnp.sum(e * e, axis=-1, keepdims=True) * (1.0 / D) - (m - c) * (m - c)
    w = _rb(_rb(jnp.maximum(v, 0.0)) + 1e-5)
    den = _rb(w * lax.rsqrt(w))
    if mode == 2:
        return _rb(_rb(e) / den)
    return e * (1.0 / den)


def _rowsum(x, first=None):
    acc = x[:, 0:128] if first is None else first
    for c in range(1, x.shape[1] // 128):
        acc = acc + x[:, 128 * c:128 * c + 128]
    return jnp.sum(acc, axis=-1, keepdims=True)


def _stats(x):
    m = _rowsum(x) * (1.0 / D)
    v = jnp.maximum(_rowsum(x * x) * (1.0 / D) - m * m, 0.0)
    return m, lax.rsqrt(v + 1e-5)


def _kernel(x_hbm, wq_hbm, wk_hbm, wv_hbm, wo_hbm, beta_hbm, wr_hbm, wg_hbm, wu_hbm, wd_hbm,
            out_hbm,
            z_ref, x_ref, xb_ref, x1_ref, w_ref, wo_ref, wg_ref, wu_ref, wd_ref,
            gate_ref, bias_ref, m_ref, r_ref, nd_ref,
            s0_ref, s1_ref, s2_ref, s3_ref, p0_ref, p1_ref, p2_ref, p3_ref,
            qk0, vt0, qk1, vt1, o_ref, xa_ref, wrf_ref, mx_ref, wr_ref, beta_ref, sems):
    qkv = ((qk0, vt0), (qk1, vt1))
    s_refs = (s0_ref, s1_ref, s2_ref, s3_ref)
    p_refs = (p0_ref, p1_ref, p2_ref, p3_ref)
    xa_b, xb_b = xa_ref.bitcast(bf16), xb_ref.bitcast(bf16)
    w_u, wo_u, wg_u, wu_u, wd_u = (r.bitcast(u32) for r in (w_ref, wo_ref, wg_ref, wu_ref, wd_ref))

    def cp_x0(c):
        rows = pl.ds(pl.multiple_of(128 * c, 128), 128)
        return pltpu.make_async_copy(x_hbm.at[0, rows], x_ref.at[0, rows], sems.at[SEM_XC + c])

    def cp_x1():
        return pltpu.make_async_copy(x_hbm.at[1], x_ref.at[1], sems.at[SEM_X1])

    def cp_xn():
        return pltpu.make_async_copy(xa_ref.at[L // 2:L], xb_ref.at[0:L // 2], sems.at[SEM_XN])

    def cp_xr(g):
        r0 = pl.multiple_of(g * CH, CH)
        return pltpu.make_async_copy(x_hbm.at[2:NSEG, pl.ds(r0, CH), :],
                                     x_ref.at[2:NSEG, pl.ds(r0, CH), :], sems.at[SEM_P + g // 2])

    def cp_w(g, j):
        c0 = pl.multiple_of(g * 128, 128)
        src = (wq_hbm, wk_hbm, wv_hbm)[j]
        sem = (SEM_W0 + j // 2 * (1 - CFG['vearly'])) if isinstance(g, int) and g == 0 else SEM_P + (g - 1) // 2
        return pltpu.make_async_copy(src.at[:, pl.ds(c0, 128)], w_ref.at[3 * g + j], sems.at[sem])

    def slabs(src, dst, n, sem):
        return [pltpu.make_async_copy(src.at[:, 128 * c:128 * c + 128], dst.at[c], sems.at[sem]) for c in range(n)]

    def cp_wo():
        return slabs(wo_hbm, wo_ref, NG, SEM_P + 3)

    def cp_small():
        return (pltpu.make_async_copy(beta_hbm, beta_ref, sems.at[SEM_SM]),
                pltpu.make_async_copy(wr_hbm, wr_ref, sems.at[SEM_SM]))

    def cp_ff():
        return (slabs(wg_hbm, wg_ref, NF, SEM_FF) + slabs(wu_hbm, wu_ref, NF, SEM_FF)
                + slabs(wd_hbm, wd_ref, NG, SEM_FF))

    def cp_out_seg(s):
        return pltpu.make_async_copy(x_ref.at[s], out_hbm.at[s], sems.at[SEM_OUT])

    def after(x, tok, frac):
        if tok is None or not CFG['pace']:
            return x
        r = 8 * int(frac * tok.shape[0] // 8)
        t = pltpu.bitcast(tok[r:r + 8, 0:128], u32) & z_ref[0:8, :]
        t = jnp.tile(t, (x.shape[0] // 8, x.shape[1] // 128))
        return pltpu.bitcast(pltpu.bitcast(x, u32) | t, x.dtype)

    def proj_items(s, nxt, g, par):
        xn_r, seg = (xa_ref, nxt) if isinstance(s, int) and s == 0 else (xb_ref, s - 1 + nxt)
        qk_r, vt_r = (r.bitcast(bf16) for r in qkv[par])
        part = {}

        def item(m, n, h):
            xn = _unpack(xn_r[pl.ds(pl.multiple_of(seg * (L // 2) + 64 * m, 64), 64), 512 * h:512 * h + 512])
            y = _dot(xn, _unpack(w_u[3 * g + n, 256 * h:256 * h + 256, :]))
            if h == 0:
                part[m, n] = y
                return y
            y = y + part.pop((m, n))
            rows = slice(128 * m, 128 * m + 128)
            if n == 0:
                qk_r[rows, 0:128] = (y * QSCALE).astype(bf16)
                qk_r[rows, 128:256] = _phi(y).astype(bf16)
            elif n == 1:
                qk_r[rows, 256:384] = y.astype(bf16)
                qk_r[rows, 384:512] = _phi(y).astype(bf16)
            else:
                vt_r[0:128, rows] = y.T.astype(bf16)
            return y
        return item

    def attn_items(g, par, seg, use_mem):
        qk_r, vt_r = qkv[par]
        st = {}

        def nd():
            ml = m_ref[g].astype(bf16)
            nd_ref[...] = lax.dot_general(ml, _unpack(qk_r[:, 128:256]), NT, preferred_element_type=f32)

        def upd():
            u = _dot(_unpack(vt_r[...]), _unpack(qk_r[:, 384:512]))
            r2 = lax.broadcasted_iota(i32, (144, 128), 0)
            c2 = lax.broadcasted_iota(i32, (144, 128), 1) >> 5
            keep = jnp.where(r2 < 128, r2 >> 5, r2 - 128) == c2
            u = jnp.where(keep, u, 0.0)
            m_ref[g] = (m_ref[g] + u) if use_mem else u

        def qk(i):
            lane = lax.broadcasted_iota(i32, (16, 128), 1) >> 5
            for be in (range(4) if i % 2 else range(3, -1, -1)):
                b = 4 * i + be
                n = 32 * (b + 1)
                qu = qk_r[16 * b:16 * b + 16, 0:128]
                wq = _unpack(jnp.concatenate(
                    [jnp.where(lane == (c - be) % 4, qu, jnp.uint32(0)) for c in range(4)], axis=0))
                s = lax.dot_general(_unpack(qk_r[0:n // 2, 256:384]), wq, NT, preferred_element_type=f32)
                cols = slice(128 * be, 128 * be + 128)
                if b > 0:
                    s_refs[i][0:n - 32, cols] = s[0:n - 32]
                s_refs[i][n - 32:n, cols] = s[n - 32:n] + bias_ref[...]

        def mx(i, mode='m'):
            for be in range(4):
                if mode == 'load':
                    st[i, 'm', be] = mx_ref[4 * i + be:4 * i + be + 1, :]
                    continue
                n = 32 * (4 * i + be + 1)
                sv = s_refs[i][0:n, 128 * be:128 * be + 128]
                m = jnp.max(jnp.max(sv.reshape(n // 8, 8, 128), axis=0), axis=0, keepdims=True)
                if mode == 'store':
                    mx_ref[4 * i + be:4 * i + be + 1, :] = m
                else:
                    st[i, 'm', be] = m

        def pr(i, t, tok):
            ps = []
            for be in range(4):
                n = 128 if t < i else 32 * (be + 1)
                m8 = after(jnp.broadcast_to(st[i, 'm', be], (8, 128)), tok, be / 4)
                p = jnp.exp2(s_refs[i][128 * t:128 * t + n, 128 * be:128 * be + 128].reshape(n // 8, 8, 128) - m8)
                ls = jnp.sum(p, axis=0)
                p = p.reshape(n, 128)
                st[i, 'l', be] = ls if t == 0 else st[i, 'l', be] + ls
                p_refs[i].bitcast(bf16)[128 * t:128 * t + n, 128 * be:128 * be + 128] = p.astype(bf16)

        def pv(i, t):
            ps = [p_refs[i][64 * t:64 * t + (64 if t < i else 16 * (be + 1)), 128 * be:128 * be + 128]
                  for be in range(4)]
            if t < i:
                ts = _unskew(ps)
            else:
                blk = [_unskew([ps[be][16 * u:16 * u + 16] if be >= u else None for be in range(4)])
                       for u in range(4)]
                ts = [jnp.concatenate([blk[u][j] for u in range(4)], axis=0) for j in range(4)]
            for j in range(4):
                o = _dot(_unpack(vt_r[16 * j:16 * j + 16, 128 * t:128 * t + 128]), _unpack(ts[j]))
                st[i, 'o', j] = o if t == 0 else st[i, 'o', j] + o

        def fin(i):
            ls = _unskew([jnp.sum(st.pop((i, 'l', be)), axis=0, keepdims=True) for be in range(4)])
            parts = []
            for j in range(4):
                gt = gate_ref[pl.ds(4 * g + j, 1), :]
                omg = gate_ref[pl.ds(32 + 4 * g + j, 1), :]
                o = st.pop((i, 'o', j)) * (omg / ls[j])
                if j > 0:
                    o = pltpu.roll(o, 128 - 32 * j, 1)
                if use_mem:
                    den = nd_ref[128 + j:129 + j, 128 * i:128 * i + 128] + 1e-6
                    o = o + nd_ref[32 * j:32 * j + 32, 128 * i:128 * i + 128] * (gt / den)
                parts.append(o)
            ot = jnp.concatenate(parts, axis=0)
            o_ref.bitcast(bf16)[pl.ds(pl.multiple_of((seg % 2 * 4 + g // 2) * L + 128 * i, 128), 128),
                                128 * par:128 * par + 128] = ot.T.astype(bf16)

        def ex(kind, i, t, tok):
            if kind in 'ep':
                pr(i, t, tok)
            if kind in 'ev':
                pv(i, t)
                if t == i:
                    fin(i)
        return nd, upd, qk, mx, ex

    def ln1(seg, r, tok=None, reload=True):
        r0 = pl.multiple_of(r * SUB, SUB)
        x = x_ref[seg, pl.ds(r0, SUB), :].astype(f32)
        if tok is not None:
            x = jnp.concatenate([after(x[:, 0:128], tok, CFG['xfrac']), x[:, 128:]], axis=1)
        if CFG['one']:
            m, rs = _stats(x)
            if CFG['reload'] and reload:
                mx_ref[16:24, :] = jnp.broadcast_to(m[0:8], (8, 128))
                x = x_ref[seg, pl.ds(r0, SUB), :].astype(f32)
            xn = ((x - m) * rs).astype(bf16)
        else:
            xn = _ln(x).astype(bf16)
        if seg < 2:
            xa_b[pl.ds(pl.multiple_of(seg * L + r0, SUB), SUB), :] = xn
        else:
            xb_b[pl.ds(pl.multiple_of((seg - 1) * L + r0, SUB), SUB), :] = xn
        return xn

    def oproj(seg, r0, rows, n, k0=0, k1=NG, deps=()):
        h0 = pl.multiple_of(r0 // 2, rows // 2)
        r0 = pl.multiple_of(r0, rows)
        lhs = jnp.concatenate(
            [o_ref[pl.ds(pl.multiple_of((seg % 2 * 4 + p) * (L // 2) + h0, rows // 2), rows // 2), :]
             for p in range(k0 // 2, k1 // 2)], axis=1)
        for d in deps:
            top = jnp.concatenate([after(lhs[0:8, 0:128], d, 0.0), lhs[0:8, 128:]], axis=1)
            lhs = jnp.concatenate([top, lhs[8:]], axis=0)
        lhs = _unpack(lhs)
        y = _dot(lhs, _unpack(wo_u[n, 64 * k0:64 * k1, :]))
        cols = slice(128 * n, 128 * n + 128)
        if k0 > 0:
            y = y + x1_ref[seg, pl.ds(r0, rows), cols]
        if k1 == NG:
            y = _rb(x_ref[seg, pl.ds(r0, rows), cols].astype(f32) + y)
        x1_ref[seg, pl.ds(r0, rows), cols] = y
        return y

    def ln2(seg, c, t, tok=None, defer=False):
        r0 = pl.multiple_of(c * CH + t * SUB, SUB)
        lane = lax.broadcasted_iota(i32, (SUB, 128), 1)
        x1 = x1_ref[seg, pl.ds(r0, SUB), :]
        if tok is not None and CFG['pace2']:
            x1 = jnp.concatenate([after(x1[:, 0:128], tok, CFG['xfrac']), x1[:, 128:]], axis=1)
        if CFG['one']:
            m, rs = _stats(x1)
            r = _rb((_rowsum(x1 * jnp.tile(wrf_ref[0:8, :], (2, 1))) - m * jnp.tile(wrf_ref[8:16, 0:128], (2, 1))) * rs)
        else:
            xn2 = _ln(x1, CFG['lnmode'])
            r = _rb(jnp.sum(xn2 * wrf_ref[0:1, :], axis=-1, keepdims=True))
        r_ref[SUB * t:SUB * t + SUB, :] = jnp.where(lane == seg * NG + c, r, r_ref[SUB * t:SUB * t + SUB, :])

        def fin(tok2=None):
            if CFG['one']:
                xr = x1_ref[seg, pl.ds(r0, SUB), :] if CFG['reload'] else x1
                if tok2 is not None:
                    xr = jnp.concatenate([after(xr[:, 0:128], tok2, CFG['xfrac']), xr[:, 128:]], axis=1)
                x2 = xr * (1.0 + rs) - m * rs
            else:
                x2 = x1 + xn2
            x_ref[seg, pl.ds(r0, SUB), :] = x2.astype(bf16)
        if defer:
            return r, fin
        fin()
        return r, None

    def group(s, g, par, last=False):
        kind = s if isinstance(s, int) else 1
        nd, upd, qk, mx, ex = attn_items(g, par, s, kind > 0)
        fill = []
        extra = []
        if kind > 0:
            for n in range(NG):
                fill.append((128, lambda n=n: oproj(s - 1, g * CH, CH, n)))
            extra = [lambda tok, t=t: ln2(s - 1, g, t, tok) for t in range(CH // SUB)]
        else:
            extra = [lambda tok, seg=seg, t=t: ln1(seg, g * (CH // SUB) + t, tok)
                     for seg in range(2, NSEG) for t in range(CH // SUB)]
        if not last:
            gn = g + 1
            pj = proj_items(s, gn // NG, gn % NG, 1 - par)
            for m, n in PORDER:
                for h in range(2):
                    fill.append((128, lambda m=m, n=n, h=h: pj(m, n, h)))
        else:
            for m in range(4):
                for n in range(NG):
                    fill.append((128, lambda m=m, n=n: oproj(s, 128 * m, 128, n, 0, 4)))
        sched = CFG['sched0' if kind == 0 else 'schedL' if last else 'sched'].split()
        y = None
        for tok in sched:
            if tok == 'f':
                y = fill.pop(0)[1]()
            elif tok == 'F':
                while fill:
                    fill.pop(0)[1]()
            elif tok == 'x':
                extra.pop(0)(y)
            elif tok == 'n':
                nd()
            elif tok == 'u':
                if kind < NSEG - 1:
                    upd()
            elif tok[0] == 'q':
                qk(int(tok[1]))
            elif tok[0] == 'Q':
                nxt = attn_items(None, 1 - par, None, None)
                nxt[2](int(tok[1]))
                nxt[3](int(tok[1]), 'store')
            elif tok[0] == 'M':
                mx(int(tok[1]), 'load')
            elif tok[0] == 'm':
                mx(int(tok[1]))
            else:
                ex(tok[0], int(tok[1]), int(tok[2]), y)
        for it in fill:
            it[1]()
        for e in extra:
            e(None)

    early = {'a': cp_x0(0), 'b': cp_x0(1), 'c': cp_x0(2), 'd': cp_x0(3), 'q': cp_w(0, 0), 'k': cp_w(0, 1),
             'v': cp_w(0, 2), 'x': cp_x1(), 's': cp_small()[0], 'r': cp_small()[1]}
    issue = CFG['issue'].split()
    for k in issue[0]:
        early[k].start()

    z_ref[0:8, :] = jnp.zeros((8, 128), u32)
    ones = jnp.full((8, 512), 0x3F803F80, u32)
    vt0[64:72, :] = ones
    vt1[64:72, :] = ones
    bias_ref[...] = jnp.where(lax.broadcasted_iota(i32, (32, 128), 0)
                              <= (lax.broadcasted_iota(i32, (32, 128), 1) & 31), 0.0, NEG)

    def ln0_body(c, carry):
        cp_x0(c).wait()
        for n in range(1, len(issue)):
            @pl.when(c == n - 1)
            def _():
                for k in issue[n].strip('-'):
                    early[k].start()
        for t in range(128 // SUB):
            ln1(0, c * (128 // SUB) + t)
        return carry
    lax.fori_loop(0, 4, ln0_body, 0)
    for g in range(1, NG):
        for j in range(3):
            cp_w(g, j).start()
        cp_xr(g - 1).start()
    cp_xr(NG - 1).start()
    for cp in cp_wo():
        cp.start()

    for cp in cp_small():
        cp.wait()
    wr = wr_ref[...].astype(f32)
    for c in range(D // 128):
        wrf_ref[0:8, 128 * c:128 * c + 128] = jnp.broadcast_to(wr[c:c + 1, :], (8, 128))
    wrf_ref[8:16, :] = jnp.broadcast_to(jnp.sum(wr, axis=(0, 1), keepdims=True), (8, D))
    gl = _rb(jax.nn.sigmoid(beta_ref[...].astype(f32)))
    hr = lax.broadcasted_iota(i32, (32, 32), 0)
    hc = lax.broadcasted_iota(i32, (32, 32), 1)
    gcol = jnp.sum(jnp.where(hr == hc, gl, 0.0), axis=1, keepdims=True)
    gate_ref[0:32, :] = jnp.broadcast_to(gcol, (32, 128))
    gate_ref[32:64, :] = jnp.broadcast_to(_rb(1.0 - gcol), (32, 128))
    for j in range(2 + CFG['vearly']):
        cp_w(0, j).wait()
    if CFG['prewait']:
        for g in range(NG):
            cp_xr(g).wait()
            for j in range(3 * (g > 0)):
                cp_w(g, j).wait()
        for cp in cp_wo():
            cp.wait()

    def layer(li, carry):
        first = li == 0
        r_ref[...] = jnp.full((CH, 128), -jnp.inf, f32)
        pj = proj_items(0, 0, 0, 0)
        fill = [(m, n, h) for m, n in PORDER for h in range(2)]
        extra = list(range(L // SUB))
        y = None
        for tok in CFG['pre'].split():
            if tok == 'f':
                y = pj(*fill.pop(0))
            elif tok == 'x':
                ln1(1, extra.pop(0), y)
            elif tok in 'wW':
                @pl.when(first)
                def _():
                    if not CFG['vearly']:
                        cp_w(0, 2).wait()
                    cp_x1().wait()
                    if tok == 'W':
                        lax.fori_loop(0, CFG['n1'] // 4, lambda i, c: [ln1(1, 4 * i + j) for j in range(4)] and c, 0)
                extra = extra[CFG['n1'] * (tok == 'W'):]
                y = None
            else:
                nxt = attn_items(None, 0, None, None)
                nxt[2](int(tok[1]))
                nxt[3](int(tok[1]), 'store')
        assert not fill and not extra
        cp_xn().start()

        def pair(s, p, last=False):
            for par in range(2):
                group(s, 2 * p + par, par, last and par == 1)

        def seg0(p, c2):
            if not CFG['prewait']:
                @pl.when(first)
                def _():
                    for par in range(2):
                        cp_xr(2 * p + par).wait()
                    for j in range(3):
                        cp_w(2 * p + 1, j).wait()

                    @pl.when(p < NG // 2 - 1)
                    def _():
                        for j in range(3):
                            cp_w(jnp.minimum(2 * p + 2, NG - 2), j).wait()

                    @pl.when(p == NG // 2 - 1)
                    def _():
                        for cp in cp_wo():
                            cp.wait()
            pair(0, p)
            return c2
        _loop('s0', NG // 2, seg0)
        cp_xn().wait()

        @pl.when(first)
        def _():
            for cp in cp_ff():
                cp.start()

        def mid(t, c2):
            pair(1 + t // (NG // 2), t % (NG // 2))
            return c2
        _loop('s1', NG + (NG // 2 - 1) * CFG['merge3'], mid)

        def wait_ff():
            @pl.when(first)
            def _():
                for cp in cp_ff():
                    cp.wait()

        @pl.when(li == CFG['nl'] - 1)
        def _():
            cp_out_seg(0).start()
            cp_out_seg(1).start()

        def seg3(p, c2):
            pair(NSEG - 1, p)
            return c2
        if not CFG['merge3']:
            _loop('s3', NG // 2 - 1, seg3)
        if CFG['ffearly']:
            wait_ff()
        pair(NSEG - 1, NG // 2 - 1, last=True)

        s = NSEG - 1
        pend = []
        r0 = L
        late, gate, step, glag = [], {}, 0, 0
        for rows, nlag in zip(CFG['tail'], CFG['glag']):
            r0 -= rows
            for n in range(NG):
                y = oproj(s, r0, rows, n, 4, NG, gate.pop(step, ()))
                if pend:
                    r, fin = pend.pop(0)(y)
                    late.append(fin)
                    if glag:
                        gate.setdefault(step + glag, []).append(r)
                step += 1
            pend = [lambda tok, r=r: ln2(s, r // CH, r % CH // SUB, tok, r < CFG['defer'])
                    for r in range(r0, r0 + rows, SUB)]
            glag = nlag
        assert r0 == 0
        late = [e for e in late + [e(None)[1] for e in pend] if e is not None]

        def start_out():
            cp_out_seg(NSEG - 2).start()
            cp_out_seg(NSEG - 1).start()
        if not late:
            start_out()

        rm = r_ref[...]
        rb = pltpu.bitcast(jnp.where(rm == 0.0, 0.0, rm), i32)
        lane = lax.broadcasted_iota(i32, (CH, 128), 1)
        base = jnp.where(lane < S // CH, (1 << 29) + S - 1 - lane * CH - lax.broadcasted_iota(i32, (CH, 128), 0), 0)
        mono = rb ^ ((rb >> 31) | jnp.int32(-2 ** 31))
        key = pltpu.bitcast(base + (lax.shift_right_logical(mono, 5) & 0x07FFF800), f32)
        k1 = jnp.max(key, axis=(0, 1), keepdims=True)
        k2 = jnp.max(jnp.where(key == k1, 0.0, key), axis=(0, 1), keepdims=True)
        toks = [jnp.clip(jnp.max((S - 1 - (pltpu.bitcast(k, i32) & (S - 1))).astype(f32)).astype(i32), 0, S - 1)
                for k in (k1, k2)]

        if not CFG['ffearly']:
            wait_ff()

        row = lax.broadcasted_iota(i32, (SUB, D), 0)
        x1s = jnp.concatenate([x1_ref[t >> 9, pl.ds(pl.multiple_of(t & (L - 8), 8), 8), :] for t in toks], axis=0)
        ms, rss = _stats(x1s)
        xs = ((x1s - ms) * rss).astype(bf16)
        hs, ys, todo = [], [None] * NG, list(range(L // SUB + CFG['n1'] * ('W' in CFG['pre'])))
        dlag, kc, snaps = CFG['dlag'], CFG['kc'], []

        two = int(len(todo) > NF + 7)

        def ffln(tok):
            r = todo.pop(0)
            ln1(r // (L // SUB), r % (L // SUB), tok, CFG['freload'])
        for c in range(NF + dlag):
            if c < NF:
                ga = _rb(_dot(xs, _unpack(wg_u[c])))
                up = _rb(_dot(xs, _unpack(wu_u[c])))
                hs.append((_rb(ga * _rb(jax.nn.sigmoid(ga))) * up).astype(bf16))
                ffln(ga)
                if two and len(todo) > NF - 1 - c:
                    ffln(up)
                if late:
                    late.pop(0)(ga)
                    if not late:
                        start_out()
            k = c - dlag + 1 - kc
            if k >= 0 and k % kc == 0:
                snaps.append(list(ys))
                if CFG['alag'] and len(snaps) > CFG['alag'] + 1:
                    t = None
                    for yv in snaps[-1 - CFG['alag'] + 1]:
                        for u in (yv[0:8], yv[8:16]):
                            t = pltpu.bitcast(u, u32) if t is None else t | pltpu.bitcast(u, u32)
                    hs[k] = pltpu.bitcast(pltpu.bitcast(hs[k], u32) | (t & z_ref[0:8, :]), bf16)
                h = jnp.concatenate(hs[k:k + kc], axis=1)
                for n in range(NG):
                    part = _dot(h, _unpack(wd_u[n, 64 * k:64 * (k + kc), :]))
                    ys[n] = part if ys[n] is None else ys[n] + part
                    if n % (NG >> two) == 0 and len(todo) > max(NF - 1 - c, 0) << two and c >= CFG['xln']:
                        ffln(part)
        assert not todo
        y = _rb(jnp.concatenate(ys, axis=1))
        ksel = pltpu.bitcast(jnp.where(lax.broadcasted_iota(i32, (SUB, 128), 0) < 8, k1, k2), i32)
        hi = (ksel << 5) & -65536
        rsel = pltpu.bitcast(jnp.where(hi < 0, hi ^ jnp.int32(-2 ** 31), ~hi & -65536), f32)[:, 0:1]
        y = _rb(y * _rb(jax.nn.sigmoid(rsel)))
        x2s = _rb(x1s + _rb(xs.astype(f32) + y))
        ms, rss = _stats(x2s)
        xns = (x2s - ms) * rss

        @pl.when(li == CFG['nl'] - 1)
        def _():
            for s in range(NSEG - 2):
                cp_out_seg(s).wait()
        for s in range(NSEG - 2, NSEG):
            cp_out_seg(s).wait()

        blks = []
        xa_rows = range(2 * L if 'W' in CFG['pre'] else L)
        for n, t in enumerate(toks):
            sg = t >> 9
            b0 = pl.multiple_of(t & (L - SUB), SUB)
            b2 = t & (len(xa_rows) - SUB)
            hb = pl.multiple_of(b2 >> 1, SUB // 2)
            hit = row == (t & (SUB - 1))
            old = x_ref[sg, pl.ds(b0, SUB), :].astype(f32)
            x_ref[sg, pl.ds(b0, SUB), :] = jnp.where(hit, jnp.tile(x2s[8 * n:8 * n + 8], (2, 1)), old).astype(bf16)
            oldn = _unpack(xa_ref[pl.ds(hb, SUB // 2), :]).astype(f32)
            xa_ref[pl.ds(hb, SUB // 2), :] = _pack(jnp.where(row == t - b2, jnp.tile(xns[8 * n:8 * n + 8], (2, 1)), oldn))
            blks.append((sg, b0))

        @pl.when(li == CFG['nl'] - 1)
        def _():
            def cp_fix(n):
                sg, b0 = blks[n]
                return pltpu.make_async_copy(x_ref.at[sg, pl.ds(b0, SUB), :],
                                             out_hbm.at[sg, pl.ds(b0, SUB), :], sems.at[SEM_FIX])
            differ = (toks[0] >> 4) != (toks[1] >> 4)
            cp_fix(0).start()

            @pl.when(differ)
            def _():
                cp_fix(1).start()
                cp_fix(1).wait()
            cp_fix(0).wait()
        return carry

    lax.fori_loop(0, CFG['nl'], layer, 0)


@jax.jit
def pallas_interleave_layers__memory_aug_infini_attn__moe_arch_mod__prompt_kernel(
    A_x: jax.Array,
    A_wq: jax.Array,
    A_wk: jax.Array,
    A_wv: jax.Array,
    A_wo: jax.Array,
    A_beta: jax.Array,
    B_x: jax.Array,
    B_w_r: jax.Array,
    B_w_gate: jax.Array,
    B_w_up: jax.Array,
    B_w_down: jax.Array,
):
    del B_x
    qkv_bufs = [pltpu.VMEM((L // 2, 512), u32), pltpu.VMEM((72, L), u32)]
    scratch = [
        pltpu.VMEM((8 * CFG['zpad'], 128), u32),
        pltpu.VMEM((NSEG, L, D), bf16),
        pltpu.VMEM((3 * L // 2, D), u32),
        pltpu.VMEM((NSEG, L, D), f32),
        pltpu.VMEM((3 * NG, D, 128), bf16),
        pltpu.VMEM((NG, D, 128), bf16),
        pltpu.VMEM((NF, D, 128), bf16),
        pltpu.VMEM((NF, D, 128), bf16),
        pltpu.VMEM((NG, F, 128), bf16),
        pltpu.VMEM((64, 128), f32),
        pltpu.VMEM((32, 128), f32),
        pltpu.VMEM((NG, 144, 128), f32),
        pltpu.VMEM((CH, 128), f32),
        pltpu.VMEM((144, L), f32),
        pltpu.VMEM((128, L), f32), pltpu.VMEM((256, L), f32),
        pltpu.VMEM((384, L), f32), pltpu.VMEM((512, L), f32),
        pltpu.VMEM((64, L), u32), pltpu.VMEM((128, L), u32),
        pltpu.VMEM((192, L), u32), pltpu.VMEM((256, L), u32),
        *qkv_bufs, *qkv_bufs,
        pltpu.VMEM((NG * L // 2, 256), u32),
        pltpu.VMEM((L, D), u32),
        pltpu.VMEM((16, D), f32),
        pltpu.VMEM((24 + 8 * CFG['mpad'], 128), f32),
        pltpu.VMEM((8, 128), bf16),
        pltpu.VMEM((1, 32), bf16),
        pltpu.SemaphoreType.DMA((NSEM,)),
    ]
    out = pl.pallas_call(
        _kernel,
        out_shape=jax.ShapeDtypeStruct((NSEG, L, D), bf16),
        in_specs=[pl.BlockSpec(memory_space=pl.ANY)] * 10,
        out_specs=pl.BlockSpec(memory_space=pl.ANY),
        scratch_shapes=scratch,
        compiler_params=pltpu.CompilerParams(vmem_limit_bytes=100 * 2 ** 20),
    )(A_x.reshape(NSEG, L, D), A_wq, A_wk, A_wv, A_wo, A_beta.reshape(1, 32), B_w_r.reshape(8, 128),
      B_w_gate, B_w_up, B_w_down)
    return out.reshape(1, S, D)
```

```python
import jax
import jax.numpy as jnp
from jax import lax
import jax.experimental.pallas as pl
import jax.experimental.pallas.tpu as pltpu

bf16 = jnp.bfloat16
f32 = jnp.float32
u32 = jnp.uint32
i32 = jnp.int32

S = 2048
D = 1024
L = 512
NSEG = 4
NG = 8
F = 3584
CH = 64
SUB = 16
NEG = -1e30
QSCALE = (32 ** -0.5) * 1.4426950408889634
NT = (((1,), (1,)), ((), ()))

SEM_XC = 0
SEM_W0 = 4
SEM_X1 = 5
SEM_SM = 6
SEM_P = 7
NSEM = 11
SEM_OUT, SEM_FIX, SEM_FF, SEM_XN = 0, 1, 2, 3
NF = F // 128
PORDER = [(m, n) for m in range(4) for n in range(2)] + [(m, 2) for m in range(4)]

CFG = dict(
    tail=(128, 128, 128, 64, 32, 32), defer=64, dlag=2, kc=4, xln=4, alag=0, n1=32, vearly=1, mpad=2, glag=(0, 0, 0, 0, 0, 0), rep={}, cnt={}, merge3=0, zpad=4, issue='abcdqkvsr x', lnmode=0, nl=2, prewait=False, gp=2, pace=True, pace2=True, one=True, reload=True, chain=True, xfrac=0.0, freload=False, lag=0, fskip=0,
    pre='f ' * 18 + 'Q3 ' + 'f ' * 6 + 'W',
    sched='M3 f p30 f n q2 v30 p31 f f v31 p32 f f m2 v32 p33 f f v33 p20 f f q1 v20 p21 f x f v21 p22 f x f '
          'm1 v22 p10 f x f q0 v10 p11 f x f u v11 m0 f p00 f f v00 F Q3',
    sched0='M3 f p30 f q2 v30 p31 f f v31 p32 f f x m2 v32 p33 f f x v33 p20 f f x q1 v20 p21 f f x '
           'v21 p22 f f x m1 v22 p10 f f x q0 v10 p11 f x f u v11 m0 f x p00 f f v00 F Q3',
    schedL='M3 f p30 f n q2 v30 p31 f f v31 p32 f f m2 v32 p33 f f v33 p20 f f q1 v20 p21 f x f v21 p22 f x f '
          'm1 v22 p10 f x f q0 v10 p11 f x f v11 m0 f p00 f f v00 F',
)


def _loop(name, n, body):
    rep = CFG['rep'].get(name, 1)
    n = CFG['cnt'].get(name, n)
    if n == 0:
        return 0
    if rep == 1:
        return lax.fori_loop(0, n, body, 0)
    return lax.fori_loop(0, n * rep, lambda i, c: body(i // rep, c), 0)


def _rb(x):
    return x.astype(bf16).astype(f32)


def _pack(x):
    return pltpu.bitcast(x.astype(bf16), u32)


def _unpack(u):
    return pltpu.bitcast(u, bf16)


def _phi(t):
    return jnp.where(t > 0, t + 1.0, jnp.exp(t))


def _dot(a, b):
    return jnp.dot(a, b, preferred_element_type=f32)


def _unskew(ps):
    shape, dt = next((p.shape, p.dtype) for p in ps if p is not None)
    c = lax.broadcasted_iota(i32, shape, 1) >> 5
    even = (c & 1) == 0
    lo = c < 2
    mid = jnp.logical_or(c == 1, c == 2)

    def sel(mask, a, b):
        if a is None and b is None:
            return None
        z = jnp.zeros(shape, dt)
        return jnp.where(mask, z if a is None else a, z if b is None else b)
    x0, x1 = sel(even, ps[0], ps[1]), sel(even, ps[1], ps[0])
    x2, x3 = sel(even, ps[2], ps[3]), sel(even, ps[3], ps[2])
    return [sel(lo, x0, x2), sel(mid, x1, x3), sel(lo, x2, x0), sel(mid, x3, x1)]


def _ln(x, mode=0):
    acc = x
    if CFG['chain']:
        acc = x[:, 0:128]
        for c in range(1, x.shape[1] // 128):
            acc = acc + x[:, 128 * c:128 * c + 128]
    m = jnp.sum(acc, axis=-1, keepdims=True) * (1.0 / D)
    if mode == 0:
        e = x - m
        v = jnp.sum(e * e, axis=-1, keepdims=True) * (1.0 / D)
        return e * lax.rsqrt(v + 1e-5)
    c = _rb(m)
    e = x - c
    v = jnp.sum(e * e, axis=-1, keepdims=True) * (1.0 / D) - (m - c) * (m - c)
    w = _rb(_rb(jnp.maximum(v, 0.0)) + 1e-5)
    den = _rb(w * lax.rsqrt(w))
    if mode == 2:
        return _rb(_rb(e) / den)
    return e * (1.0 / den)


def _rowsum(x, first=None):
    acc = x[:, 0:128] if first is None else first
    for c in range(1, x.shape[1] // 128):
        acc = acc + x[:, 128 * c:128 * c + 128]
    return jnp.sum(acc, axis=-1, keepdims=True)


def _stats(x):
    m = _rowsum(x) * (1.0 / D)
    v = jnp.maximum(_rowsum(x * x) * (1.0 / D) - m * m, 0.0)
    return m, lax.rsqrt(v + 1e-5)


def _kernel(x_hbm, wq_hbm, wk_hbm, wv_hbm, wo_hbm, beta_hbm, wr_hbm, wg_hbm, wu_hbm, wd_hbm,
            out_hbm,
            z_ref, x_ref, xb_ref, x1_ref, w_ref, wo_ref, wg_ref, wu_ref, wd_ref,
            gate_ref, bias_ref, m_ref, r_ref, nd_ref,
            s0_ref, s1_ref, s2_ref, s3_ref, p0_ref, p1_ref, p2_ref, p3_ref,
            qk0, vt0, qk1, vt1, o_ref, xa_ref, wrf_ref, mx_ref, wr_ref, beta_ref, sems):
    qkv = ((qk0, vt0), (qk1, vt1))
    s_refs = (s0_ref, s1_ref, s2_ref, s3_ref)
    p_refs = (p0_ref, p1_ref, p2_ref, p3_ref)
    xa_b, xb_b = xa_ref.bitcast(bf16), xb_ref.bitcast(bf16)
    w_u, wo_u, wg_u, wu_u, wd_u = (r.bitcast(u32) for r in (w_ref, wo_ref, wg_ref, wu_ref, wd_ref))

    def cp_x0(c):
        rows = pl.ds(pl.multiple_of(128 * c, 128), 128)
        return pltpu.make_async_copy(x_hbm.at[0, rows], x_ref.at[0, rows], sems.at[SEM_XC + c])

    def cp_x1():
        return pltpu.make_async_copy(x_hbm.at[1], x_ref.at[1], sems.at[SEM_X1])

    def cp_xn():
        return pltpu.make_async_copy(xa_ref.at[L // 2:L], xb_ref.at[0:L // 2], sems.at[SEM_XN])

    def cp_xr(g):
        r0 = pl.multiple_of(g * CH, CH)
        return pltpu.make_async_copy(x_hbm.at[2:NSEG, pl.ds(r0, CH), :],
                                     x_ref.at[2:NSEG, pl.ds(r0, CH), :], sems.at[SEM_P + g // 2])

    def cp_w(g, j):
        c0 = pl.multiple_of(g * 128, 128)
        src = (wq_hbm, wk_hbm, wv_hbm)[j]
        sem = (SEM_W0 + j // 2 * (1 - CFG['vearly'])) if isinstance(g, int) and g == 0 else SEM_P + (g - 1) // 2
        return pltpu.make_async_copy(src.at[:, pl.ds(c0, 128)], w_ref.at[3 * g + j], sems.at[sem])

    def slabs(src, dst, n, sem):
        return [pltpu.make_async_copy(src.at[:, 128 * c:128 * c + 128], dst.at[c], sems.at[sem]) for c in range(n)]

    def cp_wo():
        return slabs(wo_hbm, wo_ref, NG, SEM_P + 3)

    def cp_small():
        return (pltpu.make_async_copy(beta_hbm, beta_ref, sems.at[SEM_SM]),
                pltpu.make_async_copy(wr_hbm, wr_ref, sems.at[SEM_SM]))

    def cp_ff():
        return (slabs(wg_hbm, wg_ref, NF, SEM_FF) + slabs(wu_hbm, wu_ref, NF, SEM_FF)
                + slabs(wd_hbm, wd_ref, NG, SEM_FF))

    def cp_out_seg(s):
        return pltpu.make_async_copy(x_ref.at[s], out_hbm.at[s], sems.at[SEM_OUT])

    def after(x, tok, frac):
        if tok is None or not CFG['pace']:
            return x
        r = 8 * int(frac * tok.shape[0] // 8)
        t = pltpu.bitcast(tok[r:r + 8, 0:128], u32) & z_ref[0:8, :]
        t = jnp.tile(t, (x.shape[0] // 8, x.shape[1] // 128))
        return pltpu.bitcast(pltpu.bitcast(x, u32) | t, x.dtype)

    def proj_items(s, nxt, g, par):
        xn_r, seg = (xa_ref, nxt) if isinstance(s, int) and s == 0 else (xb_ref, s - 1 + nxt)
        qk_r, vt_r = (r.bitcast(bf16) for r in qkv[par])
        part = {}

        def item(m, n, h):
            xn = _unpack(xn_r[pl.ds(pl.multiple_of(seg * (L // 2) + 64 * m, 64), 64), 512 * h:512 * h + 512])
            y = _dot(xn, _unpack(w_u[3 * g + n, 256 * h:256 * h + 256, :]))
            if h == 0:
                part[m, n] = y
                return y
            y = y + part.pop((m, n))
            rows = slice(128 * m, 128 * m + 128)
            if n == 0:
                qk_r[rows, 0:128] = (y * QSCALE).astype(bf16)
                qk_r[rows, 128:256] = _phi(y).astype(bf16)
            elif n == 1:
                qk_r[rows, 256:384] = y.astype(bf16)
                qk_r[rows, 384:512] = _phi(y).astype(bf16)
            else:
                vt_r[0:128, rows] = y.T.astype(bf16)
            return y
        return item

    def attn_items(g, par, seg, use_mem):
        qk_r, vt_r = qkv[par]
        st = {}

        def nd():
            ml = m_ref[g].astype(bf16)
            nd_ref[...] = lax.dot_general(ml, _unpack(qk_r[:, 128:256]), NT, preferred_element_type=f32)

        def upd():
            u = _dot(_unpack(vt_r[...]), _unpack(qk_r[:, 384:512]))
            r2 = lax.broadcasted_iota(i32, (144, 128), 0)
            c2 = lax.broadcasted_iota(i32, (144, 128), 1) >> 5
            keep = jnp.where(r2 < 128, r2 >> 5, r2 - 128) == c2
            u = jnp.where(keep, u, 0.0)
            m_ref[g] = (m_ref[g] + u) if use_mem else u

        def qk(i):
            lane = lax.broadcasted_iota(i32, (16, 128), 1) >> 5
            for be in (range(4) if i % 2 else range(3, -1, -1)):
                b = 4 * i + be
                n = 32 * (b + 1)
                qu = qk_r[16 * b:16 * b + 16, 0:128]
                wq = _unpack(jnp.concatenate(
                    [jnp.where(lane == (c - be) % 4, qu, jnp.uint32(0)) for c in range(4)], axis=0))
                s = lax.dot_general(_unpack(qk_r[0:n // 2, 256:384]), wq, NT, preferred_element_type=f32)
                cols = slice(128 * be, 128 * be + 128)
                if b > 0:
                    s_refs[i][0:n - 32, cols] = s[0:n - 32]
                s_refs[i][n - 32:n, cols] = s[n - 32:n] + bias_ref[...]

        def mx(i, mode='m'):
            for be in range(4):
                if mode == 'load':
                    st[i, 'm', be] = mx_ref[4 * i + be:4 * i + be + 1, :]
                    continue
                n = 32 * (4 * i + be + 1)
                sv = s_refs[i][0:n, 128 * be:128 * be + 128]
                m = jnp.max(jnp.max(sv.reshape(n // 8, 8, 128), axis=0), axis=0, keepdims=True)
                if mode == 'store':
                    mx_ref[4 * i + be:4 * i + be + 1, :] = m
                else:
                    st[i, 'm', be] = m

        def pr(i, t, tok):
            ps = []
            for be in range(4):
                n = 128 if t < i else 32 * (be + 1)
                m8 = after(jnp.broadcast_to(st[i, 'm', be], (8, 128)), tok, be / 4)
                p = jnp.exp2(s_refs[i][128 * t:128 * t + n, 128 * be:128 * be + 128].reshape(n // 8, 8, 128) - m8)
                ls = jnp.sum(p, axis=0)
                p = p.reshape(n, 128)
                st[i, 'l', be] = ls if t == 0 else st[i, 'l', be] + ls
                p_refs[i].bitcast(bf16)[128 * t:128 * t + n, 128 * be:128 * be + 128] = p.astype(bf16)

        def pv(i, t):
            ps = [p_refs[i][64 * t:64 * t + (64 if t < i else 16 * (be + 1)), 128 * be:128 * be + 128]
                  for be in range(4)]
            if t < i:
                ts = _unskew(ps)
            else:
                blk = [_unskew([ps[be][16 * u:16 * u + 16] if be >= u else None for be in range(4)])
                       for u in range(4)]
                ts = [jnp.concatenate([blk[u][j] for u in range(4)], axis=0) for j in range(4)]
            for j in range(4):
                o = _dot(_unpack(vt_r[16 * j:16 * j + 16, 128 * t:128 * t + 128]), _unpack(ts[j]))
                st[i, 'o', j] = o if t == 0 else st[i, 'o', j] + o

        def fin(i):
            ls = _unskew([jnp.sum(st.pop((i, 'l', be)), axis=0, keepdims=True) for be in range(4)])
            parts = []
            for j in range(4):
                gt = gate_ref[pl.ds(4 * g + j, 1), :]
                omg = gate_ref[pl.ds(32 + 4 * g + j, 1), :]
                o = st.pop((i, 'o', j)) * (omg / ls[j])
                if j > 0:
                    o = pltpu.roll(o, 128 - 32 * j, 1)
                if use_mem:
                    den = nd_ref[128 + j:129 + j, 128 * i:128 * i + 128] + 1e-6
                    o = o + nd_ref[32 * j:32 * j + 32, 128 * i:128 * i + 128] * (gt / den)
                parts.append(o)
            ot = jnp.concatenate(parts, axis=0)
            o_ref.bitcast(bf16)[pl.ds(pl.multiple_of((seg % 2 * 4 + g // 2) * L + 128 * i, 128), 128),
                                128 * par:128 * par + 128] = ot.T.astype(bf16)

        def ex(kind, i, t, tok):
            if kind in 'ep':
                pr(i, t, tok)
            if kind in 'ev':
                pv(i, t)
                if t == i:
                    fin(i)
        return nd, upd, qk, mx, ex

    def ln1(seg, r, tok=None, reload=True):
        r0 = pl.multiple_of(r * SUB, SUB)
        x = x_ref[seg, pl.ds(r0, SUB), :].astype(f32)
        if tok is not None:
            x = jnp.concatenate([after(x[:, 0:128], tok, CFG['xfrac']), x[:, 128:]], axis=1)
        if CFG['one']:
            m, rs = _stats(x)
            if CFG['reload'] and reload:
                mx_ref[16:24, :] = jnp.broadcast_to(m[0:8], (8, 128))
                x = x_ref[seg, pl.ds(r0, SUB), :].astype(f32)
            xn = ((x - m) * rs).astype(bf16)
        else:
            xn = _ln(x).astype(bf16)
        if seg < 2:
            xa_b[pl.ds(pl.multiple_of(seg * L + r0, SUB), SUB), :] = xn
        else:
            xb_b[pl.ds(pl.multiple_of((seg - 1) * L + r0, SUB), SUB), :] = xn
        return xn

    def oproj(seg, r0, rows, n, k0=0, k1=NG, deps=()):
        h0 = pl.multiple_of(r0 // 2, rows // 2)
        r0 = pl.multiple_of(r0, rows)
        lhs = jnp.concatenate(
            [o_ref[pl.ds(pl.multiple_of((seg % 2 * 4 + p) * (L // 2) + h0, rows // 2), rows // 2), :]
             for p in range(k0 // 2, k1 // 2)], axis=1)
        for d in deps:
            top = jnp.concatenate([after(lhs[0:8, 0:128], d, 0.0), lhs[0:8, 128:]], axis=1)
            lhs = jnp.concatenate([top, lhs[8:]], axis=0)
        lhs = _unpack(lhs)
        y = _dot(lhs, _unpack(wo_u[n, 64 * k0:64 * k1, :]))
        cols = slice(128 * n, 128 * n + 128)
        if k0 > 0:
            y = y + x1_ref[seg, pl.ds(r0, rows), cols]
        if k1 == NG:
            y = _rb(x_ref[seg, pl.ds(r0, rows), cols].astype(f32) + y)
        x1_ref[seg, pl.ds(r0, rows), cols] = y
        return y

    def ln2(seg, c, t, tok=None, defer=False):
        r0 = pl.multiple_of(c * CH + t * SUB, SUB)
        lane = lax.broadcasted_iota(i32, (SUB, 128), 1)
        x1 = x1_ref[seg, pl.ds(r0, SUB), :]
        if tok is not None and CFG['pace2']:
            x1 = jnp.concatenate([after(x1[:, 0:128], tok, CFG['xfrac']), x1[:, 128:]], axis=1)
        if CFG['one']:
            m, rs = _stats(x1)
            r = _rb((_rowsum(x1 * jnp.tile(wrf_ref[0:8, :], (2, 1))) - m * jnp.tile(wrf_ref[8:16, 0:128], (2, 1))) * rs)
        else:
            xn2 = _ln(x1, CFG['lnmode'])
            r = _rb(jnp.sum(xn2 * wrf_ref[0:1, :], axis=-1, keepdims=True))
        r_ref[SUB * t:SUB * t + SUB, :] = jnp.where(lane == seg * NG + c, r, r_ref[SUB * t:SUB * t + SUB, :])

        def fin(tok2=None):
            if CFG['one']:
                xr = x1_ref[seg, pl.ds(r0, SUB), :] if CFG['reload'] else x1
                if tok2 is not None:
                    xr = jnp.concatenate([after(xr[:, 0:128], tok2, CFG['xfrac']), xr[:, 128:]], axis=1)
                x2 = xr * (1.0 + rs) - m * rs
            else:
                x2 = x1 + xn2
            x_ref[seg, pl.ds(r0, SUB), :] = x2.astype(bf16)
        if defer:
            return r, fin
        fin()
        return r, None

    def group(s, g, par, last=False):
        kind = s if isinstance(s, int) else 1
        nd, upd, qk, mx, ex = attn_items(g, par, s, kind > 0)
        fill = []
        extra = []
        if kind > 0:
            for n in range(NG):
                fill.append((128, lambda n=n: oproj(s - 1, g * CH, CH, n)))
            extra = [lambda tok, t=t: ln2(s - 1, g, t, tok) for t in range(CH // SUB)]
        else:
            extra = [lambda tok, seg=seg, t=t: ln1(seg, g * (CH // SUB) + t, tok)
                     for seg in range(2, NSEG) for t in range(CH // SUB)]
        if not last:
            gn = g + 1
            pj = proj_items(s, gn // NG, gn % NG, 1 - par)
            for m, n in PORDER:
                for h in range(2):
                    fill.append((128, lambda m=m, n=n, h=h: pj(m, n, h)))
        else:
            for m in range(4):
                for n in range(NG):
                    fill.append((128, lambda m=m, n=n: oproj(s, 128 * m, 128, n, 0, 4)))
        sched = CFG['sched0' if kind == 0 else 'schedL' if last else 'sched'].split()
        y = None
        for tok in sched:
            if tok == 'f':
                y = fill.pop(0)[1]()
            elif tok == 'F':
                while fill:
                    fill.pop(0)[1]()
            elif tok == 'x':
                extra.pop(0)(y)
            elif tok == 'n':
                nd()
            elif tok == 'u':
                if kind < NSEG - 1:
                    upd()
            elif tok[0] == 'q':
                qk(int(tok[1]))
            elif tok[0] == 'Q':
                nxt = attn_items(None, 1 - par, None, None)
                nxt[2](int(tok[1]))
                nxt[3](int(tok[1]), 'store')
            elif tok[0] == 'M':
                mx(int(tok[1]), 'load')
            elif tok[0] == 'm':
                mx(int(tok[1]))
            else:
                ex(tok[0], int(tok[1]), int(tok[2]), y)
        for it in fill:
            it[1]()
        for e in extra:
            e(None)

    early = {'a': cp_x0(0), 'b': cp_x0(1), 'c': cp_x0(2), 'd': cp_x0(3), 'q': cp_w(0, 0), 'k': cp_w(0, 1),
             'v': cp_w(0, 2), 'x': cp_x1(), 's': cp_small()[0], 'r': cp_small()[1]}
    issue = CFG['issue'].split()
    for k in issue[0]:
        early[k].start()

    z_ref[0:8, :] = jnp.zeros((8, 128), u32)
    ones = jnp.full((8, 512), 0x3F803F80, u32)
    vt0[64:72, :] = ones
    vt1[64:72, :] = ones
    bias_ref[...] = jnp.where(lax.broadcasted_iota(i32, (32, 128), 0)
                              <= (lax.broadcasted_iota(i32, (32, 128), 1) & 31), 0.0, NEG)

    def ln0_body(c, carry):
        cp_x0(c).wait()
        for n in range(1, len(issue)):
            @pl.when(c == n - 1)
            def _():
                for k in issue[n].strip('-'):
                    early[k].start()
        for t in range(128 // SUB):
            ln1(0, c * (128 // SUB) + t)
        return carry
    lax.fori_loop(0, 4, ln0_body, 0)
    for g in range(1, NG):
        for j in range(3):
            cp_w(g, j).start()
        cp_xr(g - 1).start()
    cp_xr(NG - 1).start()
    for cp in cp_wo():
        cp.start()

    for cp in cp_small():
        cp.wait()
    wr = wr_ref[...].astype(f32)
    for c in range(D // 128):
        wrf_ref[0:8, 128 * c:128 * c + 128] = jnp.broadcast_to(wr[c:c + 1, :], (8, 128))
    wrf_ref[8:16, :] = jnp.broadcast_to(jnp.sum(wr, axis=(0, 1), keepdims=True), (8, D))
    gl = _rb(jax.nn.sigmoid(beta_ref[...].astype(f32)))
    hr = lax.broadcasted_iota(i32, (32, 32), 0)
    hc = lax.broadcasted_iota(i32, (32, 32), 1)
    gcol = jnp.sum(jnp.where(hr == hc, gl, 0.0), axis=1, keepdims=True)
    gate_ref[0:32, :] = jnp.broadcast_to(gcol, (32, 128))
    gate_ref[32:64, :] = jnp.broadcast_to(_rb(1.0 - gcol), (32, 128))
    for j in range(2 + CFG['vearly']):
        cp_w(0, j).wait()
    if CFG['prewait']:
        for g in range(NG):
            cp_xr(g).wait()
            for j in range(3 * (g > 0)):
                cp_w(g, j).wait()
        for cp in cp_wo():
            cp.wait()

    def layer(li, carry):
        first = li == 0
        r_ref[...] = jnp.full((CH, 128), -jnp.inf, f32)
        pj = proj_items(0, 0, 0, 0)
        fill = [(m, n, h) for m, n in PORDER for h in range(2)]
        extra = list(range(L // SUB))
        y = None
        for tok in CFG['pre'].split():
            if tok == 'f':
                y = pj(*fill.pop(0))
            elif tok == 'x':
                ln1(1, extra.pop(0), y)
            elif tok in 'wW':
                @pl.when(first)
                def _():
                    if not CFG['vearly']:
                        cp_w(0, 2).wait()
                    cp_x1().wait()
                    if tok == 'W':
                        lax.fori_loop(0, CFG['n1'] // 4, lambda i, c: [ln1(1, 4 * i + j) for j in range(4)] and c, 0)
                extra = extra[CFG['n1'] * (tok == 'W'):]
                y = None
            else:
                nxt = attn_items(None, 0, None, None)
                nxt[2](int(tok[1]))
                nxt[3](int(tok[1]), 'store')
        assert not fill and not extra
        cp_xn().start()

        def pair(s, p, last=False):
            for par in range(2):
                group(s, 2 * p + par, par, last and par == 1)

        def seg0(p, c2):
            if not CFG['prewait']:
                @pl.when(first)
                def _():
                    for par in range(2):
                        cp_xr(2 * p + par).wait()
                    for j in range(3):
                        cp_w(2 * p + 1, j).wait()

                    @pl.when(p < NG // 2 - 1)
                    def _():
                        for j in range(3):
                            cp_w(jnp.minimum(2 * p + 2, NG - 2), j).wait()

                    @pl.when(p == NG // 2 - 1)
                    def _():
                        for cp in cp_wo():
                            cp.wait()
            pair(0, p)
            return c2
        _loop('s0', NG // 2, seg0)
        cp_xn().wait()

        @pl.when(first)
        def _():
            for cp in cp_ff():
                cp.start()

        def mid(t, c2):
            pair(1 + t // (NG // 2), t % (NG // 2))
            return c2
        _loop('s1', NG + (NG // 2 - 1) * CFG['merge3'], mid)

        def wait_ff():
            @pl.when(first)
            def _():
                for cp in cp_ff():
                    cp.wait()

            @pl.when(li == CFG['nl'] - 1)
            def _():
                for s in range(NSEG - 2):
                    cp_out_seg(s).wait()

        @pl.when(li == CFG['nl'] - 1)
        def _():
            cp_out_seg(0).start()
            cp_out_seg(1).start()

        def seg3(p, c2):
            pair(NSEG - 1, p)
            return c2
        if not CFG['merge3']:
            _loop('s3', NG // 2 - 1, seg3)
        wait_ff()
        pair(NSEG - 1, NG // 2 - 1, last=True)

        s = NSEG - 1
        pend = []
        r0 = L
        late, gate, step, glag = [], {}, 0, 0
        for rows, nlag in zip(CFG['tail'], CFG['glag']):
            r0 -= rows
            for n in range(NG):
                y = oproj(s, r0, rows, n, 4, NG, gate.pop(step, ()))
                if pend:
                    r, fin = pend.pop(0)(y)
                    late.append(fin)
                    if glag:
                        gate.setdefault(step + glag, []).append(r)
                step += 1
            pend = [lambda tok, r=r: ln2(s, r // CH, r % CH // SUB, tok, r < CFG['defer'])
                    for r in range(r0, r0 + rows, SUB)]
            glag = nlag
        assert r0 == 0
        late = [e for e in late + [e(None)[1] for e in pend] if e is not None]

        def start_out():
            cp_out_seg(NSEG - 2).start()
            cp_out_seg(NSEG - 1).start()
        if not late:
            start_out()

        rm = r_ref[...]
        rb = pltpu.bitcast(jnp.where(rm == 0.0, 0.0, rm), i32)
        lane = lax.broadcasted_iota(i32, (CH, 128), 1)
        base = jnp.where(lane < S // CH, (1 << 29) + S - 1 - lane * CH - lax.broadcasted_iota(i32, (CH, 128), 0), 0)
        mono = rb ^ ((rb >> 31) | jnp.int32(-2 ** 31))
        key = pltpu.bitcast(base + (lax.shift_right_logical(mono, 5) & 0x07FFF800), f32)
        k1 = jnp.max(key, axis=(0, 1), keepdims=True)
        k2 = jnp.max(jnp.where(key == k1, 0.0, key), axis=(0, 1), keepdims=True)
        toks = [jnp.clip(jnp.max((S - 1 - (pltpu.bitcast(k, i32) & (S - 1))).astype(f32)).astype(i32), 0, S - 1)
                for k in (k1, k2)]

        row = lax.broadcasted_iota(i32, (SUB, D), 0)
        x1s = jnp.concatenate([x1_ref[t >> 9, pl.ds(pl.multiple_of(t & (L - 8), 8), 8), :] for t in toks], axis=0)
        ms, rss = _stats(x1s)
        xs = ((x1s - ms) * rss).astype(bf16)
        hs, ys, todo = [], [None] * NG, list(range(L // SUB + CFG['n1'] * ('W' in CFG['pre'])))
        dlag, kc, snaps = CFG['dlag'], CFG['kc'], []

        two = int(len(todo) > NF + 7)

        def ffln(tok):
            r = todo.pop(0)
            ln1(r // (L // SUB), r % (L // SUB), tok, CFG['freload'])
        for c in range(NF + dlag):
            if c < NF:
                ga = _rb(_dot(xs, _unpack(wg_u[c])))
                up = _rb(_dot(xs, _unpack(wu_u[c])))
                hs.append((_rb(ga * _rb(jax.nn.sigmoid(ga))) * up).astype(bf16))
                ffln(ga)
                if two and len(todo) > NF - 1 - c:
                    ffln(up)
                if late:
                    late.pop(0)(ga)
                    if not late:
                        start_out()
            k = c - dlag + 1 - kc
            if k >= 0 and k % kc == 0:
                snaps.append(list(ys))
                if CFG['alag'] and len(snaps) > CFG['alag'] + 1:
                    t = None
                    for yv in snaps[-1 - CFG['alag'] + 1]:
                        for u in (yv[0:8], yv[8:16]):
                            t = pltpu.bitcast(u, u32) if t is None else t | pltpu.bitcast(u, u32)
                    hs[k] = pltpu.bitcast(pltpu.bitcast(hs[k], u32) | (t & z_ref[0:8, :]), bf16)
                h = jnp.concatenate(hs[k:k + kc], axis=1)
                for n in range(NG):
                    part = _dot(h, _unpack(wd_u[n, 64 * k:64 * (k + kc), :]))
                    ys[n] = part if ys[n] is None else ys[n] + part
                    if n % (NG >> two) == 0 and len(todo) > max(NF - 1 - c, 0) << two and c >= CFG['xln']:
                        ffln(part)
        assert not todo
        y = _rb(jnp.concatenate(ys, axis=1))
        ksel = pltpu.bitcast(jnp.where(lax.broadcasted_iota(i32, (SUB, 128), 0) < 8, k1, k2), i32)
        hi = (ksel << 5) & -65536
        rsel = pltpu.bitcast(jnp.where(hi < 0, hi ^ jnp.int32(-2 ** 31), ~hi & -65536), f32)[:, 0:1]
        y = _rb(y * _rb(jax.nn.sigmoid(rsel)))
        x2s = _rb(x1s + _rb(xs.astype(f32) + y))
        ms, rss = _stats(x2s)

        for s in range(NSEG - 2, NSEG):
            cp_out_seg(s).wait()

        blks = []
        for n, t in enumerate(toks):
            sg = t >> 9
            b0 = pl.multiple_of(t & (L - SUB), SUB)
            old = x_ref[sg, pl.ds(b0, SUB), :].astype(f32)
            x_ref[sg, pl.ds(b0, SUB), :] = jnp.where(
                row == (t & (SUB - 1)), jnp.tile(x2s[8 * n:8 * n + 8], (2, 1)), old).astype(bf16)
            blks.append((sg, b0))

        @pl.when(li < CFG['nl'] - 1)
        def _():
            xns = (x2s - ms) * rss
            for n, t in enumerate(toks):
                b2 = t & ((2 * L if 'W' in CFG['pre'] else L) - SUB)
                hb = pl.multiple_of(b2 >> 1, SUB // 2)
                oldn = _unpack(xa_ref[pl.ds(hb, SUB // 2), :]).astype(f32)
                xa_ref[pl.ds(hb, SUB // 2), :] = _pack(
                    jnp.where(row == t - b2, jnp.tile(xns[8 * n:8 * n + 8], (2, 1)), oldn))

        @pl.when(li == CFG['nl'] - 1)
        def _():
            def cp_fix(n):
                sg, b0 = blks[n]
                return pltpu.make_async_copy(x_ref.at[sg, pl.ds(b0, SUB), :],
                                             out_hbm.at[sg, pl.ds(b0, SUB), :], sems.at[SEM_FIX])
            differ = (toks[0] >> 4) != (toks[1] >> 4)
            cp_fix(0).start()

            @pl.when(differ)
            def _():
                cp_fix(1).start()
                cp_fix(1).wait()
            cp_fix(0).wait()
        return carry

    lax.fori_loop(0, CFG['nl'], layer, 0)


@jax.jit
def pallas_interleave_layers__memory_aug_infini_attn__moe_arch_mod__prompt_kernel(
    A_x: jax.Array,
    A_wq: jax.Array,
    A_wk: jax.Array,
    A_wv: jax.Array,
    A_wo: jax.Array,
    A_beta: jax.Array,
    B_x: jax.Array,
    B_w_r: jax.Array,
    B_w_gate: jax.Array,
    B_w_up: jax.Array,
    B_w_down: jax.Array,
):
    del B_x
    qkv_bufs = [pltpu.VMEM((L // 2, 512), u32), pltpu.VMEM((72, L), u32)]
    scratch = [
        pltpu.VMEM((8 * CFG['zpad'], 128), u32),
        pltpu.VMEM((NSEG, L, D), bf16),
        pltpu.VMEM((3 * L // 2, D), u32),
        pltpu.VMEM((NSEG, L, D), f32),
        pltpu.VMEM((3 * NG, D, 128), bf16),
        pltpu.VMEM((NG, D, 128), bf16),
        pltpu.VMEM((NF, D, 128), bf16),
        pltpu.VMEM((NF, D, 128), bf16),
        pltpu.VMEM((NG, F, 128), bf16),
        pltpu.VMEM((64, 128), f32),
        pltpu.VMEM((32, 128), f32),
        pltpu.VMEM((NG, 144, 128), f32),
        pltpu.VMEM((CH, 128), f32),
        pltpu.VMEM((144, L), f32),
        pltpu.VMEM((128, L), f32), pltpu.VMEM((256, L), f32),
        pltpu.VMEM((384, L), f32), pltpu.VMEM((512, L), f32),
        pltpu.VMEM((64, L), u32), pltpu.VMEM((128, L), u32),
        pltpu.VMEM((192, L), u32), pltpu.VMEM((256, L), u32),
        *qkv_bufs, *qkv_bufs,
        pltpu.VMEM((NG * L // 2, 256), u32),
        pltpu.VMEM((L, D), u32),
        pltpu.VMEM((16, D), f32),
        pltpu.VMEM((24 + 8 * CFG['mpad'], 128), f32),
        pltpu.VMEM((8, 128), bf16),
        pltpu.VMEM((1, 32), bf16),
        pltpu.SemaphoreType.DMA((NSEM,)),
    ]
    out = pl.pallas_call(
        _kernel,
        out_shape=jax.ShapeDtypeStruct((NSEG, L, D), bf16),
        in_specs=[pl.BlockSpec(memory_space=pl.ANY)] * 10,
        out_specs=pl.BlockSpec(memory_space=pl.ANY),
        scratch_shapes=scratch,
        compiler_params=pltpu.CompilerParams(vmem_limit_bytes=100 * 2 ** 20),
    )(A_x.reshape(NSEG, L, D), A_wq, A_wk, A_wv, A_wo, A_beta.reshape(1, 32), B_w_r.reshape(8, 128),
      B_w_gate, B_w_up, B_w_down)
    return out.reshape(1, S, D)
```

```python
import jax
import jax.numpy as jnp
from jax import lax
import jax.experimental.pallas as pl
import jax.experimental.pallas.tpu as pltpu

bf16 = jnp.bfloat16
f32 = jnp.float32
u32 = jnp.uint32
i32 = jnp.int32

S = 2048
D = 1024
L = 512
NSEG = 4
NG = 8
F = 3584
CH = 64
SUB = 16
NEG = -1e30
QSCALE = (32 ** -0.5) * 1.4426950408889634
NT = (((1,), (1,)), ((), ()))

SEM_XC = 0
SEM_W0 = 4
SEM_X1 = 5
SEM_SM = 6
SEM_P = 7
NSEM = 11
SEM_OUT, SEM_FIX, SEM_FF, SEM_XN = 0, 1, 2, 3
NF = F // 128
PORDER = [(m, n) for m in range(4) for n in range(2)] + [(m, 2) for m in range(4)]

CFG = dict(
    tail=(128, 128, 128, 64, 32, 32), defer=64, dlag=2, kc=4, xln=4, alag=0, n1=32, wun=8, vearly=1, mpad=2, glag=(0, 0, 0, 0, 0, 0), rep={}, cnt={}, merge3=0, zpad=4, issue='abcdqkvsr x', lnmode=0, nl=2, prewait=False, gp=2, pace=True, pace2=True, one=True, reload=True, chain=True, xfrac=0.0, freload=False, lag=0, fskip=0,
    pre='f ' * 18 + 'Q3 ' + 'f ' * 6 + 'W',
    sched='M3 f p30 f n q2 v30 p31 f f v31 p32 f f m2 v32 p33 f f v33 p20 f f q1 v20 p21 f x f v21 p22 f x f '
          'm1 v22 p10 f x f q0 v10 p11 f x f u v11 m0 f p00 f f v00 F Q3',
    sched0='M3 f p30 f q2 v30 p31 f f v31 p32 f f x m2 v32 p33 f f x v33 p20 f f x q1 v20 p21 f f x '
           'v21 p22 f f x m1 v22 p10 f f x q0 v10 p11 f x f u v11 m0 f x p00 f f v00 F Q3',
    schedL='M3 f p30 f n q2 v30 p31 f f v31 p32 f f m2 v32 p33 f f v33 p20 f f q1 v20 p21 f x f v21 p22 f x f '
          'm1 v22 p10 f x f q0 v10 p11 f x f v11 m0 f p00 f f v00 F',
)


def _loop(name, n, body):
    rep = CFG['rep'].get(name, 1)
    n = CFG['cnt'].get(name, n)
    if n == 0:
        return 0
    if rep == 1:
        return lax.fori_loop(0, n, body, 0)
    return lax.fori_loop(0, n * rep, lambda i, c: body(i // rep, c), 0)


def _rb(x):
    return x.astype(bf16).astype(f32)


def _pack(x):
    return pltpu.bitcast(x.astype(bf16), u32)


def _unpack(u):
    return pltpu.bitcast(u, bf16)


def _phi(t):
    return jnp.where(t > 0, t + 1.0, jnp.exp(t))


def _dot(a, b):
    return jnp.dot(a, b, preferred_element_type=f32)


def _unskew(ps):
    shape, dt = next((p.shape, p.dtype) for p in ps if p is not None)
    c = lax.broadcasted_iota(i32, shape, 1) >> 5
    even = (c & 1) == 0
    lo = c < 2
    mid = jnp.logical_or(c == 1, c == 2)

    def sel(mask, a, b):
        if a is None and b is None:
            return None
        z = jnp.zeros(shape, dt)
        return jnp.where(mask, z if a is None else a, z if b is None else b)
    x0, x1 = sel(even, ps[0], ps[1]), sel(even, ps[1], ps[0])
    x2, x3 = sel(even, ps[2], ps[3]), sel(even, ps[3], ps[2])
    return [sel(lo, x0, x2), sel(mid, x1, x3), sel(lo, x2, x0), sel(mid, x3, x1)]


def _ln(x, mode=0):
    acc = x
    if CFG['chain']:
        acc = x[:, 0:128]
        for c in range(1, x.shape[1] // 128):
            acc = acc + x[:, 128 * c:128 * c + 128]
    m = jnp.sum(acc, axis=-1, keepdims=True) * (1.0 / D)
    if mode == 0:
        e = x - m
        v = jnp.sum(e * e, axis=-1, keepdims=True) * (1.0 / D)
        return e * lax.rsqrt(v + 1e-5)
    c = _rb(m)
    e = x - c
    v = jnp.sum(e * e, axis=-1, keepdims=True) * (1.0 / D) - (m - c) * (m - c)
    w = _rb(_rb(jnp.maximum(v, 0.0)) + 1e-5)
    den = _rb(w * lax.rsqrt(w))
    if mode == 2:
        return _rb(_rb(e) / den)
    return e * (1.0 / den)


def _rowsum(x, first=None):
    acc = x[:, 0:128] if first is None else first
    for c in range(1, x.shape[1] // 128):
        acc = acc + x[:, 128 * c:128 * c + 128]
    return jnp.sum(acc, axis=-1, keepdims=True)


def _stats(x):
    m = _rowsum(x) * (1.0 / D)
    v = jnp.maximum(_rowsum(x * x) * (1.0 / D) - m * m, 0.0)
    return m, lax.rsqrt(v + 1e-5)


def _kernel(x_hbm, wq_hbm, wk_hbm, wv_hbm, wo_hbm, beta_hbm, wr_hbm, wg_hbm, wu_hbm, wd_hbm,
            out_hbm,
            z_ref, x_ref, xb_ref, x1_ref, w_ref, wo_ref, wg_ref, wu_ref, wd_ref,
            gate_ref, bias_ref, m_ref, r_ref, nd_ref,
            s0_ref, s1_ref, s2_ref, s3_ref, p0_ref, p1_ref, p2_ref, p3_ref,
            qk0, vt0, qk1, vt1, o_ref, xa_ref, wrf_ref, mx_ref, wr_ref, beta_ref, sems):
    qkv = ((qk0, vt0), (qk1, vt1))
    s_refs = (s0_ref, s1_ref, s2_ref, s3_ref)
    p_refs = (p0_ref, p1_ref, p2_ref, p3_ref)
    xa_b, xb_b = xa_ref.bitcast(bf16), xb_ref.bitcast(bf16)
    w_u, wo_u, wg_u, wu_u, wd_u = (r.bitcast(u32) for r in (w_ref, wo_ref, wg_ref, wu_ref, wd_ref))

    def cp_x0(c):
        rows = pl.ds(pl.multiple_of(128 * c, 128), 128)
        return pltpu.make_async_copy(x_hbm.at[0, rows], x_ref.at[0, rows], sems.at[SEM_XC + c])

    def cp_x1():
        return pltpu.make_async_copy(x_hbm.at[1], x_ref.at[1], sems.at[SEM_X1])

    def cp_xn():
        return pltpu.make_async_copy(xa_ref.at[L // 2:L], xb_ref.at[0:L // 2], sems.at[SEM_XN])

    def cp_xr(g):
        r0 = pl.multiple_of(g * CH, CH)
        return pltpu.make_async_copy(x_hbm.at[2:NSEG, pl.ds(r0, CH), :],
                                     x_ref.at[2:NSEG, pl.ds(r0, CH), :], sems.at[SEM_P + g // 2])

    def cp_w(g, j):
        c0 = pl.multiple_of(g * 128, 128)
        src = (wq_hbm, wk_hbm, wv_hbm)[j]
        sem = (SEM_W0 + j // 2 * (1 - CFG['vearly'])) if isinstance(g, int) and g == 0 else SEM_P + (g - 1) // 2
        return pltpu.make_async_copy(src.at[:, pl.ds(c0, 128)], w_ref.at[3 * g + j], sems.at[sem])

    def slabs(src, dst, n, sem):
        return [pltpu.make_async_copy(src.at[:, 128 * c:128 * c + 128], dst.at[c], sems.at[sem]) for c in range(n)]

    def cp_wo():
        return slabs(wo_hbm, wo_ref, NG, SEM_P + 3)

    def cp_small():
        return (pltpu.make_async_copy(beta_hbm, beta_ref, sems.at[SEM_SM]),
                pltpu.make_async_copy(wr_hbm, wr_ref, sems.at[SEM_SM]))

    def cp_ff():
        return (slabs(wg_hbm, wg_ref, NF, SEM_FF) + slabs(wu_hbm, wu_ref, NF, SEM_FF)
                + slabs(wd_hbm, wd_ref, NG, SEM_FF))

    def cp_out_seg(s):
        return pltpu.make_async_copy(x_ref.at[s], out_hbm.at[s], sems.at[SEM_OUT])

    def after(x, tok, frac):
        if tok is None or not CFG['pace']:
            return x
        r = 8 * int(frac * tok.shape[0] // 8)
        t = pltpu.bitcast(tok[r:r + 8, 0:128], u32) & z_ref[0:8, :]
        t = jnp.tile(t, (x.shape[0] // 8, x.shape[1] // 128))
        return pltpu.bitcast(pltpu.bitcast(x, u32) | t, x.dtype)

    def proj_items(s, nxt, g, par):
        xn_r, seg = (xa_ref, nxt) if isinstance(s, int) and s == 0 else (xb_ref, s - 1 + nxt)
        qk_r, vt_r = (r.bitcast(bf16) for r in qkv[par])
        part = {}

        def item(m, n, h):
            xn = _unpack(xn_r[pl.ds(pl.multiple_of(seg * (L // 2) + 64 * m, 64), 64), 512 * h:512 * h + 512])
            y = _dot(xn, _unpack(w_u[3 * g + n, 256 * h:256 * h + 256, :]))
            if h == 0:
                part[m, n] = y
                return y
            y = y + part.pop((m, n))
            rows = slice(128 * m, 128 * m + 128)
            if n == 0:
                qk_r[rows, 0:128] = (y * QSCALE).astype(bf16)
                qk_r[rows, 128:256] = _phi(y).astype(bf16)
            elif n == 1:
                qk_r[rows, 256:384] = y.astype(bf16)
                qk_r[rows, 384:512] = _phi(y).astype(bf16)
            else:
                vt_r[0:128, rows] = y.T.astype(bf16)
            return y
        return item

    def attn_items(g, par, seg, use_mem):
        qk_r, vt_r = qkv[par]
        st = {}

        def nd():
            ml = m_ref[g].astype(bf16)
            nd_ref[...] = lax.dot_general(ml, _unpack(qk_r[:, 128:256]), NT, preferred_element_type=f32)

        def upd():
            u = _dot(_unpack(vt_r[...]), _unpack(qk_r[:, 384:512]))
            r2 = lax.broadcasted_iota(i32, (144, 128), 0)
            c2 = lax.broadcasted_iota(i32, (144, 128), 1) >> 5
            keep = jnp.where(r2 < 128, r2 >> 5, r2 - 128) == c2
            u = jnp.where(keep, u, 0.0)
            m_ref[g] = (m_ref[g] + u) if use_mem else u

        def qk(i):
            lane = lax.broadcasted_iota(i32, (16, 128), 1) >> 5
            for be in (range(4) if i % 2 else range(3, -1, -1)):
                b = 4 * i + be
                n = 32 * (b + 1)
                qu = qk_r[16 * b:16 * b + 16, 0:128]
                wq = _unpack(jnp.concatenate(
                    [jnp.where(lane == (c - be) % 4, qu, jnp.uint32(0)) for c in range(4)], axis=0))
                s = lax.dot_general(_unpack(qk_r[0:n // 2, 256:384]), wq, NT, preferred_element_type=f32)
                cols = slice(128 * be, 128 * be + 128)
                if b > 0:
                    s_refs[i][0:n - 32, cols] = s[0:n - 32]
                s_refs[i][n - 32:n, cols] = s[n - 32:n] + bias_ref[...]

        def mx(i, mode='m'):
            for be in range(4):
                if mode == 'load':
                    st[i, 'm', be] = mx_ref[4 * i + be:4 * i + be + 1, :]
                    continue
                n = 32 * (4 * i + be + 1)
                sv = s_refs[i][0:n, 128 * be:128 * be + 128]
                m = jnp.max(jnp.max(sv.reshape(n // 8, 8, 128), axis=0), axis=0, keepdims=True)
                if mode == 'store':
                    mx_ref[4 * i + be:4 * i + be + 1, :] = m
                else:
                    st[i, 'm', be] = m

        def pr(i, t, tok):
            ps = []
            for be in range(4):
                n = 128 if t < i else 32 * (be + 1)
                m8 = after(jnp.broadcast_to(st[i, 'm', be], (8, 128)), tok, be / 4)
                p = jnp.exp2(s_refs[i][128 * t:128 * t + n, 128 * be:128 * be + 128].reshape(n // 8, 8, 128) - m8)
                ls = jnp.sum(p, axis=0)
                p = p.reshape(n, 128)
                st[i, 'l', be] = ls if t == 0 else st[i, 'l', be] + ls
                p_refs[i].bitcast(bf16)[128 * t:128 * t + n, 128 * be:128 * be + 128] = p.astype(bf16)

        def pv(i, t):
            ps = [p_refs[i][64 * t:64 * t + (64 if t < i else 16 * (be + 1)), 128 * be:128 * be + 128]
                  for be in range(4)]
            if t < i:
                ts = _unskew(ps)
            else:
                blk = [_unskew([ps[be][16 * u:16 * u + 16] if be >= u else None for be in range(4)])
                       for u in range(4)]
                ts = [jnp.concatenate([blk[u][j] for u in range(4)], axis=0) for j in range(4)]
            for j in range(4):
                o = _dot(_unpack(vt_r[16 * j:16 * j + 16, 128 * t:128 * t + 128]), _unpack(ts[j]))
                st[i, 'o', j] = o if t == 0 else st[i, 'o', j] + o

        def fin(i):
            ls = _unskew([jnp.sum(st.pop((i, 'l', be)), axis=0, keepdims=True) for be in range(4)])
            parts = []
            for j in range(4):
                gt = gate_ref[pl.ds(4 * g + j, 1), :]
                omg = gate_ref[pl.ds(32 + 4 * g + j, 1), :]
                o = st.pop((i, 'o', j)) * (omg / ls[j])
                if j > 0:
                    o = pltpu.roll(o, 128 - 32 * j, 1)
                if use_mem:
                    den = nd_ref[128 + j:129 + j, 128 * i:128 * i + 128] + 1e-6
                    o = o + nd_ref[32 * j:32 * j + 32, 128 * i:128 * i + 128] * (gt / den)
                parts.append(o)
            ot = jnp.concatenate(parts, axis=0)
            o_ref.bitcast(bf16)[pl.ds(pl.multiple_of((seg % 2 * 4 + g // 2) * L + 128 * i, 128), 128),
                                128 * par:128 * par + 128] = ot.T.astype(bf16)

        def ex(kind, i, t, tok):
            if kind in 'ep':
                pr(i, t, tok)
            if kind in 'ev':
                pv(i, t)
                if t == i:
                    fin(i)
        return nd, upd, qk, mx, ex

    def ln1(seg, r, tok=None, reload=True):
        r0 = pl.multiple_of(r * SUB, SUB)
        x = x_ref[seg, pl.ds(r0, SUB), :].astype(f32)
        if tok is not None:
            x = jnp.concatenate([after(x[:, 0:128], tok, CFG['xfrac']), x[:, 128:]], axis=1)
        if CFG['one']:
            m, rs = _stats(x)
            if CFG['reload'] and reload:
                mx_ref[16:24, :] = jnp.broadcast_to(m[0:8], (8, 128))
                x = x_ref[seg, pl.ds(r0, SUB), :].astype(f32)
            xn = ((x - m) * rs).astype(bf16)
        else:
            xn = _ln(x).astype(bf16)
        if seg < 2:
            xa_b[pl.ds(pl.multiple_of(seg * L + r0, SUB), SUB), :] = xn
        else:
            xb_b[pl.ds(pl.multiple_of((seg - 1) * L + r0, SUB), SUB), :] = xn
        return xn

    def oproj(seg, r0, rows, n, k0=0, k1=NG, deps=()):
        h0 = pl.multiple_of(r0 // 2, rows // 2)
        r0 = pl.multiple_of(r0, rows)
        lhs = jnp.concatenate(
            [o_ref[pl.ds(pl.multiple_of((seg % 2 * 4 + p) * (L // 2) + h0, rows // 2), rows // 2), :]
             for p in range(k0 // 2, k1 // 2)], axis=1)
        for d in deps:
            top = jnp.concatenate([after(lhs[0:8, 0:128], d, 0.0), lhs[0:8, 128:]], axis=1)
            lhs = jnp.concatenate([top, lhs[8:]], axis=0)
        lhs = _unpack(lhs)
        y = _dot(lhs, _unpack(wo_u[n, 64 * k0:64 * k1, :]))
        cols = slice(128 * n, 128 * n + 128)
        if k0 > 0:
            y = y + x1_ref[seg, pl.ds(r0, rows), cols]
        if k1 == NG:
            y = _rb(x_ref[seg, pl.ds(r0, rows), cols].astype(f32) + y)
        x1_ref[seg, pl.ds(r0, rows), cols] = y
        return y

    def ln2(seg, c, t, tok=None, defer=False):
        r0 = pl.multiple_of(c * CH + t * SUB, SUB)
        lane = lax.broadcasted_iota(i32, (SUB, 128), 1)
        x1 = x1_ref[seg, pl.ds(r0, SUB), :]
        if tok is not None and CFG['pace2']:
            x1 = jnp.concatenate([after(x1[:, 0:128], tok, CFG['xfrac']), x1[:, 128:]], axis=1)
        if CFG['one']:
            m, rs = _stats(x1)
            r = _rb((_rowsum(x1 * jnp.tile(wrf_ref[0:8, :], (2, 1))) - m * jnp.tile(wrf_ref[8:16, 0:128], (2, 1))) * rs)
        else:
            xn2 = _ln(x1, CFG['lnmode'])
            r = _rb(jnp.sum(xn2 * wrf_ref[0:1, :], axis=-1, keepdims=True))
        r_ref[SUB * t:SUB * t + SUB, :] = jnp.where(lane == seg * NG + c, r, r_ref[SUB * t:SUB * t + SUB, :])

        def fin(tok2=None):
            if CFG['one']:
                xr = x1_ref[seg, pl.ds(r0, SUB), :] if CFG['reload'] else x1
                if tok2 is not None:
                    xr = jnp.concatenate([after(xr[:, 0:128], tok2, CFG['xfrac']), xr[:, 128:]], axis=1)
                x2 = xr * (1.0 + rs) - m * rs
            else:
                x2 = x1 + xn2
            x_ref[seg, pl.ds(r0, SUB), :] = x2.astype(bf16)
        if defer:
            return r, fin
        fin()
        return r, None

    def group(s, g, par, last=False):
        kind = s if isinstance(s, int) else 1
        nd, upd, qk, mx, ex = attn_items(g, par, s, kind > 0)
        fill = []
        extra = []
        if kind > 0:
            for n in range(NG):
                fill.append((128, lambda n=n: oproj(s - 1, g * CH, CH, n)))
            extra = [lambda tok, t=t: ln2(s - 1, g, t, tok) for t in range(CH // SUB)]
        else:
            extra = [lambda tok, seg=seg, t=t: ln1(seg, g * (CH // SUB) + t, tok)
                     for seg in range(2, NSEG) for t in range(CH // SUB)]
        if not last:
            gn = g + 1
            pj = proj_items(s, gn // NG, gn % NG, 1 - par)
            for m, n in PORDER:
                for h in range(2):
                    fill.append((128, lambda m=m, n=n, h=h: pj(m, n, h)))
        else:
            for m in range(4):
                for n in range(NG):
                    fill.append((128, lambda m=m, n=n: oproj(s, 128 * m, 128, n, 0, 4)))
        sched = CFG['sched0' if kind == 0 else 'schedL' if last else 'sched'].split()
        y = None
        for tok in sched:
            if tok == 'f':
                y = fill.pop(0)[1]()
            elif tok == 'F':
                while fill:
                    fill.pop(0)[1]()
            elif tok == 'x':
                extra.pop(0)(y)
            elif tok == 'n':
                nd()
            elif tok == 'u':
                if kind < NSEG - 1:
                    upd()
            elif tok[0] == 'q':
                qk(int(tok[1]))
            elif tok[0] == 'Q':
                nxt = attn_items(None, 1 - par, None, None)
                nxt[2](int(tok[1]))
                nxt[3](int(tok[1]), 'store')
            elif tok[0] == 'M':
                mx(int(tok[1]), 'load')
            elif tok[0] == 'm':
                mx(int(tok[1]))
            else:
                ex(tok[0], int(tok[1]), int(tok[2]), y)
        for it in fill:
            it[1]()
        for e in extra:
            e(None)

    early = {'a': cp_x0(0), 'b': cp_x0(1), 'c': cp_x0(2), 'd': cp_x0(3), 'q': cp_w(0, 0), 'k': cp_w(0, 1),
             'v': cp_w(0, 2), 'x': cp_x1(), **dict(zip('sr', cp_small()))}
    issue = CFG['issue'].split()
    for k in issue[0]:
        early[k].start()

    z_ref[0:8, :] = jnp.zeros((8, 128), u32)
    ones = jnp.full((8, 512), 0x3F803F80, u32)
    vt0[64:72, :] = ones
    vt1[64:72, :] = ones
    bias_ref[...] = jnp.where(lax.broadcasted_iota(i32, (32, 128), 0)
                              <= (lax.broadcasted_iota(i32, (32, 128), 1) & 31), 0.0, NEG)

    def ln0_body(c, carry):
        cp_x0(c).wait()
        for n in range(1, len(issue)):
            @pl.when(c == n - 1)
            def _():
                for k in issue[n].strip('-'):
                    early[k].start()
        for t in range(128 // SUB):
            ln1(0, c * (128 // SUB) + t)
        return carry
    lax.fori_loop(0, 4, ln0_body, 0)
    for g in range(1, NG):
        for j in range(3):
            cp_w(g, j).start()
        cp_xr(g - 1).start()
    cp_xr(NG - 1).start()
    for cp in cp_wo():
        cp.start()

    for cp in cp_small():
        cp.wait()
    wr = wr_ref[...].astype(f32)
    for c in range(D // 128):
        wrf_ref[0:8, 128 * c:128 * c + 128] = jnp.broadcast_to(wr[c:c + 1, :], (8, 128))
    wrf_ref[8:16, :] = jnp.broadcast_to(jnp.sum(wr, axis=(0, 1), keepdims=True), (8, D))
    gl = _rb(jax.nn.sigmoid(beta_ref[...].astype(f32)))
    hr = lax.broadcasted_iota(i32, (32, 32), 0)
    hc = lax.broadcasted_iota(i32, (32, 32), 1)
    gcol = jnp.sum(jnp.where(hr == hc, gl, 0.0), axis=1, keepdims=True)
    gate_ref[0:32, :] = jnp.broadcast_to(gcol, (32, 128))
    gate_ref[32:64, :] = jnp.broadcast_to(_rb(1.0 - gcol), (32, 128))
    for j in range(2 + CFG['vearly']):
        cp_w(0, j).wait()
    if CFG['prewait']:
        for g in range(NG):
            cp_xr(g).wait()
            for j in range(3 * (g > 0)):
                cp_w(g, j).wait()
        for cp in cp_wo():
            cp.wait()

    def layer(li, carry):
        first = li == 0
        r_ref[...] = jnp.full((CH, 128), -jnp.inf, f32)
        pj = proj_items(0, 0, 0, 0)
        fill = [(m, n, h) for m, n in PORDER for h in range(2)]
        extra = list(range(L // SUB))
        y = None
        for tok in CFG['pre'].split():
            if tok == 'f':
                y = pj(*fill.pop(0))
            elif tok == 'x':
                ln1(1, extra.pop(0), y)
            elif tok in 'wW':
                @pl.when(first)
                def _():
                    if not CFG['vearly']:
                        cp_w(0, 2).wait()
                    cp_x1().wait()
                    if tok == 'W':
                        wu = CFG['wun']
                        lax.fori_loop(0, CFG['n1'] // wu, lambda i, c: [ln1(1, wu * i + j) for j in range(wu)] and c, 0)
                extra = extra[CFG['n1'] * (tok == 'W'):]
                y = None
            else:
                nxt = attn_items(None, 0, None, None)
                nxt[2](int(tok[1]))
                nxt[3](int(tok[1]), 'store')
        assert not fill and not extra
        cp_xn().start()

        def pair(s, p, last=False):
            for par in range(2):
                group(s, 2 * p + par, par, last and par == 1)

        def seg0(p, c2):
            if not CFG['prewait']:
                @pl.when(first)
                def _():
                    for par in range(2):
                        cp_xr(2 * p + par).wait()
                    for j in range(3):
                        cp_w(2 * p + 1, j).wait()

                    @pl.when(p < NG // 2 - 1)
                    def _():
                        for j in range(3):
                            cp_w(jnp.minimum(2 * p + 2, NG - 2), j).wait()

                    @pl.when(p == NG // 2 - 1)
                    def _():
                        for cp in cp_wo():
                            cp.wait()
            pair(0, p)
            return c2
        _loop('s0', NG // 2, seg0)
        cp_xn().wait()

        @pl.when(first)
        def _():
            for cp in cp_ff():
                cp.start()

        def mid(t, c2):
            pair(1 + t // (NG // 2), t % (NG // 2))
            return c2
        _loop('s1', NG + (NG // 2 - 1) * CFG['merge3'], mid)

        def wait_ff():
            @pl.when(first)
            def _():
                for cp in cp_ff():
                    cp.wait()

            @pl.when(li == CFG['nl'] - 1)
            def _():
                for s in range(NSEG - 2):
                    cp_out_seg(s).wait()

        @pl.when(li == CFG['nl'] - 1)
        def _():
            cp_out_seg(0).start()
            cp_out_seg(1).start()

        def seg3(p, c2):
            pair(NSEG - 1, p)
            return c2
        if not CFG['merge3']:
            _loop('s3', NG // 2 - 1, seg3)
        wait_ff()
        pair(NSEG - 1, NG // 2 - 1, last=True)

        s = NSEG - 1
        pend = []
        r0 = L
        late, gate, step, glag = [], {}, 0, 0
        for rows, nlag in zip(CFG['tail'], CFG['glag']):
            r0 -= rows
            for n in range(NG):
                y = oproj(s, r0, rows, n, 4, NG, gate.pop(step, ()))
                if pend:
                    r, fin = pend.pop(0)(y)
                    late.append(fin)
                    if glag:
                        gate.setdefault(step + glag, []).append(r)
                step += 1
            pend = [lambda tok, r=r: ln2(s, r // CH, r % CH // SUB, tok, r < CFG['defer'])
                    for r in range(r0, r0 + rows, SUB)]
            glag = nlag
        assert r0 == 0
        late = [e for e in late + [e(None)[1] for e in pend] if e is not None]

        def start_out():
            cp_out_seg(NSEG - 2).start()
            cp_out_seg(NSEG - 1).start()
        if not late:
            start_out()

        rm = r_ref[...]
        rb = pltpu.bitcast(jnp.where(rm == 0.0, 0.0, rm), i32)
        lane = lax.broadcasted_iota(i32, (CH, 128), 1)
        base = jnp.where(lane < S // CH, (1 << 29) + S - 1 - lane * CH - lax.broadcasted_iota(i32, (CH, 128), 0), 0)
        mono = rb ^ ((rb >> 31) | jnp.int32(-2 ** 31))
        key = pltpu.bitcast(base + (lax.shift_right_logical(mono, 5) & 0x07FFF800), f32)
        k1 = jnp.max(key, axis=(0, 1), keepdims=True)
        k2 = jnp.max(jnp.where(key == k1, 0.0, key), axis=(0, 1), keepdims=True)
        toks = [jnp.clip(jnp.max((S - 1 - (pltpu.bitcast(k, i32) & (S - 1))).astype(f32)).astype(i32), 0, S - 1)
                for k in (k1, k2)]

        row = lax.broadcasted_iota(i32, (SUB, D), 0)
        x1s = jnp.concatenate([x1_ref[t >> 9, pl.ds(pl.multiple_of(t & (L - 8), 8), 8), :] for t in toks], axis=0)
        ms, rss = _stats(x1s)
        xs = ((x1s - ms) * rss).astype(bf16)
        hs, ys, todo = [], [None] * NG, list(range(L // SUB + CFG['n1'] * ('W' in CFG['pre'])))
        dlag, kc, snaps = CFG['dlag'], CFG['kc'], []

        two = int(len(todo) > NF + 7)

        def ffln(tok):
            r = todo.pop(0)
            ln1(r // (L // SUB), r % (L // SUB), tok, CFG['freload'])
        for c in range(NF + dlag):
            if c < NF:
                ga = _rb(_dot(xs, _unpack(wg_u[c])))
                up = _rb(_dot(xs, _unpack(wu_u[c])))
                hs.append((_rb(ga * _rb(jax.nn.sigmoid(ga))) * up).astype(bf16))
                ffln(ga)
                if two and len(todo) > NF - 1 - c:
                    ffln(up)
                if late:
                    late.pop(0)(ga)
                    if not late:
                        start_out()
            k = c - dlag + 1 - kc
            if k >= 0 and k % kc == 0:
                snaps.append(list(ys))
                if CFG['alag'] and len(snaps) > CFG['alag'] + 1:
                    t = None
                    for yv in snaps[-1 - CFG['alag'] + 1]:
                        for u in (yv[0:8], yv[8:16]):
                            t = pltpu.bitcast(u, u32) if t is None else t | pltpu.bitcast(u, u32)
                    hs[k] = pltpu.bitcast(pltpu.bitcast(hs[k], u32) | (t & z_ref[0:8, :]), bf16)
                h = jnp.concatenate(hs[k:k + kc], axis=1)
                for n in range(NG):
                    part = _dot(h, _unpack(wd_u[n, 64 * k:64 * (k + kc), :]))
                    ys[n] = part if ys[n] is None else ys[n] + part
                    if n % (NG >> two) == 0 and len(todo) > max(NF - 1 - c, 0) << two and c >= CFG['xln']:
                        ffln(part)
        assert not todo
        y = _rb(jnp.concatenate(ys, axis=1))
        ksel = pltpu.bitcast(jnp.where(lax.broadcasted_iota(i32, (SUB, 128), 0) < 8, k1, k2), i32)
        hi = (ksel << 5) & -65536
        rsel = pltpu.bitcast(jnp.where(hi < 0, hi ^ jnp.int32(-2 ** 31), ~hi & -65536), f32)[:, 0:1]
        y = _rb(y * _rb(jax.nn.sigmoid(rsel)))
        x2s = _rb(x1s + _rb(xs.astype(f32) + y))
        ms, rss = _stats(x2s)

        for s in range(NSEG - 2, NSEG):
            cp_out_seg(s).wait()

        blks = []
        for n, t in enumerate(toks):
            sg = t >> 9
            b0 = pl.multiple_of(t & (L - SUB), SUB)
            old = x_ref[sg, pl.ds(b0, SUB), :].astype(f32)
            x_ref[sg, pl.ds(b0, SUB), :] = jnp.where(
                row == (t & (SUB - 1)), jnp.tile(x2s[8 * n:8 * n + 8], (2, 1)), old).astype(bf16)
            blks.append((sg, b0))

        @pl.when(li < CFG['nl'] - 1)
        def _():
            xns = (x2s - ms) * rss
            for n, t in enumerate(toks):
                b2 = t & ((2 * L if 'W' in CFG['pre'] else L) - SUB)
                hb = pl.multiple_of(b2 >> 1, SUB // 2)
                oldn = _unpack(xa_ref[pl.ds(hb, SUB // 2), :]).astype(f32)
                xa_ref[pl.ds(hb, SUB // 2), :] = _pack(
                    jnp.where(row == t - b2, jnp.tile(xns[8 * n:8 * n + 8], (2, 1)), oldn))

        @pl.when(li == CFG['nl'] - 1)
        def _():
            def cp_fix(n):
                sg, b0 = blks[n]
                return pltpu.make_async_copy(x_ref.at[sg, pl.ds(b0, SUB), :],
                                             out_hbm.at[sg, pl.ds(b0, SUB), :], sems.at[SEM_FIX])
            differ = (toks[0] >> 4) != (toks[1] >> 4)
            cp_fix(0).start()

            @pl.when(differ)
            def _():
                cp_fix(1).start()
                cp_fix(1).wait()
            cp_fix(0).wait()
        return carry

    lax.fori_loop(0, CFG['nl'], layer, 0)


@jax.jit
def pallas_interleave_layers__memory_aug_infini_attn__moe_arch_mod__prompt_kernel(
    A_x: jax.Array,
    A_wq: jax.Array,
    A_wk: jax.Array,
    A_wv: jax.Array,
    A_wo: jax.Array,
    A_beta: jax.Array,
    B_x: jax.Array,
    B_w_r: jax.Array,
    B_w_gate: jax.Array,
    B_w_up: jax.Array,
    B_w_down: jax.Array,
):
    del B_x
    qkv_bufs = [pltpu.VMEM((L // 2, 512), u32), pltpu.VMEM((72, L), u32)]
    scratch = [
        pltpu.VMEM((8 * CFG['zpad'], 128), u32),
        pltpu.VMEM((NSEG, L, D), bf16),
        pltpu.VMEM((3 * L // 2, D), u32),
        pltpu.VMEM((NSEG, L, D), f32),
        pltpu.VMEM((3 * NG, D, 128), bf16),
        pltpu.VMEM((NG, D, 128), bf16),
        pltpu.VMEM((NF, D, 128), bf16),
        pltpu.VMEM((NF, D, 128), bf16),
        pltpu.VMEM((NG, F, 128), bf16),
        pltpu.VMEM((64, 128), f32),
        pltpu.VMEM((32, 128), f32),
        pltpu.VMEM((NG, 144, 128), f32),
        pltpu.VMEM((CH, 128), f32),
        pltpu.VMEM((144, L), f32),
        pltpu.VMEM((128, L), f32), pltpu.VMEM((256, L), f32),
        pltpu.VMEM((384, L), f32), pltpu.VMEM((512, L), f32),
        pltpu.VMEM((64, L), u32), pltpu.VMEM((128, L), u32),
        pltpu.VMEM((192, L), u32), pltpu.VMEM((256, L), u32),
        *qkv_bufs, *qkv_bufs,
        pltpu.VMEM((NG * L // 2, 256), u32),
        pltpu.VMEM((L, D), u32),
        pltpu.VMEM((16, D), f32),
        pltpu.VMEM((24 + 8 * CFG['mpad'], 128), f32),
        pltpu.VMEM((8, 128), bf16),
        pltpu.VMEM((1, 32), bf16),
        pltpu.SemaphoreType.DMA((NSEM,)),
    ]
    out = pl.pallas_call(
        _kernel,
        out_shape=jax.ShapeDtypeStruct((NSEG, L, D), bf16),
        in_specs=[pl.BlockSpec(memory_space=pl.ANY)] * 10,
        out_specs=pl.BlockSpec(memory_space=pl.ANY),
        scratch_shapes=scratch,
        compiler_params=pltpu.CompilerParams(vmem_limit_bytes=100 * 2 ** 20),
    )(A_x.reshape(NSEG, L, D), A_wq, A_wk, A_wv, A_wo, A_beta.reshape(1, 32), B_w_r.reshape(8, 128),
      B_w_gate, B_w_up, B_w_down)
    return out.reshape(1, S, D)
```
